```python
import jax
import jax.numpy as jnp

def _softmax(x, axis=-1):
    return jax.nn.softmax(x, axis=axis)

def _gelu(x):
    return jax.nn.gelu(x, approximate=True)

def _silu(x):
    return jax.nn.silu(x)

def _sigmoid(x):
    return jax.nn.sigmoid(x)

def _layernorm(x, axis=-1, eps=1e-05):
    m = jnp.mean(x, axis=axis, keepdims=True)
    v = jnp.var(x, axis=axis, keepdims=True)
    return (x - m) / jnp.sqrt(v + eps)

def _scatter_add(tgt, idx, src, axis=0):
    return tgt.at[idx].add(src)

def _segment_sum(src, seg, n):
    return jax.ops.segment_sum(src, seg, n)

class _Rng:

    def __init__(self, key):
        self._k = key

    def _next(self):
        self._k, sub = jax.random.split(self._k)
        return sub

    def normal(self, shape):
        return jax.random.normal(self._next(), shape, dtype=jnp.bfloat16)

    def randint(self, lo, hi, shape):
        return jax.random.randint(self._next(), shape, lo, hi, dtype=jnp.int32)

    def uniform(self, shape, lo=0.0, hi=1.0):
        return jax.random.uniform(self._next(), shape, jnp.bfloat16, lo, hi)

    def permutation(self, n):
        return jax.random.permutation(self._next(), n)
kernel_name = 'interleave_layers__memory_aug_recurrent_mem_tr__moe_arch_mod__prompt'

def setup_inputs():
    _rng = _Rng(jax.random.key(int.from_bytes(__import__("os").urandom(4), "little")))
    _w = lambda a: (lambda t: t.astype(jnp.bfloat16) if jnp.issubdtype(t.dtype, jnp.floating) else t)(jnp.asarray(a))

    def _A_setup():
        B, S, Dm = (1, 2048, 512)
        H, Dh = (32, 128)
        M, seg = (8, 32)
        seg = min(seg, S)
        S = S // seg * seg
        return {'x': _w((lambda *s: _rng.normal(s) * 0.05)(B, S, Dm)), 'mem0': _w((lambda *s: _rng.normal(s) * 0.05)(B, M, Dm)), 'Wq': _w((lambda *s: _rng.normal(s) * 0.05)(Dm, H, Dh) * Dm ** (-0.5)), 'Wk': _w((lambda *s: _rng.normal(s) * 0.05)(Dm, H, Dh) * Dm ** (-0.5)), 'Wv': _w((lambda *s: _rng.normal(s) * 0.05)(Dm, H, Dh) * Dm ** (-0.5)), 'Wo': _w((lambda *s: _rng.normal(s) * 0.05)(H, Dh, Dm) * (H * Dh) ** (-0.5)), 'seg_len': seg}
    _A_in = _A_setup()

    def _B_setup():
        B, S, D, F, C = (1, 2048, 512, 1792, 1)
        return {'x': _w((lambda *s: _rng.normal(s) * 0.05)(B, S, D)), 'w_r': _w((lambda *s: _rng.normal(s) * 0.05)(D)), 'w_gate': _w((lambda *s: _rng.normal(s) * 0.05)(D, F)), 'w_up': _w((lambda *s: _rng.normal(s) * 0.05)(D, F)), 'w_down': _w((lambda *s: _rng.normal(s) * 0.05)(F, D))}
    _B_in = _B_setup()
    return {'A_x': _A_in['x'], 'A_mem0': _A_in['mem0'], 'A_Wq': _A_in['Wq'], 'A_Wk': _A_in['Wk'], 'A_Wv': _A_in['Wv'], 'A_Wo': _A_in['Wo'], 'A_seg_len': _A_in['seg_len'], 'B_x': _B_in['x'], 'B_w_r': _B_in['w_r'], 'B_w_gate': _B_in['w_gate'], 'B_w_up': _B_in['w_up'], 'B_w_down': _B_in['w_down']}

def reference(A_x, A_mem0, A_Wq, A_Wk, A_Wv, A_Wo, A_seg_len, B_x, B_w_r, B_w_gate, B_w_up, B_w_down):

    def _A_ref(x, mem0, Wq, Wk, Wv, Wo, seg_len):
        B, S, Dm = x.shape
        H, Dh = (Wq.shape[1], Wq.shape[2])
        M = mem0.shape[1]
        scale = Dh ** (-0.5)
        n_seg = S // seg_len
        L = M + seg_len
        idx = jnp.arange(L)
        mask = (idx[:, None] < M) | (idx[:, None] >= idx[None, :])
        mem = mem0
        outs = []
        for s in range(n_seg):
            xs = x[:, s * seg_len:(s + 1) * seg_len, :].copy()
            h = jnp.concatenate([mem, xs], axis=1)
            q = jnp.einsum('btd,dhe->bhte', h, Wq)
            k = jnp.einsum('btd,dhe->bhte', h, Wk)
            v = jnp.einsum('btd,dhe->bhte', h, Wv)
            scores = jnp.einsum('bhqe,bhke->bhqk', q, k) * scale
            scores = jnp.where(mask[None, None], scores, -1000000000.0)
            p = _softmax(scores, axis=-1)
            o = jnp.einsum('bhqk,bhke->bhqe', p, v)
            o = jnp.einsum('bhte,hed->btd', o, Wo)
            mem = o[:, :M, :].copy()
            outs.append(o[:, M:, :])
        return jnp.concatenate(outs, axis=1)

    def _B_ref(x, w_r, w_gate, w_up, w_down):
        B, S, D = x.shape
        C = 1
        r = x @ w_r
        idx = jnp.argsort(-r, axis=-1)[:, :C]
        idx_e = jnp.repeat(idx.reshape(B, C, 1), D, axis=2)
        x_sel = jnp.take_along_axis(x, idx_e, axis=1)
        g = _silu(x_sel @ w_gate)
        u = x_sel @ w_up
        y = g * u @ w_down
        r_sel = _sigmoid(jnp.take_along_axis(r, idx, axis=1))
        y = y * r_sel.reshape(B, C, 1)
        b_off = (jnp.arange(B) * S).reshape(B, 1)
        flat_idx = (idx + b_off).reshape(B * C)
        zero = (x * 0.0).reshape(B * S, D)
        upd = _scatter_add(zero, flat_idx, y.reshape(B * C, D), axis=0)
        return x + upd.reshape(B, S, D)
    x = A_x
    x = x + _A_ref(_layernorm(x, axis=-1), A_mem0, A_Wq, A_Wk, A_Wv, A_Wo, A_seg_len)
    x = x + _B_ref(_layernorm(x, axis=-1), B_w_r, B_w_gate, B_w_up, B_w_down)
    x = x + _A_ref(_layernorm(x, axis=-1), A_mem0, A_Wq, A_Wk, A_Wv, A_Wo, A_seg_len)
    x = x + _B_ref(_layernorm(x, axis=-1), B_w_r, B_w_gate, B_w_up, B_w_down)
    return x
```

```python
import functools

import jax
import jax.numpy as jnp
from jax import lax
import jax.experimental.pallas as pl
import jax.experimental.pallas.tpu as pltpu

BF = jnp.bfloat16
F32 = jnp.float32
U32 = jnp.uint32
I32 = jnp.int32


def _rb(v):
    return v.astype(BF).astype(F32)


def _layernorm(x):
    inv_n = 1.0 / x.shape[-1]
    m = jnp.sum(x, axis=-1, keepdims=True) * inv_n
    d = x - m
    v = _rb(jnp.sum(d * d, axis=-1, keepdims=True) * inv_n)
    den = _rb(jnp.sqrt(_rb(v + 1.0013580322265625e-05)))
    return _rb(_rb(x - _rb(m)) * (1.0 / den))


def _dot(a, b):
    return jnp.dot(a, b, preferred_element_type=F32)


def _kernel(x_hbm, mem0_ref, wq_hbm, wk_hbm, wv_hbm, wo_hbm, wr_ref, wg_hbm, wu_hbm, wd_hbm,
            out_hbm,
            raw, wo_raw, w_s, wo_s, xin, xres, hbuf, xmid, outs, wg_s, wu_s, wd_s, sems,
            *, S, D, H, E, M, T):
    NSEG = S // T
    L = M + T
    HP = H // 2

    cp_x = pltpu.make_async_copy(x_hbm, xin, sems.at[0])
    cp_w = [pltpu.make_async_copy(w, raw.at[j], sems.at[1 + j]) for j, w in enumerate((wq_hbm, wk_hbm, wv_hbm))]
    cp_o = pltpu.make_async_copy(wo_hbm, wo_raw, sems.at[4])
    cp_b = [pltpu.make_async_copy(w, s, sems.at[5 + j])
            for j, (w, s) in enumerate(((wg_hbm, wg_s), (wu_hbm, wu_s), (wd_hbm, wd_s)))]
    cp_x.start()
    for c in cp_w:
        c.start()
    cp_o.start()
    for c in cp_b:
        c.start()

    cp_x.wait()
    xres[0] = jnp.zeros((T, D), F32)

    def ln0(i, c):
        for u in range(4):
            s = i * 4 + u
            xv = xin[pl.ds(pl.multiple_of(s * T, T), T), :].astype(F32)
            xres[s + 1] = xv
            hbuf[s + 1] = _layernorm(xv)
        return c
    lax.fori_loop(0, NSEG // 4, ln0, 0)

    raw32 = raw.bitcast(U32)
    for j in range(3):
        cp_w[j].wait()

        def relay(i, c, j=j):
            CH = 64
            src = raw32.at[j, pl.ds(pl.multiple_of(i * CH * HP, CH * HP), CH * HP)]
            dst = pl.ds(pl.multiple_of(i * (CH // 2), CH // 2), CH // 2)
            for p in range(HP):
                w = src[pl.ds(p, CH, stride=HP), :]
                lo = pltpu.bitcast(w << 16, F32).astype(BF)
                hi = pltpu.bitcast(w & jnp.uint32(0xFFFF0000), F32).astype(BF)
                w_s[p, 0, j, dst] = pltpu.bitcast(lo, U32)
                w_s[p, 1, j, dst] = pltpu.bitcast(hi, U32)
            return c
        lax.fori_loop(0, D // 64, relay, 0)
    cp_o.wait()

    def relay_o(a, c):
        wo_s[a] = pltpu.bitcast(wo_raw[pl.ds(pl.multiple_of(a * E, E), E), :], U32)
        return c
    lax.fori_loop(0, H, relay_o, 0)
    for c in cp_b:
        c.wait()

    scale = E ** -0.5
    wr = wr_ref[...].astype(F32)

    def epilogue(slot, o_tok, best, bidx):
        x1 = _rb(xres[slot] + _rb(o_tok))
        xn = _layernorm(x1)
        r = _rb(jnp.sum(xn * wr, axis=-1, keepdims=True))
        x2 = (x1 + xn).astype(BF)
        xmid[slot] = x1
        outs[slot] = x2
        x2 = x2.astype(F32)
        xres[slot] = x2
        hbuf[slot] = _layernorm(x2)
        sub = lax.broadcasted_iota(I32, (8, 128), 0)
        for t in range(T // 8):
            rt = jnp.broadcast_to(r[t * 8:t * 8 + 8], (8, 128))
            it = sub + ((slot - 1) * T + t * 8)
            better = (rt > best) & (it >= 0)
            best = jnp.where(better, rt, best)
            bidx = jnp.where(better, it, bidx)
        return best, bidx

    def step(s, carry):
        mem, o_prev, best, bidx = carry
        best, bidx = epilogue(s, o_prev, best, bidx)
        row = lax.broadcasted_iota(I32, (L, L), 0)
        col = lax.broadcasted_iota(I32, (L, L), 1)
        mask = (row < M) | (row >= col)
        h = jnp.concatenate([mem, hbuf[s + 1]], axis=0)
        G, L1, L2, L3 = 4, 1, 2, 2
        NG = H // G
        q, k, v, p, o = {}, {}, {}, {}, {}
        acc = None
        for t in range(NG + L1 + L2 + L3):
            g = t
            if g < NG:
                for a in range(g * G, g * G + G):
                    q[a], k[a], v[a] = [_dot(h, pltpu.bitcast(w_s[a // 2, a % 2, j], BF)) for j in range(3)]
            g = t - L1
            if 0 <= g < NG:
                for a in range(g * G, g * G + G):
                    sc = lax.dot_general(q[a], k[a].astype(BF), (((1,), (1,)), ((), ())),
                                         preferred_element_type=F32) * scale
                    sc = jnp.where(mask, sc, -1e9)
                    e = jnp.exp(sc - jnp.max(sc, axis=-1, keepdims=True))
                    p[a] = e / jnp.sum(e, axis=-1, keepdims=True)
            g = t - L1 - L2
            if 0 <= g < NG:
                for a in range(g * G, g * G + G):
                    o[a] = _dot(p[a], v[a].astype(BF))
            g = t - L1 - L2 - L3
            if 0 <= g < NG:
                for a in range(g * G, g * G + G):
                    d = _dot(o[a], pltpu.bitcast(wo_s[a], BF))
                    acc = d if acc is None else acc + d
        return _rb(acc[:M]), acc[M:], best, bidx

    def layer(l, c):
        init = (mem0_ref[...].astype(F32), jnp.zeros((T, D), F32),
                jnp.full((8, 128), -jnp.inf, F32), jnp.full((8, 128), S, I32))
        _, o_last, best, bidx = lax.fori_loop(0, NSEG, step, init)
        best, bidx = epilogue(NSEG, o_last, best, bidx)
        top = jnp.max(best, axis=0, keepdims=True)
        idx = jnp.min(jnp.where(best == top, bidx, S))
        idx = jnp.where(idx >= S, 0, idx)
        slot = idx // T + 1
        x1 = xmid[slot]
        xn = _layernorm(x1)
        r = _rb(jnp.sum(xn * wr, axis=-1, keepdims=True))
        g = _rb(_dot(xn, wg_s[...]))
        u = _rb(_dot(xn, wu_s[...]))
        g = _rb(g * _rb(jax.nn.sigmoid(g)))
        y = _rb(_dot(_rb(g * u), wd_s[...]))
        y = _rb(y * _rb(jax.nn.sigmoid(r)))
        sel = lax.broadcasted_iota(I32, (T, D), 0) == idx % T
        x2 = (x1 + _rb(xn + jnp.where(sel, y, 0.0))).astype(BF)
        outs[slot] = x2
        x2 = x2.astype(F32)
        xres[slot] = x2
        hbuf[slot] = _layernorm(x2)
        return c

    lax.fori_loop(0, 2, layer, 0)
    cp = pltpu.make_async_copy(outs.at[pl.ds(1, NSEG)], out_hbm, sems.at[0])
    cp.start()
    cp.wait()


@functools.partial(jax.jit, static_argnames=("A_seg_len",))
def pallas_interleave_layers__memory_aug_recurrent_mem_tr__moe_arch_mod__prompt_kernel(
    A_x, A_mem0, A_Wq, A_Wk, A_Wv, A_Wo, A_seg_len, B_x, B_w_r, B_w_gate, B_w_up, B_w_down,
):
    del B_x
    B, S, D = A_x.shape
    _, H, E = A_Wq.shape
    M = A_mem0.shape[1]
    F = B_w_gate.shape[1]
    T = int(A_seg_len)
    assert B == 1 and S % T == 0
    NSEG = S // T
    hbm = pl.BlockSpec(memory_space=pl.ANY)
    vmem = pl.BlockSpec(memory_space=pltpu.VMEM)
    out = pl.pallas_call(
        functools.partial(_kernel, S=S, D=D, H=H, E=E, M=M, T=T),
        out_shape=jax.ShapeDtypeStruct((NSEG, T, D), A_x.dtype),
        in_specs=[hbm, vmem, hbm, hbm, hbm, hbm, vmem, hbm, hbm, hbm],
        out_specs=hbm,
        scratch_shapes=[
            pltpu.VMEM((3, D * H, E), BF),
            pltpu.VMEM((H * E, D), BF),
            pltpu.VMEM((H // 2, 2, 3, D // 2, E), U32),
            pltpu.VMEM((H, E // 2, D), U32),
            pltpu.VMEM((S, D), BF),
            pltpu.VMEM((NSEG + 1, T, D), F32),
            pltpu.VMEM((NSEG + 1, T, D), F32),
            pltpu.VMEM((NSEG + 1, T, D), F32),
            pltpu.VMEM((NSEG + 1, T, D), BF),
            pltpu.VMEM((D, F), BF),
            pltpu.VMEM((D, F), BF),
            pltpu.VMEM((F, D), BF),
            pltpu.SemaphoreType.DMA((8,)),
        ],
        compiler_params=pltpu.CompilerParams(vmem_limit_bytes=100 * 2**20),
        name="rmt_mod",
    )(
        A_x.reshape(S, D), A_mem0.reshape(M, D),
        A_Wq.reshape(D * H, E), A_Wk.reshape(D * H, E), A_Wv.reshape(D * H, E), A_Wo.reshape(H * E, D),
        B_w_r.reshape(1, D), B_w_gate, B_w_up, B_w_down,
    )
    return out.reshape(B, S, D)
```

```python
import functools

import jax
import jax.numpy as jnp
from jax import lax
import jax.experimental.pallas as pl
import jax.experimental.pallas.tpu as pltpu

BF = jnp.bfloat16
F32 = jnp.float32
U32 = jnp.uint32
I32 = jnp.int32

GS = 4
PRE = 6

SEQ_FULL = ("LL....L....L...L....L....L...L....L...EL..q..q....L...L....p...L....p..q...L..q....L....L....p...L..q..q"
            "....p...L....N....p..q..oNoooopooqoooNoooNoooopooopoooNooooNooooo")
SEQ_LIGHT = ("NNE..................q.......N.....q......p.....q......p.....q......p.....q......p.....q......p.....q"
             "......p.....ooqoooooopooooNoooooNooooopoooooNooooo")


def _rb(v):
    return v.astype(BF).astype(F32)


def _pack(v):
    return pltpu.bitcast(v.astype(BF), U32)


def _unpack(w):
    return pltpu.bitcast(w, BF)


def _layernorm(x):
    inv_n = 1.0 / x.shape[-1]
    m = jnp.sum(x, axis=-1, keepdims=True) * inv_n
    d = x - m
    v = _rb(jnp.sum(d * d, axis=-1, keepdims=True) * inv_n)
    den = _rb(jnp.sqrt(_rb(v + 1.0013580322265625e-05)))
    return _rb(_rb(x - _rb(m)) * (1.0 / den))


def _dot(a, b):
    return jnp.dot(a, b, preferred_element_type=F32)


def _strassen_rhs(b11, b12, b21, b22):
    return (b11, b21 - b11, b12 - b22, b22, b11 + b22, b11 + b12, b21 + b22)


def _kernel(x_hbm, mem0_ref, wq_hbm, wk_hbm, wv_hbm, wo_hbm, wr_ref, wg_hbm, wu_hbm, wd_hbm,
            out_hbm,
            raw, stg, wo_raw, ws, wos, xbuf, xmid, hc, hn, tq, on, oc, to, state, bidx_ref,
            wg_s, wu_s, wd_s, sems,
            *, S, D, H, E, M, T):
    NG = S // (T * GS)
    L = M + T
    TH = T // 2
    DH = D // 2
    NP = H // 2
    NHG = H // 8
    NC = 3 * NHG
    GR = GS * TH
    R = tq.shape[0]
    w_hbm = (wq_hbm, wk_hbm, wv_hbm)

    def cp_w(j, hg):
        return pltpu.make_async_copy(w_hbm[j].at[:, hg], raw.at[j * NHG + hg], sems.at[j * NHG + hg])

    def cp_o(k):
        return pltpu.make_async_copy(wo_hbm.at[k], wo_raw.at[k], sems.at[NC + k])

    def cp_x(lo, hi, k):
        return pltpu.make_async_copy(x_hbm.at[pl.ds(lo, hi - lo)], xbuf.at[pl.ds(lo, hi - lo)], sems.at[NC + NHG + k])

    def cp_out(lo, hi, k):
        return pltpu.make_async_copy(xbuf.at[pl.ds(lo, hi - lo)], out_hbm.at[pl.ds(lo, hi - lo)], sems.at[NC + NHG + k])

    cp_b = [pltpu.make_async_copy(w, s, sems.at[NC + NHG + 2 + j])
            for j, (w, s) in enumerate(((wg_hbm, wg_s), (wu_hbm, wu_s), (wd_hbm, wd_s)))]

    def start_chunk(c):
        for j in range(3):
            @pl.when(c // NHG == j)
            def _(j=j):
                cp_w(j, c % NHG).start()

        @pl.when(c // NHG == 3)
        def _():
            cp_o(c % NHG).start()

    def prenorm(g, u):
        h = _layernorm(xbuf[g, u].astype(F32))
        a11, a12, a21, a22 = h[:TH, :DH], h[:TH, DH:], h[TH:, :DH], h[TH:, DH:]
        for m, v in enumerate((a21 + a22, a22, a11, a11 + a12)):
            hc[g, u, m] = v
        for m, v in enumerate((a11 + a22, a21 - a11, a12 - a22)):
            hn[m, g, u] = _pack(v)

    def group_lhs(m, g):
        return _unpack(hn[m, g].reshape(GR // 2, DH))

    cp_x(0, PRE, 0).start()
    cp_w(0, 0).start()
    cp_w(0, 1).start()
    zero_bf = jnp.zeros((GS, T, D), BF)
    xbuf[NG] = zero_bf
    for k in range(4):
        oc[k] = jnp.zeros(oc.shape[1:], F32)
    to[...] = jnp.zeros(to.shape, F32)
    on[1] = jnp.zeros(on.shape[1:], U32)
    cp_x(0, PRE, 0).wait()

    def norm0(g, c):
        for u in range(GS):
            prenorm(g, u)
        return c
    lax.fori_loop(0, PRE, norm0, 0)

    def prep_qkv(c, carry):
        start_chunk(c + 2)
        pltpu.make_async_copy(raw.at[c], raw.at[c], sems.at[c]).wait()
        stg[:D * 4] = pltpu.bitcast(raw[c].reshape(D * 8, E), U32)
        lhs = [_unpack(hn[m, :PRE].reshape(PRE * GR // 2, DH)) for m in range(3)]
        for i in range(4):
            w1 = stg[pl.ds(i, DH, stride=4), :]
            w2 = stg[pl.ds(DH * 4 + i, DH, stride=4), :]
            ops = _strassen_rhs(pltpu.bitcast(w1 << 16, F32), pltpu.bitcast(w1 & jnp.uint32(0xFFFF0000), F32),
                                pltpu.bitcast(w2 << 16, F32), pltpu.bitcast(w2 & jnp.uint32(0xFFFF0000), F32))
            ops = [_pack(v) for v in ops]
            for m in range(7):
                ws[c, i, m] = ops[m]
            m1 = _dot(lhs[0], _unpack(ops[4]))
            tq[:PRE, c, i, 0] = (m1 + _dot(lhs[2], _unpack(ops[6]))).reshape(PRE, GR, E)
            tq[:PRE, c, i, 1] = (m1 + _dot(lhs[1], _unpack(ops[5]))).reshape(PRE, GR, E)
        return carry
    lax.fori_loop(0, NC, prep_qkv, 0)
    for k in range(2, NHG):
        cp_o(k).start()

    def prep_o(k, carry):
        cp_o(k).wait()
        for i in range(4):
            wa = wo_raw[k, 2 * i].astype(F32)
            wb = wo_raw[k, 2 * i + 1].astype(F32)
            for m, v in enumerate(_strassen_rhs(wa[:, :DH], wa[:, DH:], wb[:, :DH], wb[:, DH:])):
                wos[m, k, pl.ds(i * (E // 2), E // 2)] = _pack(v)
        return carry
    lax.fori_loop(0, NHG, prep_o, 0)
    cp_x(PRE, NG, 1).start()
    for c in cp_b:
        c.start()

    def reset_state():
        state[:M] = mem0_ref[...].astype(F32)
        state[M:] = jnp.full((8, D), -jnp.inf, F32)
        bidx_ref[...] = jnp.full((8, 128), S, I32)
    reset_state()

    def router(xn):
        return _rb(jnp.sum(xn * wr_ref[...].astype(F32), axis=-1, keepdims=True))

    def epilogue(g, u, slot, best, bidx):
        rows = pl.ds(u * TH, TH)
        c = oc[slot, u]
        top = jnp.concatenate([c[:TH, :DH] + to[slot % 2, 0, rows], c[:TH, DH:]], axis=1)
        bot = jnp.concatenate([c[TH:, :DH], c[TH:, DH:] + to[slot % 2, 1, rows]], axis=1)
        x1 = (xbuf[g, u].astype(F32) + _rb(jnp.concatenate([top, bot], axis=0))).astype(BF)
        xmid[g, u] = x1
        x1 = x1.astype(F32)
        xn = _layernorm(x1)
        r = router(xn)
        xbuf[g, u] = (x1 + xn).astype(BF)
        sub = lax.broadcasted_iota(I32, (8, 128), 0)
        for t in range(T // 8):
            it = sub + ((g * GS + u) * T + t * 8)
            rt = jnp.where(it < S, jnp.broadcast_to(r[t * 8:t * 8 + 8], (8, 128)), -jnp.inf)
            better = rt > best
            best = jnp.where(better, rt, best)
            bidx = jnp.where(better, it, bidx)
        return best, bidx

    def qkv_group_rounds(g, slot, st):
        units = [(j * NHG + hg, i) for hg in range(NHG) for j in range(3) for i in range(4)]

        def rnd(n, part):
            a, b = units[2 * n], units[2 * n + 1]

            def prod(unit, m):
                return _dot(group_lhs(m, g), _unpack(ws[unit + (4 + m,)]))
            if part == 0:
                st["m1"] = prod(a, 0)
                tq[(slot,) + a + (0,)] = st["m1"] + prod(a, 2)
            elif part == 1:
                tq[(slot,) + a + (1,)] = st.pop("m1") + prod(a, 1)
                st["m1"] = prod(b, 0)
            else:
                tq[(slot,) + b + (0,)] = st["m1"] + prod(b, 2)
                tq[(slot,) + b + (1,)] = st.pop("m1") + prod(b, 1)
        return [functools.partial(rnd, n, part) for n in range(len(units) // 2) for part in range(3)]

    def out_group_rounds(par, st):
        def rnd(c, m, k):
            cols = pl.ds(c * 128, 128)
            d = _dot(_unpack(on[par, m, k]), _unpack(wos[4 + m, k, :, cols]))
            st["n", m] = d if k == 0 else st["n", m] + d
            if k == NHG - 1 and m == 1:
                to[par, 1, :, cols] = st["n", 0] + st["n", 1]
            if k == NHG - 1 and m == 2:
                to[par, 0, :, cols] = st["n", 0] + st["n", 2]
        return [functools.partial(rnd, c, m, k) for c in range(DH // 128) for m in range(3) for k in range(NHG)]

    def segment(G, u, mem, seq, longs, norms):
        g = G % NG
        st = {}
        row = lax.broadcasted_iota(I32, (L, L), 0)
        col = lax.broadcasted_iota(I32, (L, L), 1)
        mask = (row < M) | (row >= col)
        a1, a2 = mem[:, :DH], mem[:, DH:]
        a12 = a1 + a2
        lhs = [jnp.concatenate([hc[g, u, m], a], axis=0) for m, a in enumerate((a12, a2, a1, a12))]
        rows = pl.ds(u * TH, TH)

        def qkv(p, j, half):
            unit = (j * NHG + p // 4, p % 4)
            for m in (2 * half, 2 * half + 1):
                st[m] = _dot(lhs[m], _unpack(ws[unit + (m,)]))
            if half:
                m2, m4, m3, m5 = st[0], st[1], st[2], st[3]
                ca, cb = m2 + m4, m3 + m5
                c11 = tq[(G % R,) + unit + (0, rows)] + (m4[:TH] - m5[:TH])
                c22 = tq[(G % R,) + unit + (1, rows)] + (m3[:TH] - m2[:TH])
                ha = jnp.concatenate([ca[TH:], c11, ca[:TH]], axis=0)
                hb = jnp.concatenate([cb[TH:], cb[:TH], c22], axis=0)
                st[j, 2 * p] = ha if j == 0 else ha.astype(BF)
                st[j, 2 * p + 1] = hb if j == 0 else hb.astype(BF)

        def scores(n):
            for a in range(4 * n, 4 * n + 4):
                sc = lax.dot_general(st.pop((0, a)), st.pop((1, a)), (((1,), (1,)), ((), ())),
                                     preferred_element_type=F32)
                sc = jnp.where(mask, sc, -1e9 * E ** 0.5)
                e = jnp.exp2((sc - jnp.max(sc, axis=-1, keepdims=True)) * (E ** -0.5 * 1.4426950408889634))
                st["p", a] = e * pltpu.reciprocal(jnp.sum(e, axis=-1, keepdims=True), full_range=False)

        def values(n):
            for a in range(4 * n, 4 * n + 4):
                st["o", a] = _dot(st.pop(("p", a)), st.pop((2, a)))

        def oproj(p, half):
            oa, ob = st["o", 2 * p], st["o", 2 * p + 1]
            k, blk = p // 4, pl.ds((p % 4) * (E // 2), E // 2)
            if half == 0:
                st["ab", p] = oa + ob
                left = [jnp.concatenate([v[:M], v[M + TH:]], axis=0) for v in (st["ab", p], ob)]
            else:
                left = [oa[:M + TH], st["ab", p][:M + TH]]
                a11, a12_, a21, a22 = oa[M:M + TH], ob[M:M + TH], oa[M + TH:], ob[M + TH:]
                for m, v in enumerate((a11 + a22, a21 - a11, a12_ - a22)):
                    on[G % 2, m, k, pl.ds(u * (TH // 2), TH // 2), pl.ds((p % 4) * E, E)] = _pack(v)
            for m, v in zip((2 * half, 2 * half + 1), left):
                d = _dot(v, _unpack(wos[m, k, blk]))
                st["acc", m] = d if p == 0 else st["acc", m] + d

        chain = [functools.partial(qkv, p, j, half)
                 for n in range(H // 4) for j in range(3) for p in (2 * n, 2 * n + 1) for half in (0, 1)]
        chain += [functools.partial(oproj, p, half) for p in range(NP) for half in (0, 1)]
        chain = iter(chain)
        its = {".": chain, "o": chain, "L": longs[0], "N": longs[1], "E": iter([norms]),
               "q": iter([functools.partial(scores, n) for n in range(H // 4)]),
               "p": iter([functools.partial(values, n) for n in range(H // 4)])}
        for ch in seq:
            next(its[ch])()
        assert all(next(its[ch], None) is None for ch in ".qpE")
        m2, m4, m3, m5 = (st["acc", m] for m in range(4))
        ca, cb = m2 + m4, m3 + m5
        oc[G % 4, u, :TH, :DH] = m4[M:] - m5[M:]
        oc[G % 4, u, :TH, DH:] = cb[M:]
        oc[G % 4, u, TH:, :DH] = ca[M:]
        oc[G % 4, u, TH:, DH:] = m3[M:] - m2[M:]
        return _rb(jnp.concatenate([ca[:M], cb[:M]], axis=1))

    def group(G, full):
        g = G % NG
        mem, top = state[:M], [state[M:, :128], bidx_ref[...]]
        longs = [iter(qkv_group_rounds((G + 1) % NG, (G + 1) % R, {}) if full else []),
                 iter(out_group_rounds((G + 1) % 2, {}))]

        def norms(u):
            top[:] = epilogue(jnp.where(g >= 2, g - 2, NG), u, (G + 2) % 4, *top)
            prenorm((G + 2) % NG, u)
        for u in range(GS):
            mem = segment(G, u, mem, SEQ_FULL if full else SEQ_LIGHT, longs, functools.partial(norms, u))
        assert all(next(it, None) is None for it in longs)
        state[:M] = mem
        state[M:, :128], bidx_ref[...] = top

    def finish_layer(G):
        last = G == 2 * NG - 1
        best, bidx = state[M:, :128], bidx_ref[...]
        for u in range(GS):
            best, bidx = epilogue(NG - 2, u, (NG - 2) % 4, best, bidx)
        for f in out_group_rounds((NG - 1) % 2, {}):
            f()
        for u in range(GS):
            best, bidx = epilogue(NG - 1, u, (NG - 1) % 4, best, bidx)

        @pl.when(last)
        def _():
            cp_out(NG - 3, NG, 1).start()

        top = jnp.max(best, axis=0, keepdims=True)
        idx = jnp.min(jnp.where(best == top, bidx, S))
        idx = jnp.where(idx >= S, 0, idx)
        g, u = idx // (T * GS), (idx // T) % GS
        x1 = xmid[g, u].astype(F32)
        xn = _layernorm(x1)
        sel = lax.broadcasted_iota(I32, (T, D), 0) == idx % T
        xs = jnp.where(sel, xn, 0.0)
        xs = sum(xs[t * 8:t * 8 + 8] for t in range(T // 8))
        gate = _rb(_dot(xs, wg_s[...]))
        up = _rb(_dot(xs, wu_s[...]))
        gate = _rb(gate * _rb(jax.nn.sigmoid(gate)))
        y = _rb(_dot(_rb(gate * up), wd_s[...]))
        y = _rb(y * _rb(jax.nn.sigmoid(router(xs))))
        y = jnp.concatenate([y] * (T // 8), axis=0)
        x2 = (x1 + _rb(xn + jnp.where(sel, y, 0.0))).astype(BF)

        @pl.when(last)
        def _():
            cp_out(0, NG - 3, 0).wait()
            cp_out(NG - 3, NG, 1).wait()
            xbuf[g, u] = x2
            cp = pltpu.make_async_copy(xbuf.at[g, u], out_hbm.at[g, u], sems.at[0])
            cp.start()
            cp.wait()

        @pl.when(jnp.logical_not(last))
        def _():
            xbuf[g, u] = x2
            prenorm(g, u)
            reset_state()

            @pl.when(g == 0)
            def _():
                def redo(c, carry):
                    for i in range(4):
                        m1, m6, m7 = (_dot(group_lhs(m, 0), _unpack(ws[c, i, 4 + m])) for m in range(3))
                        tq[NG % R, c, i, 0] = m1 + m7
                        tq[NG % R, c, i, 1] = m1 + m6
                    return carry
                lax.fori_loop(0, NC, redo, 0)

    def iteration(G, carry):
        @pl.when(G == PRE - 2)
        def _():
            cp_x(PRE, NG, 1).wait()
            for c in cp_b:
                c.wait()

        @pl.when(G == 2 * NG - 1)
        def _():
            cp_out(0, NG - 3, 0).start()

        light = jnp.logical_or(G < PRE - 1, G == 2 * NG - 1)
        pl.when(light)(lambda: group(G, False))
        pl.when(jnp.logical_not(light))(lambda: group(G, True))
        pl.when(G % NG == NG - 1)(lambda: finish_layer(G))
        return carry

    lax.fori_loop(0, 2 * NG, iteration, 0)


@functools.partial(jax.jit, static_argnames=("A_seg_len",))
def pallas_interleave_layers__memory_aug_recurrent_mem_tr__moe_arch_mod__prompt_kernel(
    A_x, A_mem0, A_Wq, A_Wk, A_Wv, A_Wo, A_seg_len, B_x, B_w_r, B_w_gate, B_w_up, B_w_down,
):
    del B_x
    B, S, D = A_x.shape
    _, H, E = A_Wq.shape
    M = A_mem0.shape[1]
    F = B_w_gate.shape[1]
    T = int(A_seg_len)
    assert (B, S, D, H, E, M, T) == (1, 2048, 512, 32, 128, 8, 32)
    NG = S // (T * GS)
    NHG = H // 8
    GR = GS * T // 2
    hbm = pl.BlockSpec(memory_space=pl.ANY)
    vmem = pl.BlockSpec(memory_space=pltpu.VMEM)
    out = pl.pallas_call(
        functools.partial(_kernel, S=S, D=D, H=H, E=E, M=M, T=T),
        out_shape=jax.ShapeDtypeStruct((NG, GS, T, D), A_x.dtype),
        in_specs=[hbm, vmem, hbm, hbm, hbm, hbm, vmem, hbm, hbm, hbm],
        out_specs=hbm,
        scratch_shapes=[
            pltpu.VMEM((3 * NHG, D, 8, E), BF),
            pltpu.VMEM((D * 4 + 8, E), U32),
            pltpu.VMEM((NHG, 8, E, D), BF),
            pltpu.VMEM((3 * NHG, 4, 7, D // 4, E), U32),
            pltpu.VMEM((7, NHG, 2 * E, D // 2), U32),
            pltpu.VMEM((NG + 1, GS, T, D), BF),
            pltpu.VMEM((NG + 1, GS, T, D), BF),
            pltpu.VMEM((NG, GS, 4, T // 2, D // 2), F32),
            pltpu.VMEM((3, NG, GS, T // 4, D // 2), U32),
            pltpu.VMEM((PRE, 3 * NHG, 4, 2, GR, E), F32),
            pltpu.VMEM((2, 3, NHG, GR // 2, 4 * E), U32),
            pltpu.VMEM((4, GS, T, D), F32),
            pltpu.VMEM((2, 2, GR, D // 2), F32),
            pltpu.VMEM((M + 8, D), F32),
            pltpu.VMEM((8, 128), I32),
            pltpu.VMEM((D, F), BF),
            pltpu.VMEM((D, F), BF),
            pltpu.VMEM((F, D), BF),
            pltpu.SemaphoreType.DMA((4 * NHG + 5,)),
        ],
        compiler_params=pltpu.CompilerParams(vmem_limit_bytes=116 * 2**20),
        name="rmt_mod",
    )(
        A_x.reshape(NG, GS, T, D), A_mem0.reshape(M, D),
        A_Wq.reshape(D, NHG, 8, E), A_Wk.reshape(D, NHG, 8, E), A_Wv.reshape(D, NHG, 8, E),
        A_Wo.reshape(NHG, 8, E, D),
        B_w_r.reshape(1, D), B_w_gate, B_w_up, B_w_down,
    )
    return out.reshape(B, S, D)
```

```python
import functools

import jax
import jax.numpy as jnp
from jax import lax
import jax.experimental.pallas as pl
import jax.experimental.pallas.tpu as pltpu

BF = jnp.bfloat16
F32 = jnp.float32
U32 = jnp.uint32
I32 = jnp.int32

GS = 4
PRE = 6

SEQ_FULL = (
    "L....L...L....HL...L..q...EL...EL....EL..q...EL....L...L....p...L....L..q..q....p...L..q...L....p...L....p...L....L..q...p...N..q...pooqooooNooooNoooopoooNoooopoooNooooNoooo",
    "L....L...L....HL...L..q...EL...EL....EL..q...EL....L...L....p...L....L..q..q....p...L..q...L....p...L....p...L....L..q...p...N..q...pooqooooNooooNoooopoooNoooopoooNooooNoooo",
    "L....L...L....HL...L..q...EL...EL....EL..q...EL....L...L....p...L....L..q..q....p...L..q...L....p...L....p...L....L..q...p...N..q...pooqooooNooooNoooopoooNoooopoooNooooNoooo",
    "L....L...L....HL...L..q...EL...EL....EL..q...EL....L...L....p...L....L..q..q....p...L..q...L....p...L....p...L....L..q...p...N..q...pooqooooNooooNoooopoooNoooopoooNooooNoooo",
)
SEQ_LIGHT = (
    "N........N......N...q......H.....q.....E......p...p...q....E......q....p......q.....E.....q....p...p....E...q....N...opooooopooqoooooNooooNoooopooooooooooo",
    "N........N......N...q......H.....q.....E......p...p...q....E......q....p......q.....E.....q....p...p....E...q....N...opooooopooqoooooNooooNoooopooooooooooo",
    "N........N......N...q......H.....q.....E......p...p...q....E......q....p......q.....E.....q....p...p....E...q....N...opooooopooqoooooNooooNoooopooooooooooo",
    "N........N......N...q......H.....q.....E......p...p...q....E......q....p......q.....E.....q....p...p....E...q....N...opooooopooqoooooNooooNoooopooooooooooo",
)


def _rb(v):
    return v.astype(BF).astype(F32)


def _pack(v):
    return pltpu.bitcast(v.astype(BF), U32)


def _unpack(w):
    return pltpu.bitcast(w, BF)


def _layernorm(x):
    inv_n = 1.0 / x.shape[-1]
    m = jnp.sum(x, axis=-1, keepdims=True) * inv_n
    d = x - m
    v = _rb(jnp.sum(d * d, axis=-1, keepdims=True) * inv_n)
    den = _rb(jnp.sqrt(_rb(v + 1.0013580322265625e-05)))
    return _rb(_rb(x - _rb(m)) * (1.0 / den))


def _dot(a, b):
    return jnp.dot(a, b, preferred_element_type=F32)


def _strassen_rhs(b11, b12, b21, b22):
    return (b11, b21 - b11, b12 - b22, b22, b11 + b22, b11 + b12, b21 + b22)


def _kernel(x_hbm, mem0_ref, wq_hbm, wk_hbm, wv_hbm, wo_hbm, wr_ref, wg_hbm, wu_hbm, wd_hbm,
            out_hbm,
            raw, wo_raw, ws, wos, xbuf, xmid, hc, hn, tq, on, oc, to, state, bidx_ref,
            wg_s, wu_s, wd_s, sems,
            *, S, D, H, E, M, T):
    NG = S // (T * GS)
    L = M + T
    TH = T // 2
    DH = D // 2
    NP = H // 2
    NHG = H // 8
    NC = 3 * NHG
    GR = GS * TH
    R = PRE
    NO = 3
    w_hbm = (wq_hbm, wk_hbm, wv_hbm)

    def cp_w(j, hg):
        return pltpu.make_async_copy(w_hbm[j].at[:, hg], raw.at[j * NHG + hg], sems.at[j * NHG + hg])

    def cp_o(k):
        return pltpu.make_async_copy(wo_hbm.at[k], wo_raw.at[k], sems.at[NC + k])

    def cp_x(lo, hi, k):
        return pltpu.make_async_copy(x_hbm.at[pl.ds(lo, hi - lo)], xbuf.at[pl.ds(lo, hi - lo)], sems.at[NC + NHG + k])

    def cp_out(lo, hi, k):
        return pltpu.make_async_copy(xbuf.at[pl.ds(lo, hi - lo)], out_hbm.at[pl.ds(lo, hi - lo)], sems.at[NC + NHG + k])

    cp_b = [pltpu.make_async_copy(w, s, sems.at[NC + NHG + 2 + j])
            for j, (w, s) in enumerate(((wg_hbm, wg_s), (wu_hbm, wu_s), (wd_hbm, wd_s)))]

    def normed(x):
        x = x.astype(F32)
        d = x - jnp.sum(x, axis=-1, keepdims=True) * (1.0 / D)
        return d * lax.rsqrt(jnp.sum(d * d, axis=-1, keepdims=True) * (1.0 / D) + 1e-5)

    def prenorm(g, u):
        store_lhs(g, u, normed(xbuf[g, u]))

    def store_lhs(g, u, h):
        a11, a12, a21, a22 = h[:TH, :DH], h[:TH, DH:], h[TH:, :DH], h[TH:, DH:]
        for m, v in enumerate((a21 + a22, a22, a11, a11 + a12)):
            hc[g, u, m] = v
        for m, v in enumerate((a11 + a22, a21 - a11, a12 - a22)):
            hn[m, g, u] = _pack(v)

    def t_rows(i, k, start=0, size=GR):
        return pl.ds((2 * i + k) * GR + start, size)

    def group_lhs(m, g):
        return _unpack(hn[m, g].reshape(GR // 2, DH))

    cp_x(0, PRE, 0).start()
    for c in range(NC):
        cp_w(c // NHG, c % NHG).start()
    for k in range(NHG):
        cp_o(k).start()
    cp_x(PRE, NG, 1).start()
    for c in cp_b:
        c.start()
    zero_bf = jnp.zeros((GS, T, D), BF)
    xbuf[NG] = zero_bf
    oc[...] = jnp.zeros(oc.shape, F32)
    on[1] = jnp.zeros(on.shape[1:], U32)
    to[...] = jnp.zeros(to.shape, F32)
    cp_x(0, PRE, 0).wait()

    norm = normed(xbuf[:PRE].reshape(PRE * GS * T, D))
    for n in range(PRE * GS):
        store_lhs(n // GS, n % GS, norm[n * T:n * T + T])

    def prep_qkv(c, part):
        n, i = divmod(part, 4)
        r, spare = 32 * n, R + c % 2
        if i == 0:
            for k in range(2):
                words = pltpu.bitcast(raw[c, pl.ds(k * DH + r, 32)].reshape(256, E), U32)
                tq[spare, n, pl.ds(k * 128, 128)] = pltpu.bitcast(words, F32)
        w1, w2 = (pltpu.bitcast(tq[spare, n, pl.ds(k * 128 + i, 32, stride=4), :], U32) for k in range(2))
        ops = _strassen_rhs(pltpu.bitcast(w1 << 16, F32), pltpu.bitcast(w1 & jnp.uint32(0xFFFF0000), F32),
                            pltpu.bitcast(w2 << 16, F32), pltpu.bitcast(w2 & jnp.uint32(0xFFFF0000), F32))
        for m, v in enumerate(ops):
            ws[c, i, m, pl.ds(r // 2, 16)] = _pack(v)

    def prep_o(k, part, spare=None):
        i, r = divmod(part * 16, E)
        for col in range(0, DH, E):
            w = [pltpu.bitcast(wo_raw[k, 2 * i + a, pl.ds(r, 16), pl.ds(b * DH + col, E)], U32)
                 for a in range(2) for b in range(2)]
            if spare is not None:
                tq[spare, k, pl.ds(part * 16 + col // E * 8, 8)] = pltpu.bitcast(w[0], F32)
                w[0] = pltpu.bitcast(tq[spare, k, pl.ds(part * 16 + col // E * 8, 8)], U32)
            ops = [_pack(v) for v in _strassen_rhs(*(_unpack(v).astype(F32) for v in w))]
            ops[0], ops[3] = w[0], w[3]
            for m, v in enumerate(ops):
                wos[m, k, pl.ds(part * 8, 8), pl.ds(col, E)] = v

    def ahead_qkv(c, others):
        others = iter(others)
        for n in range(2):
            for m in (0, 2, 1):
                lhs = _unpack(hn[m, :PRE].reshape(PRE * GR // 2, DH))
                res = [(i, _dot(lhs, _unpack(ws[c, i, 4 + m]))) for i in (2 * n, 2 * n + 1)]
                for g in range(PRE):
                    next(others, lambda: None)()
                    for i, v in res:
                        v = v[g * GR:g * GR + GR]
                        tq[g, c, t_rows(i, int(m != 2))] = v if m == 0 else v + tq[g, c, t_rows(i, 1)]
        assert next(others, None) is None

    cp_w(0, 0).wait()
    for part in range(32):
        prep_qkv(0, part)

    def stream(c, carry):
        @pl.when(c < NC - 1)
        def _():
            pltpu.make_async_copy(raw.at[c + 1], raw.at[c + 1], sems.at[c + 1]).wait()
            ahead_qkv(c, [functools.partial(prep_qkv, c + 1, part) for part in range(32)])

        @pl.when(c == NC - 1)
        def _():
            for k in range(NO):
                cp_o(k).wait()
            ahead_qkv(c, [lambda part=part: [prep_o(k, part, R + c % 2) for k in range(NO)] for part in range(32)])
        return carry
    lax.fori_loop(0, NC, stream, 0)
    for k in range(NO, NHG):
        cp_o(k).wait()
        for part in range(32):
            prep_o(k, part)

    def reset_state():
        state[:M] = mem0_ref[...].astype(F32)
        state[M:] = jnp.full((8, D), -jnp.inf, F32)
        bidx_ref[:, :128] = jnp.full((8, 128), S, I32)
    reset_state()

    def router(xn):
        return _rb(jnp.sum(xn * wr_ref[...].astype(F32).reshape(1, D), axis=-1, keepdims=True))

    def epilogue(g, u, t, par, best, bidx):
        rows = pl.ds(t * 8, 8)
        half = t * 8 // TH
        c = oc[par, u, rows]
        n = to[par, half, pl.ds(u * TH + t * 8 % TH, 8)]
        c = jnp.concatenate([c[:, :DH] + n, c[:, DH:]] if half == 0 else [c[:, :DH], c[:, DH:] + n], axis=1)
        x1 = _rb(xbuf[g, u, rows].astype(F32) + _rb(c))
        xn = _layernorm(x1)
        xmid[0, g, u, rows] = x1
        xmid[1, g, u, rows] = xn
        xbuf[g, u, rows] = (x1 + xn).astype(BF)
        it = lax.broadcasted_iota(I32, (8, 128), 0) + ((g * GS + u) * T + t * 8)
        r = jnp.where(it < S, jnp.broadcast_to(router(xn), (8, 128)), -jnp.inf)
        better = r > best
        return jnp.where(better, r, best), jnp.where(better, it, bidx)

    def qkv_group_rounds(g, slot, st):
        units = [(j * NHG + hg, i) for hg in range(NHG) for j in range(3) for i in range(4)]

        def rnd(n, part):
            a, b = units[2 * n], units[2 * n + 1]

            def prod(unit, m):
                return _dot(group_lhs(m, g), _unpack(ws[unit + (4 + m,)]))
            if part == 0:
                st["m1"] = prod(a, 0)
                tq[slot, a[0], t_rows(a[1], 0)] = st["m1"] + prod(a, 2)
            elif part == 1:
                tq[slot, a[0], t_rows(a[1], 1)] = st.pop("m1") + prod(a, 1)
                st["m1"] = prod(b, 0)
            else:
                tq[slot, b[0], t_rows(b[1], 0)] = st["m1"] + prod(b, 2)
                tq[slot, b[0], t_rows(b[1], 1)] = st.pop("m1") + prod(b, 1)
        return [functools.partial(rnd, n, part) for n in range(len(units) // 2) for part in range(3)]

    def out_group_rounds(par, st):
        def rnd(c, m, k):
            cols = pl.ds(c * 128, 128)
            d = _dot(_unpack(on[par, m, k]), _unpack(wos[4 + m, k, :, cols]))
            st["n", m] = d if k == 0 else d + st["n", m]
            if k == NHG - 1 and m == 1:
                to[par, 1, :, cols] = st["n", 0] + st["n", 1]
            if k == NHG - 1 and m == 2:
                to[par, 0, :, cols] = st["n", 0] + st["n", 2]
        return [functools.partial(rnd, c, m, k) for c in range(DH // 128) for m in range(3) for k in range(NHG)]

    def segment(G, par, u, mem, seq, longs, norms):
        g = G % NG
        st = {}
        row = lax.broadcasted_iota(I32, (L, L), 0)
        col = lax.broadcasted_iota(I32, (L, L), 1)
        mask = (row < M) | (row >= col)
        a1, a2 = mem[:, :DH], mem[:, DH:]
        a12 = a1 + a2
        lhs = [jnp.concatenate([hc[g, u, m], a], axis=0) for m, a in enumerate((a12, a2, a1, a12))]

        def qkv(*prods):
            for p, j, m in prods:
                unit = (j * NHG + p // 4, p % 4)
                st[p, j, m] = _dot(lhs[m], _unpack(ws[unit + (m,)]))
                if m == 3:
                    m2, m4, m3, m5 = (st.pop((p, j, k)) for k in range(4))
                    ca, cb = m2 + m4, m3 + m5
                    c11 = tq[G % R, unit[0], t_rows(unit[1], 0, u * TH, TH)] + (m4[:TH] - m5[:TH])
                    c22 = tq[G % R, unit[0], t_rows(unit[1], 1, u * TH, TH)] + (m3[:TH] - m2[:TH])
                    ha = jnp.concatenate([ca[TH:], c11, ca[:TH]], axis=0)
                    hb = jnp.concatenate([cb[TH:], cb[:TH], c22], axis=0)
                    st[j, 2 * p] = ha if j == 0 else ha.astype(BF)
                    st[j, 2 * p + 1] = hb if j == 0 else hb.astype(BF)

        def scores(n):
            for a in range(4 * n, 4 * n + 4):
                sc = lax.dot_general(st.pop((0, a)), st.pop((1, a)), (((1,), (1,)), ((), ())),
                                     preferred_element_type=F32)
                sc = jnp.where(mask, sc, -1e9 * E ** 0.5)
                e = jnp.exp2((sc - jnp.max(sc, axis=-1, keepdims=True)) * (E ** -0.5 * 1.4426950408889634))
                st["p", a] = e * pltpu.reciprocal(jnp.sum(e, axis=-1, keepdims=True), full_range=False)

        def values(n):
            for a in range(4 * n, 4 * n + 4):
                st["o", a] = _dot(st.pop(("p", a)), st.pop((2, a)))

        def oproj(p, half):
            oa, ob = st["o", 2 * p], st["o", 2 * p + 1]
            k, blk = p // 4, pl.ds((p % 4) * (E // 2), E // 2)
            if half == 0:
                st["ab", p] = oa + ob
                left = [jnp.concatenate([v[:M], v[M + TH:]], axis=0) for v in (st["ab", p], ob)]
            else:
                left = [oa[:M + TH], st["ab", p][:M + TH]]
                a11, a12_, a21, a22 = oa[M:M + TH], ob[M:M + TH], oa[M + TH:], ob[M + TH:]
                for m, v in enumerate((a11 + a22, a21 - a11, a12_ - a22)):
                    on[par, m, k, pl.ds(u * (TH // 2), TH // 2), pl.ds((p % 4) * E, E)] = _pack(v)
            for m, v in zip((2 * half, 2 * half + 1), left):
                d = _dot(v, _unpack(wos[m, k, blk]))
                st["acc", m] = d if p == 0 else d + st["acc", m]

        units = [(p, j) for n in range(H // 4) for j in range(3) for p in (2 * n, 2 * n + 1)]
        prods = [un + (2,) for un in units[:4]] + [un + (m,) for un in units[:4] for m in (0, 1, 3)]
        prods += [un + (m,) for un in units[4:] for m in range(4)]
        chain = [functools.partial(qkv, *prods[k:k + 2]) for k in range(0, len(prods), 2)]
        outs = [(p, half) for p in range(NP - 4) for half in (0, 1)]
        outs += [(p, half) for half in (0, 1) for p in range(NP - 4, NP)]
        its = {".": iter(chain), "o": iter([functools.partial(oproj, *a) for a in outs]),
               "L": longs[0], "N": longs[1], "E": iter(norms[:-1]), "H": iter(norms[-1:]),
               "q": iter([functools.partial(scores, n) for n in range(H // 4)]),
               "p": iter([functools.partial(values, n) for n in range(H // 4)])}
        for ch in seq:
            next(its[ch])()
        assert all(next(its[ch], None) is None for ch in ".oqpEH")
        m2, m4, m3, m5 = (st["acc", m] for m in range(4))
        ca, cb = m2 + m4, m3 + m5
        oc[par, u, :TH, :DH] = m4[M:] - m5[M:]
        oc[par, u, :TH, DH:] = cb[M:]
        oc[par, u, TH:, :DH] = ca[M:]
        oc[par, u, TH:, DH:] = m3[M:] - m2[M:]
        return _rb(jnp.concatenate([ca[:M], cb[:M]], axis=1))

    def group(G, seqs):
        mem, top = state[:M], [state[M:, :128], bidx_ref[:, :128]]
        full = "L" in seqs[0]
        g, par = G % NG, G % 2
        longs = [iter(qkv_group_rounds((G + 1) % NG, (G + 1) % R, {}) if full else []),
                 iter(out_group_rounds(1 - par, {}))]

        def post(u, t):
            top[:] = epilogue(jnp.where(g >= 2, g - 2, NG), u, t, par, *top)
            if full:
                hn[0, NG + par, 0, :, :128] = pltpu.bitcast(top[0], U32)
            else:
                tq[R + par, 0, :8] = top[0]
        for u in range(GS):
            mem = segment(G, par, u, mem, seqs[u], longs,
                          [functools.partial(post, u, t) for t in range(T // 8)]
                          + [functools.partial(prenorm, (G + 2) % NG, u)])
        assert all(next(it, None) is None for it in longs)
        state[:M] = mem
        state[M:, :128], bidx_ref[:, :128] = top

    def finish_layer(last):
        best, bidx = state[M:, :128], bidx_ref[:, :128]
        for par in range(2):
            if par:
                for f in out_group_rounds(par, {}):
                    f()
            for u in range(GS):
                for t in range(T // 8):
                    best, bidx = epilogue(NG - 2 + par, u, t, par, best, bidx)

        @pl.when(last)
        def _():
            cp_out(NG - 3, NG, 1).start()

        top = jnp.max(best, axis=0, keepdims=True)
        idx = jnp.min(jnp.where(best == top, bidx, S))
        idx = jnp.where(idx >= S, 0, idx)
        g, u = idx // (T * GS), idx // T % GS
        rows = pl.ds(pl.multiple_of(idx % T // 8 * 8, 8), 8)
        x1, xn = xmid[0, g, u, rows], xmid[1, g, u, rows]
        gate = _rb(_dot(xn, wg_s[...]))
        up = _rb(_dot(xn, wu_s[...]))
        gate = _rb(gate * _rb(jax.nn.sigmoid(gate)))
        y = _rb(_dot(_rb(gate * up), wd_s[...]))
        y = _rb(y * _rb(jax.nn.sigmoid(router(xn))))
        sel = lax.broadcasted_iota(I32, (8, D), 0) == idx % 8
        x2 = (x1 + _rb(xn + jnp.where(sel, y, 0.0))).astype(BF)

        @pl.when(last)
        def _():
            cp_out(0, NG - 3, 0).wait()
            cp_out(NG - 3, NG, 1).wait()
            xbuf[g, u, rows] = x2
            cp = pltpu.make_async_copy(xbuf.at[g, u], out_hbm.at[g, u], sems.at[0])
            cp.start()
            cp.wait()

        @pl.when(jnp.logical_not(last))
        def _():
            xbuf[g, u, rows] = x2
            prenorm(g, u)
            reset_state()

            @pl.when(g == 0)
            def _():
                def redo(c, carry):
                    for i in range(4):
                        m1, m6, m7 = (_dot(_unpack(hn[m, g, u]), _unpack(ws[c, i, 4 + m])) for m in range(3))
                        tq[(NG + g) % R, c, t_rows(i, 0, pl.multiple_of(u * TH, TH), TH)] = m1 + m7
                        tq[(NG + g) % R, c, t_rows(i, 1, pl.multiple_of(u * TH, TH), TH)] = m1 + m6
                    return carry
                lax.fori_loop(0, NC, redo, 0)

    def iteration(G, carry):
        last = G == 2 * NG - 1

        @pl.when(G == PRE - 2)
        def _():
            cp_x(PRE, NG, 1).wait()
            for c in cp_b:
                c.wait()

        @pl.when(last)
        def _():
            cp_out(0, NG - 3, 0).start()

        light = jnp.logical_or(G < PRE - 1, last)
        pl.when(light)(lambda: group(G, SEQ_LIGHT))
        pl.when(jnp.logical_not(light))(lambda: group(G, SEQ_FULL))
        pl.when(G % NG == NG - 1)(lambda: finish_layer(last))
        return carry

    lax.fori_loop(0, 2 * NG, iteration, 0)


@functools.partial(jax.jit, static_argnames=("A_seg_len",))
def pallas_interleave_layers__memory_aug_recurrent_mem_tr__moe_arch_mod__prompt_kernel(
    A_x, A_mem0, A_Wq, A_Wk, A_Wv, A_Wo, A_seg_len, B_x, B_w_r, B_w_gate, B_w_up, B_w_down,
):
    del B_x
    B, S, D = A_x.shape
    _, H, E = A_Wq.shape
    M = A_mem0.shape[1]
    F = B_w_gate.shape[1]
    T = int(A_seg_len)
    assert (B, S, D, H, E, M, T) == (1, 2048, 512, 32, 128, 8, 32)
    NG = S // (T * GS)
    NHG = H // 8
    GR = GS * T // 2
    hbm = pl.BlockSpec(memory_space=pl.ANY)
    vmem = pl.BlockSpec(memory_space=pltpu.VMEM)
    out = pl.pallas_call(
        functools.partial(_kernel, S=S, D=D, H=H, E=E, M=M, T=T),
        out_shape=jax.ShapeDtypeStruct((NG, GS, T, D), A_x.dtype),
        in_specs=[hbm, vmem, hbm, hbm, hbm, hbm, vmem, hbm, hbm, hbm],
        out_specs=hbm,
        scratch_shapes=[
            pltpu.VMEM((3 * NHG, D, 8, E), BF),
            pltpu.VMEM((NHG, 8, E, D), BF),
            pltpu.VMEM((3 * NHG, 4, 7, D // 4, E), U32),
            pltpu.VMEM((7, NHG, 2 * E, D // 2), U32),
            pltpu.VMEM((NG + 1, GS, T, D), BF),
            pltpu.VMEM((2, NG + 1, GS, T, D), F32),
            pltpu.VMEM((NG, GS, 4, T // 2, D // 2), F32),
            pltpu.VMEM((3, NG + 2, GS, T // 4, D // 2), U32),
            pltpu.VMEM((PRE + 2, 3 * NHG, 8 * GR, E), F32),
            pltpu.VMEM((2, 3, NHG, GR // 2, 4 * E), U32),
            pltpu.VMEM((2, GS, T, D), F32),
            pltpu.VMEM((2, 2, GR, D // 2), F32),
            pltpu.VMEM((M + 8, D), F32),
            pltpu.VMEM((8, 512), I32),
            pltpu.VMEM((D, F), BF),
            pltpu.VMEM((D, F), BF),
            pltpu.VMEM((F, D), BF),
            pltpu.SemaphoreType.DMA((4 * NHG + 5,)),
        ],
        compiler_params=pltpu.CompilerParams(vmem_limit_bytes=120 * 2**20),
        name="rmt_mod",
    )(
        A_x.reshape(NG, GS, T, D), A_mem0.reshape(M, D),
        A_Wq.reshape(D, NHG, 8, E), A_Wk.reshape(D, NHG, 8, E), A_Wv.reshape(D, NHG, 8, E),
        A_Wo.reshape(NHG, 8, E, D),
        B_w_r, B_w_gate, B_w_up, B_w_down,
    )
    return out.reshape(B, S, D)
```

```python
import functools

import jax
import jax.numpy as jnp
from jax import lax
import jax.experimental.pallas as pl
import jax.experimental.pallas.tpu as pltpu

BF = jnp.bfloat16
F32 = jnp.float32
U32 = jnp.uint32
I32 = jnp.int32

GS = 4
PRE = 6

SEQ_FULL = (
    "L....L....L....AL...L....EL..q....EL..q....L.....EEL....L....L...q...p....L...q...p....L..q....L....L....p...L..q....p..N...q...N.oooNooqooopHooopooopoooNoopoooNooooNoooooo",
    "L....L....L....AL...L....EL..q....EL..q....EL....EL.....L....L...q...p....L...q...p....L..q....L....L....p...L..q....p...N..q...N.oooNooqooopHooopooopoooNoopoooNooooNoooooo",
    "L...L.....L....L...L....EL..q....EL..q....EAL.....L....L....q...L...p....L...q...p....L..q....L....L....p...EL..q....p...N..q...N.oooNooqooopHooopooopoooNoopoooNooooNoooooo",
    "L....L....L...AL..q...L....EL....p...L...EL....EL....L....L..q....L....EL..q....p....L..q...p....L..q.....p...N..q...q...p.....N..oopooqoooooHNooooNoooopooopooooNooooNoooo",
)
SEQ_LIGHT = (
    "N........N......N...q......A.....q.....E......p...p...q....E......q....p......q.....E.....q....p...p....E...q....N...opoooooHpooqoooooNooooNoooopooooooooooo",
    "N........N......N...q......A.....q.....E......p...p...q....E......q....p......q.....E.....q....p...p....E...q....N...opoooooHpooqoooooNooooNoooopooooooooooo",
    "N........N......N...q......A.....q.....E......p...p...q....E......q....p......q.....E.....q....p...p....E...q....N...opoooooHpooqoooooNooooNoooopooooooooooo",
    "N........N......N...q......A.....q.....E......p...p...q....E......q....p......q.....E.....q....p...p....E...q....N...opoooooHpooqoooooNooooNoooopooooooooooo",
)


def _rb(v):
    return v.astype(BF).astype(F32)


def _pack(v):
    return pltpu.bitcast(v.astype(BF), U32)


def _unpack(w):
    return pltpu.bitcast(w, BF)


def _layernorm(x):
    inv_n = 1.0 / x.shape[-1]
    m = jnp.sum(x, axis=-1, keepdims=True) * inv_n
    d = x - m
    v = _rb(jnp.sum(d * d, axis=-1, keepdims=True) * inv_n)
    den = _rb(jnp.sqrt(_rb(v + 1.0013580322265625e-05)))
    return _rb(_rb(x - _rb(m)) * (1.0 / den))


def _dot(a, b):
    return jnp.dot(a, b, preferred_element_type=F32)


def _strassen_rhs(b11, b12, b21, b22):
    return (b11, b21 - b11, b12 - b22, b22, b11 + b22, b11 + b12, b21 + b22)


def _strassen_lhs(a11, a12, a21, a22):
    return (a21 + a22, a22, a11, a11 + a12, a11 + a22, a21 - a11, a12 - a22)


def _strassen_out(k, p):
    if k == 1:
        return {(1, 0): p[0] + p[1]}
    if k == 3:
        return {(0, 1): p[2] + p[3]}
    if k == 5:
        return {(1, 1): (p[5] + p[4]) + (p[2] - p[0])}
    if k == 6:
        return {(0, 0): (p[6] + p[4]) + (p[1] - p[3])}
    return {}


def _pack_all(vals):
    out = []
    for k in range(0, len(vals), 2):
        w = _pack(jnp.concatenate(vals[k:k + 2], axis=1))
        out += [w[:, c:c + 128] for c in range(0, w.shape[1], 128)]
    return out


def _kernel(x_hbm, mem0_ref, wq_hbm, wk_hbm, wv_hbm, wo_hbm, wr_ref, wg_hbm, wu_hbm, wd_hbm,
            out_hbm,
            raw, wo_raw, ws, wn, wos, xbuf, xmid, hc, hn, tq, on, oc, to, state, bidx_ref,
            wg_s, wu_s, wd_s, sems,
            *, S, D, H, E, M, T):
    NG = S // (T * GS)
    L = M + T
    TH = T // 2
    DH = D // 2
    NP = H // 2
    NHG = H // 8
    NC = 3 * NHG
    GR = GS * TH
    R = PRE
    NO = 3
    w_hbm = (wq_hbm, wk_hbm, wv_hbm)

    def cp_w(j, hg):
        return pltpu.make_async_copy(w_hbm[j].at[:, hg], raw.at[j * NHG + hg], sems.at[j * NHG + hg])

    def cp_o(k):
        return pltpu.make_async_copy(wo_hbm.at[k], wo_raw.at[k], sems.at[NC + k])

    def cp_x(lo, hi, k):
        return pltpu.make_async_copy(x_hbm.at[pl.ds(lo, hi - lo)], xbuf.at[pl.ds(lo, hi - lo)], sems.at[NC + NHG + k])

    def cp_out(lo, hi, k):
        return pltpu.make_async_copy(xbuf.at[pl.ds(lo, hi - lo)], out_hbm.at[pl.ds(lo, hi - lo)], sems.at[NC + NHG + k])

    cp_b = [pltpu.make_async_copy(w, s, sems.at[NC + NHG + 2 + j])
            for j, (w, s) in enumerate(((wg_hbm, wg_s), (wu_hbm, wu_s), (wd_hbm, wd_s)))]

    def normed(x):
        x = x.astype(F32)
        d = x - jnp.sum(x, axis=-1, keepdims=True) * (1.0 / D)
        return d * lax.rsqrt(jnp.sum(d * d, axis=-1, keepdims=True) * (1.0 / D) + 1e-5)

    def chain_lhs(g, u, h):
        for m, v in enumerate(_strassen_lhs(h[:TH, :DH], h[:TH, DH:], h[TH:, :DH], h[TH:, DH:])[:4]):
            hc[g, u, m] = v

    def ahead_lhs(g, u, lo=0, hi=21):
        blocks = []
        for v in (u, u + GS // 2):
            l1 = hc[g, v, 2] + hc[g, v, 1]
            blocks.append((l1, hc[g, v, 0] - l1, hc[g, v, 3] - l1))
        ops = [w for x, y in zip(*blocks) for w in _strassen_lhs(x[:, :E], x[:, E:], y[:, :E], y[:, E:])]
        for q, w in enumerate(_pack_all(ops[lo:hi])):
            hn[lo + q, g, u] = w

    def prenorm(g, u):
        chain_lhs(g, u, normed(xbuf[g, u]))

    def t_rows(i, k, start=0, size=GR):
        return pl.ds((2 * i + k) * GR + start, size)

    def ahead_products(lhs, c, n, put):
        first = {}
        for m in (0, 2, 1):
            p = {}
            for k in range(7):
                p[k] = _dot(lhs(7 * m + k), _unpack(wn[c, n, 7 * m + k]))
                for (half, i), v in _strassen_out(k, p).items():
                    if m == 0:
                        first[half, i] = v
                    else:
                        put(half, 2 * n + i, int(m == 1), v + first[half, i])
                yield

    cp_x(0, PRE, 0).start()
    for c in range(NC):
        cp_w(c // NHG, c % NHG).start()
    for k in range(NHG):
        cp_o(k).start()
    cp_x(PRE, NG, 1).start()
    for c in cp_b:
        c.start()
    zero_bf = jnp.zeros((GS, T, D), BF)
    xbuf[NG] = zero_bf
    oc[...] = jnp.zeros(oc.shape, F32)
    on[1] = jnp.zeros(on.shape[1:], U32)
    to[...] = jnp.zeros(to.shape, F32)
    cp_x(0, PRE, 0).wait()

    norm = normed(xbuf[:PRE].reshape(PRE * GS * T, D))
    for n in range(PRE * GS):
        chain_lhs(n // GS, n % GS, norm[n * T:n * T + T])
    for n in range(PRE * GS // 2):
        ahead_lhs(n // 2, n % 2)

    def prep_qkv(c):
        spare = R + c % 2
        for r in range(0, E, 16):
            for k in range(4):
                words = pltpu.bitcast(raw[c, pl.ds(k * E + r, 16)].reshape(128, E), U32)
                tq[spare, r // 16, pl.ds(k * 64, 64)] = pltpu.bitcast(words, F32)
            for n in range(2):
                ops = {}
                for k in range(2):
                    for i in range(2):
                        w1, w2 = (pltpu.bitcast(tq[spare, r // 16, pl.ds(d * 64 + 2 * n + i, 16, stride=4), :], U32)
                                  for d in (k, k + 2))
                        ops[k, i] = _strassen_rhs(
                            pltpu.bitcast(w1 << 16, F32), pltpu.bitcast(w1 & jnp.uint32(0xFFFF0000), F32),
                            pltpu.bitcast(w2 << 16, F32), pltpu.bitcast(w2 & jnp.uint32(0xFFFF0000), F32))
                        for m, w in enumerate(_pack_all(ops[k, i][:4])):
                            ws[c, 2 * n + i, m, pl.ds((k * E + r) // 2, 8)] = w
                    if k == 0:
                        yield
                ops = [w for m in (4, 5, 6) for w in _strassen_rhs(ops[0, 0][m], ops[0, 1][m], ops[1, 0][m], ops[1, 1][m])]
                for q, w in enumerate(_pack_all(ops)):
                    wn[c, n, q, pl.ds(r // 2, 8)] = w
                yield

    def prep_o(k, part, spare=None):
        i, r = divmod(part * 16, E)
        for col in range(0, DH, E):
            w = [pltpu.bitcast(wo_raw[k, 2 * i + a, pl.ds(r, 16), pl.ds(b * DH + col, E)], U32)
                 for a in range(2) for b in range(2)]
            if spare is not None:
                tq[spare, k, pl.ds(part * 16 + col // E * 8, 8)] = pltpu.bitcast(w[0], F32)
                w[0] = pltpu.bitcast(tq[spare, k, pl.ds(part * 16 + col // E * 8, 8)], U32)
            ops = [_pack(v) for v in _strassen_rhs(*(_unpack(v).astype(F32) for v in w))]
            ops[0], ops[3] = w[0], w[3]
            for m, v in enumerate(ops):
                wos[m, k, pl.ds(part * 8, 8), pl.ds(col, E)] = v

    def ahead_qkv(c, ng, others):
        for m in (0, 2, 1):
            dst = int(m != 2)
            for ks in (range(4), range(4, 7)):
                for n in range(2):
                    prods = {k: _dot(_unpack(hn[7 * m + k, :ng].reshape(ng * GR // 4, E)),
                                     _unpack(wn[c, n, 7 * m + k])) for k in ks}
                    for g in range(ng):
                        if g * 3 // ng != (g - 1) * 3 // ng:
                            next(others, None)
                        p = {k: v[g * GR // 2:(g + 1) * GR // 2] for k, v in prods.items()}
                        if 0 in p:
                            upd = {(1, 0): p[0] + p[1], (0, 1): p[2] + p[3], (1, 1): p[2] - p[0], (0, 0): p[1] - p[3]}
                        else:
                            upd = {(1, 1): p[5] + p[4], (0, 0): p[6] + p[4]}
                        for (half, i), v in upd.items():
                            def rows(k):
                                return t_rows(2 * n + i, k, half * GR // 2, GR // 2)
                            if m or 4 in p:
                                v = v + tq[g, c, rows(dst if 4 in p else 1)]
                            tq[g, c, rows(dst)] = v
        assert next(others, None) is None

    cp_w(0, 0).wait()
    for _ in prep_qkv(0):
        pass

    def stream(c, carry):
        @pl.when(c < NC - 1)
        def _():
            pltpu.make_async_copy(raw.at[c + 1], raw.at[c + 1], sems.at[c + 1]).wait()

        @pl.when(c < NC // 2)
        def _():
            ahead_qkv(c, PRE - 2, prep_qkv(c + 1))

        @pl.when(jnp.logical_and(c >= NC // 2, c < NC - 1))
        def _():
            ahead_qkv(c, PRE, prep_qkv(c + 1))

        @pl.when(c == NC - 1)
        def _():
            for k in range(NO):
                cp_o(k).wait()
            ahead_qkv(c, PRE, ([prep_o(k, part, R + c % 2) for k in range(NO)] for part in range(32)))
        return carry
    lax.fori_loop(0, NC, stream, 0)
    for k in range(NO, NHG):
        cp_o(k).wait()
        for part in range(32):
            prep_o(k, part)

    def reset_state():
        state[:M] = mem0_ref[...].astype(F32)
        state[M:] = jnp.full((8, D), -jnp.inf, F32)
        bidx_ref[:, :128] = jnp.full((8, 128), S, I32)
    reset_state()

    def router(xn):
        return _rb(jnp.sum(xn * wr_ref[...].astype(F32).reshape(1, D), axis=-1, keepdims=True))

    def epilogue(g, u, t, par, best, bidx):
        rows = pl.ds(t * 8, 8)
        half = t * 8 // TH
        c = oc[par, u, rows]
        n = to[par, half, pl.ds(u * TH + t * 8 % TH, 8)]
        c = jnp.concatenate([c[:, :DH] + n, c[:, DH:]] if half == 0 else [c[:, :DH], c[:, DH:] + n], axis=1)
        x1 = _rb(xbuf[g, u, rows].astype(F32) + _rb(c))
        xn = _layernorm(x1)
        xmid[0, g, u, rows] = x1
        xmid[1, g, u, rows] = xn
        xbuf[g, u, rows] = (x1 + xn).astype(BF)
        it = lax.broadcasted_iota(I32, (8, 128), 0) + ((g * GS + u) * T + t * 8)
        r = jnp.where(it < S, jnp.broadcast_to(router(xn), (8, 128)), -jnp.inf)
        better = r > best
        return jnp.where(better, r, best), jnp.where(better, it, bidx)

    def qkv_group_rounds(G, par):
        g, slot = G % NG, G % R

        def tiles():
            for c in range(NC // 2):
                c = par * (NC // 2) + c

                def put(half, i, k, v):
                    for d in range(2):
                        tq[slot + d, c, t_rows(i, k, half * GR // 2, GR // 2)] = v[d * GR // 2:(d + 1) * GR // 2]
                for n in range(2):
                    yield from ahead_products(lambda q: _unpack(hn[q, pl.ds(g, 2)].reshape(GR // 2, E)), c, n, put)
        it = tiles()
        return [lambda: [next(it) for _ in range(4)]] * (NC * 21 // 4)

    def out_group_rounds(par, st):
        def rnd(c, m, k):
            cols = pl.ds(c * 128, 128)
            d = _dot(_unpack(on[par, m, k]), _unpack(wos[4 + m, k, :, cols]))
            st["n", m] = d if k == 0 else d + st["n", m]
            if k == NHG - 1 and m == 1:
                to[par, 1, :, cols] = st["n", 0] + st["n", 1]
            if k == NHG - 1 and m == 2:
                to[par, 0, :, cols] = st["n", 0] + st["n", 2]
        return [functools.partial(rnd, c, m, k) for c in range(DH // 128) for m in range(3) for k in range(NHG)]

    def segment(G, par, u, mem, seq, longs, norms):
        g = G % NG
        st = {}
        row = lax.broadcasted_iota(I32, (L, L), 0)
        col = lax.broadcasted_iota(I32, (L, L), 1)
        mask = (row < M) | (row >= col)
        a1, a2 = mem[:, :DH], mem[:, DH:]
        a12 = a1 + a2
        lhs = [jnp.concatenate([hc[g, u, m], a], axis=0) for m, a in enumerate((a12, a2, a1, a12))]

        def qkv(*prods):
            for p, j, m in prods:
                unit = (j * NHG + p // 4, p % 4)
                st[p, j, m] = _dot(lhs[m], _unpack(ws[unit + (m,)]))
                if m == 3:
                    m2, m4, m3, m5 = (st.pop((p, j, k)) for k in range(4))
                    ca, cb = m2 + m4, m3 + m5
                    c11 = tq[G % R, unit[0], t_rows(unit[1], 0, u * TH, TH)] + (m4[:TH] - m5[:TH])
                    c22 = tq[G % R, unit[0], t_rows(unit[1], 1, u * TH, TH)] + (m3[:TH] - m2[:TH])
                    ha = jnp.concatenate([ca[TH:], c11, ca[:TH]], axis=0)
                    hb = jnp.concatenate([cb[TH:], cb[:TH], c22], axis=0)
                    st[j, 2 * p] = ha if j == 0 else ha.astype(BF)
                    st[j, 2 * p + 1] = hb if j == 0 else hb.astype(BF)

        def scores(n):
            for a in range(4 * n, 4 * n + 4):
                sc = lax.dot_general(st.pop((0, a)), st.pop((1, a)), (((1,), (1,)), ((), ())),
                                     preferred_element_type=F32)
                sc = jnp.where(mask, sc, -1e9 * E ** 0.5)
                e = jnp.exp2((sc - jnp.max(sc, axis=-1, keepdims=True)) * (E ** -0.5 * 1.4426950408889634))
                st["p", a] = e * pltpu.reciprocal(jnp.sum(e, axis=-1, keepdims=True), full_range=False)

        def values(n):
            for a in range(4 * n, 4 * n + 4):
                st["o", a] = _dot(st.pop(("p", a)), st.pop((2, a)))

        def oproj(p, half):
            oa, ob = st["o", 2 * p], st["o", 2 * p + 1]
            k, blk = p // 4, pl.ds((p % 4) * (E // 2), E // 2)
            if half == 0:
                st["ab", p] = oa + ob
                left = [jnp.concatenate([v[:M], v[M + TH:]], axis=0) for v in (st["ab", p], ob)]
            else:
                left = [oa[:M + TH], st["ab", p][:M + TH]]
                a11, a12_, a21, a22 = oa[M:M + TH], ob[M:M + TH], oa[M + TH:], ob[M + TH:]
                for m, v in enumerate((a11 + a22, a21 - a11, a12_ - a22)):
                    on[par, m, k, pl.ds(u * (TH // 2), TH // 2), pl.ds((p % 4) * E, E)] = _pack(v)
            for m, v in zip((2 * half, 2 * half + 1), left):
                d = _dot(v, _unpack(wos[m, k, blk]))
                st["acc", m] = d if p == 0 else d + st["acc", m]

        units = [(p, j) for n in range(H // 4) for j in range(3) for p in (2 * n, 2 * n + 1)]
        prods = [un + (2,) for un in units[:4]] + [un + (m,) for un in units[:4] for m in (0, 1, 3)]
        prods += [un + (m,) for un in units[4:] for m in range(4)]
        chain = [functools.partial(qkv, *prods[k:k + 2]) for k in range(0, len(prods), 2)]
        outs = [(p, half) for p in range(NP - 4) for half in (0, 1)]
        outs += [(p, half) for half in (0, 1) for p in range(NP - 4, NP)]
        its = {".": iter(chain), "o": iter([functools.partial(oproj, *a) for a in outs]),
               "L": longs[0], "N": longs[1], "E": iter(norms[2:]), "H": iter(norms[:1]), "A": iter(norms[1:2]),
               "q": iter([functools.partial(scores, n) for n in range(H // 4)]),
               "p": iter([functools.partial(values, n) for n in range(H // 4)])}
        for ch in seq:
            next(its[ch])()
        assert all(next(its[ch], None) is None for ch in ".oqpEHA")
        m2, m4, m3, m5 = (st["acc", m] for m in range(4))
        ca, cb = m2 + m4, m3 + m5
        oc[par, u, :TH, :DH] = m4[M:] - m5[M:]
        oc[par, u, :TH, DH:] = cb[M:]
        oc[par, u, TH:, :DH] = ca[M:]
        oc[par, u, TH:, DH:] = m3[M:] - m2[M:]
        return _rb(jnp.concatenate([ca[:M], cb[:M]], axis=1))

    def group(G, seqs):
        mem, top = state[:M], [state[M:, :128], bidx_ref[:, :128]]
        full = "L" in seqs[0]
        g, par = G % NG, G % 2
        longs = [iter(qkv_group_rounds(G + 2 - par, par) if full else []),
                 iter(out_group_rounds(1 - par, {}))]

        def post(u, t):
            top[:] = epilogue(jnp.where(g >= 2, g - 2, NG), u, t, par, *top)
            if full:
                hn[0, NG + par, 0] = pltpu.bitcast(top[0], U32)
            else:
                tq[R + par, 0, :8] = top[0]
        for u in range(GS):
            mem = segment(G, par, u, mem, seqs[u], longs,
                          [functools.partial(prenorm, (G + 5) % NG, u),
                           functools.partial(ahead_lhs, (G + 4) % NG, u // 2, 10 * (u % 2), 10 + 11 * (u % 2))]
                          + [functools.partial(post, u, t) for t in range(T // 8)])
        assert all(next(it, None) is None for it in longs)
        state[:M] = mem
        state[M:, :128], bidx_ref[:, :128] = top

    def finish_layer(last):
        best, bidx = state[M:, :128], bidx_ref[:, :128]
        for par in range(2):
            if par:
                for f in out_group_rounds(par, {}):
                    f()
            for u in range(GS):
                for t in range(T // 8):
                    best, bidx = epilogue(NG - 2 + par, u, t, par, best, bidx)

        @pl.when(last)
        def _():
            cp_out(NG - 3, NG, 1).start()

        top = jnp.max(best, axis=0, keepdims=True)
        idx = jnp.min(jnp.where(best == top, bidx, S))
        idx = jnp.where(idx >= S, 0, idx)
        g, u = idx // (T * GS), idx // T % GS
        rows = pl.ds(pl.multiple_of(idx % T // 8 * 8, 8), 8)
        x1, xn = xmid[0, g, u, rows], xmid[1, g, u, rows]
        gate = _rb(_dot(xn, wg_s[...]))
        up = _rb(_dot(xn, wu_s[...]))
        gate = _rb(gate * _rb(jax.nn.sigmoid(gate)))
        y = _rb(_dot(_rb(gate * up), wd_s[...]))
        y = _rb(y * _rb(jax.nn.sigmoid(router(xn))))
        sel = lax.broadcasted_iota(I32, (8, D), 0) == idx % 8
        x2 = (x1 + _rb(xn + jnp.where(sel, y, 0.0))).astype(BF)

        @pl.when(last)
        def _():
            cp_out(0, NG - 3, 0).wait()
            cp_out(NG - 3, NG, 1).wait()
            xbuf[g, u, rows] = x2
            cp = pltpu.make_async_copy(xbuf.at[g, u], out_hbm.at[g, u], sems.at[0])
            cp.start()
            cp.wait()

        @pl.when(jnp.logical_not(last))
        def _():
            xbuf[g, u, rows] = x2
            prenorm(g, u)
            ahead_lhs(g, u % (GS // 2))
            reset_state()

            @pl.when(g < 2)
            def _():
                def redo(c, carry):
                    def put(half, i, k, v):
                        start = pl.multiple_of(half * GR // 2 + u % (GS // 2) * TH, TH)
                        tq[NG % R + g, c, t_rows(i, k, start, TH)] = v
                    for n in range(2):
                        for _ in ahead_products(lambda q: _unpack(hn[q, g, u % (GS // 2)]), c, n, put):
                            pass
                    return carry
                lax.fori_loop(0, NC, redo, 0)

    def iteration(G, carry):
        last = G == 2 * NG - 1

        @pl.when(G == PRE - 5)
        def _():
            cp_x(PRE, NG, 1).wait()
            for c in cp_b:
                c.wait()

        @pl.when(last)
        def _():
            cp_out(0, NG - 3, 0).start()

        light = (G < PRE - 4) | (G == PRE - 3) | (G >= 2 * NG - 2)
        pl.when(light)(lambda: group(G, SEQ_LIGHT))
        pl.when(jnp.logical_not(light))(lambda: group(G, SEQ_FULL))
        pl.when(G % NG == NG - 1)(lambda: finish_layer(last))
        return carry

    lax.fori_loop(0, 2 * NG, iteration, 0)


@functools.partial(jax.jit, static_argnames=("A_seg_len",))
def pallas_interleave_layers__memory_aug_recurrent_mem_tr__moe_arch_mod__prompt_kernel(
    A_x, A_mem0, A_Wq, A_Wk, A_Wv, A_Wo, A_seg_len, B_x, B_w_r, B_w_gate, B_w_up, B_w_down,
):
    del B_x
    B, S, D = A_x.shape
    _, H, E = A_Wq.shape
    M = A_mem0.shape[1]
    F = B_w_gate.shape[1]
    T = int(A_seg_len)
    assert (B, S, D, H, E, M, T) == (1, 2048, 512, 32, 128, 8, 32)
    NG = S // (T * GS)
    NHG = H // 8
    GR = GS * T // 2
    hbm = pl.BlockSpec(memory_space=pl.ANY)
    vmem = pl.BlockSpec(memory_space=pltpu.VMEM)
    out = pl.pallas_call(
        functools.partial(_kernel, S=S, D=D, H=H, E=E, M=M, T=T),
        out_shape=jax.ShapeDtypeStruct((NG, GS, T, D), A_x.dtype),
        in_specs=[hbm, vmem, hbm, hbm, hbm, hbm, vmem, hbm, hbm, hbm],
        out_specs=hbm,
        scratch_shapes=[
            pltpu.VMEM((3 * NHG, D, 8, E), BF),
            pltpu.VMEM((NHG, 8, E, D), BF),
            pltpu.VMEM((3 * NHG, 4, 4, D // 4, E), U32),
            pltpu.VMEM((3 * NHG, 2, 21, E // 2, E), U32),
            pltpu.VMEM((7, NHG, 2 * E, D // 2), U32),
            pltpu.VMEM((NG + 1, GS, T, D), BF),
            pltpu.VMEM((2, NG + 1, GS, T, D), F32),
            pltpu.VMEM((NG, GS, 4, T // 2, D // 2), F32),
            pltpu.VMEM((21, NG + 2, GS // 2, T // 4, E), U32),
            pltpu.VMEM((PRE + 2, 3 * NHG, 8 * GR, E), F32),
            pltpu.VMEM((2, 3, NHG, GR // 2, 4 * E), U32),
            pltpu.VMEM((2, GS, T, D), F32),
            pltpu.VMEM((2, 2, GR, D // 2), F32),
            pltpu.VMEM((M + 8, D), F32),
            pltpu.VMEM((8, 512), I32),
            pltpu.VMEM((D, F), BF),
            pltpu.VMEM((D, F), BF),
            pltpu.VMEM((F, D), BF),
            pltpu.SemaphoreType.DMA((4 * NHG + 5,)),
        ],
        compiler_params=pltpu.CompilerParams(vmem_limit_bytes=120 * 2**20),
        name="rmt_mod",
    )(
        A_x.reshape(NG, GS, T, D), A_mem0.reshape(M, D),
        A_Wq.reshape(D, NHG, 8, E), A_Wk.reshape(D, NHG, 8, E), A_Wv.reshape(D, NHG, 8, E),
        A_Wo.reshape(NHG, 8, E, D),
        B_w_r, B_w_gate, B_w_up, B_w_down,
    )
    return out.reshape(B, S, D)
```

```python
import functools

import jax
import jax.numpy as jnp
from jax import lax
import jax.experimental.pallas as pl
import jax.experimental.pallas.tpu as pltpu

BF = jnp.bfloat16
F32 = jnp.float32
U32 = jnp.uint32
I32 = jnp.int32

GS = 4
PRE = 4

SEQ_FULL = (
    "L.....L....AL....L..q....L....L....EL....EL..q...p.....EL..q....L.....p.q....HL....p.q....L....L....p...L.....L..L...q...N....p..qoqooooENoooopooopoooNoooopoooNooooNoooNooo",
    "L.....L....AL....L..q...L.....L....EL....EL..q....p....EL..q....L.....p.q....L....p.q....L....L....p...L....L....L..q...N....p..qooqoooENoooopoooNooopoooopoooHNooooNoooNooo",
    "L.....L....AL....L..q....HL....L....EL....EL..q....p....EL..q....L.....p.q....L....p.q....L.....L...p...L....L...L...q...N....p..qooqoooENoooopoooNooopoooopoooNooooNoooNooo",
    "L....L....L....L...L.....EL..q....EL...EL....L..q....L..q....p....L....L....p....L....L....L....N..q.....p.q....EN....p..q..q...opoqooooopoooNoooopoooHNoooopoooANooooNoooo",
)
SEQ_LIGHT = (
    "N........N......N...q......A.....q.....E......p...p...q....E......q....p......q.....E.....q....p...p....E...q....N...opoooooHpooqoooooNooooNoooopooooooooooo",
    "N........N......N...q......A.....q.....E......p...p...q....E......q....p......q.....E.....q....p...p....E...q....N...opoooooHpooqoooooNooooNoooopooooooooooo",
    "N........N......N...q......A.....q.....E......p...p...q....E......q....p......q.....E.....q....p...p....E...q....N...opoooooHpooqoooooNooooNoooopooooooooooo",
    "N........N......N...q......A.....q.....E......p...p...q....E......q....p......q.....E.....q....p...p....E...q....N...opoooooHpooqoooooNooooNoooopooooooooooo",
)


def _rb(v):
    return v.astype(BF).astype(F32)


def _pack(v):
    return pltpu.bitcast(v.astype(BF), U32)


def _unpack(w):
    return pltpu.bitcast(w, BF)


def _layernorm(x):
    inv_n = 1.0 / x.shape[-1]
    m = jnp.sum(x, axis=-1, keepdims=True) * inv_n
    d = x - m
    v = _rb(jnp.sum(d * d, axis=-1, keepdims=True) * inv_n)
    den = _rb(jnp.sqrt(_rb(v + 1.0013580322265625e-05)))
    return _rb(_rb(x - _rb(m)) * (1.0 / den))


def _dot(a, b):
    return jnp.dot(a, b, preferred_element_type=F32)


def _strassen_rhs(b11, b12, b21, b22):
    return (b11, b21 - b11, b12 - b22, b22, b11 + b22, b11 + b12, b21 + b22)


def _strassen_lhs(a11, a12, a21, a22):
    return (a21 + a22, a22, a11, a11 + a12, a11 + a22, a21 - a11, a12 - a22)


def _strassen_out(k, p):
    if k == 1:
        return {(1, 0): p[0] + p[1]}
    if k == 3:
        return {(0, 1): p[2] + p[3]}
    if k == 5:
        return {(1, 1): (p[5] + p[4]) + (p[2] - p[0])}
    if k == 6:
        return {(0, 0): (p[6] + p[4]) + (p[1] - p[3])}
    return {}


def _pack_all(vals):
    out = []
    for k in range(0, len(vals), 2):
        w = _pack(jnp.concatenate(vals[k:k + 2], axis=1))
        out += [w[:, c:c + 128] for c in range(0, w.shape[1], 128)]
    return out


def _kernel(x_hbm, mem0_ref, wq_hbm, wk_hbm, wv_hbm, wo_hbm, wr_ref, wg_hbm, wu_hbm, wd_hbm,
            out_hbm,
            raw, wo_raw, ws, wn, wos, xbuf, xmid, hc, hn, tq, on, oc, to, state, bidx_ref,
            wg_s, wu_s, wd_s, sems,
            *, S, D, H, E, M, T):
    NG = S // (T * GS)
    L = M + T
    TH = T // 2
    DH = D // 2
    NP = H // 2
    NHG = H // 8
    NC = 3 * NHG
    GR = GS * TH
    R = PRE
    XG = 6
    NO = 2
    w_hbm = (wq_hbm, wk_hbm, wv_hbm)

    def cp_w(j, hg):
        return pltpu.make_async_copy(w_hbm[j].at[:, hg], raw.at[j * NHG + hg], sems.at[j * NHG + hg])

    def cp_o(k):
        return pltpu.make_async_copy(wo_hbm.at[k], wo_raw.at[k], sems.at[NC + k])

    def cp_x(lo, hi, k):
        return pltpu.make_async_copy(x_hbm.at[pl.ds(lo, hi - lo)], xbuf.at[pl.ds(lo, hi - lo)], sems.at[NC + NHG + k])

    def cp_out(lo, hi, k):
        return pltpu.make_async_copy(xbuf.at[pl.ds(lo, hi - lo)], out_hbm.at[pl.ds(lo, hi - lo)], sems.at[NC + NHG + k])

    cp_b = [pltpu.make_async_copy(w, s, sems.at[NC + NHG + 2 + j])
            for j, (w, s) in enumerate(((wg_hbm, wg_s), (wu_hbm, wu_s), (wd_hbm, wd_s)))]

    def normed(x):
        x = x.astype(F32)
        d = x - jnp.sum(x, axis=-1, keepdims=True) * (1.0 / D)
        return d * lax.rsqrt(jnp.sum(d * d, axis=-1, keepdims=True) * (1.0 / D) + 1e-5)

    def chain_lhs(g, u, h):
        for m, v in enumerate(_strassen_lhs(h[:TH, :DH], h[:TH, DH:], h[TH:, :DH], h[TH:, DH:])[:4]):
            hc[g, u, m] = v

    def ahead_lhs(g, u, lo=0, hi=21):
        blocks = []
        for v in (u, u + GS // 2):
            l1 = hc[g, v, 2] + hc[g, v, 1]
            blocks.append((l1, hc[g, v, 0] - l1, hc[g, v, 3] - l1))
        ops = [w for x, y in zip(*blocks) for w in _strassen_lhs(x[:, :E], x[:, E:], y[:, :E], y[:, E:])]
        for q, w in enumerate(_pack_all(ops[lo:hi])):
            hn[lo + q, g, u] = w

    def prenorm(g, u):
        chain_lhs(g, u, normed(xbuf[g, u]))

    def t_rows(i, k, start=0, size=GR):
        return pl.ds((2 * i + k) * GR + start, size)

    def ahead_products(lhs, c, n, put):
        first = {}
        for m in (0, 2, 1):
            p = {}
            for k in range(7):
                p[k] = _dot(lhs(7 * m + k), _unpack(wn[c, n, 7 * m + k]))
                for (half, i), v in _strassen_out(k, p).items():
                    if m == 0:
                        first[half, i] = v
                    else:
                        put(half, 2 * n + i, int(m == 1), v + first[half, i])
                yield

    cp_x(0, XG, 0).start()
    for c in range(NC):
        cp_w(c // NHG, c % NHG).start()
    for k in range(NHG):
        cp_o(k).start()
    cp_x(XG, NG, 1).start()
    for c in cp_b:
        c.start()
    zero_bf = jnp.zeros((GS, T, D), BF)
    xbuf[NG] = zero_bf
    oc[...] = jnp.zeros(oc.shape, F32)
    on[1] = jnp.zeros(on.shape[1:], U32)
    to[...] = jnp.zeros(to.shape, F32)
    cp_x(0, XG, 0).wait()

    norm = normed(xbuf[:XG - 1].reshape((XG - 1) * GS * T, D))
    for n in range((XG - 1) * GS):
        chain_lhs(n // GS, n % GS, norm[n * T:n * T + T])
    for n in range(PRE * GS // 2):
        ahead_lhs(n // 2, n % 2)

    def prep_qkv(c):
        spare = R + c % 2
        for r in range(0, E, 16):
            for k in range(4):
                words = pltpu.bitcast(raw[c, pl.ds(k * E + r, 16)].reshape(128, E), U32)
                tq[spare, r // 16, pl.ds(k * 64, 64)] = pltpu.bitcast(words, F32)
            for n in range(2):
                ops = {}
                for k in range(2):
                    for i in range(2):
                        w1, w2 = (pltpu.bitcast(tq[spare, r // 16, pl.ds(d * 64 + 2 * n + i, 16, stride=4), :], U32)
                                  for d in (k, k + 2))
                        ops[k, i] = _strassen_rhs(
                            pltpu.bitcast(w1 << 16, F32), pltpu.bitcast(w1 & jnp.uint32(0xFFFF0000), F32),
                            pltpu.bitcast(w2 << 16, F32), pltpu.bitcast(w2 & jnp.uint32(0xFFFF0000), F32))
                        for m, w in enumerate(_pack_all(ops[k, i][:4])):
                            ws[c, 2 * n + i, m, pl.ds((k * E + r) // 2, 8)] = w
                    if k == 0:
                        yield
                ops = [w for m in (4, 5, 6) for w in _strassen_rhs(ops[0, 0][m], ops[0, 1][m], ops[1, 0][m], ops[1, 1][m])]
                for q, w in enumerate(_pack_all(ops)):
                    wn[c, n, q, pl.ds(r // 2, 8)] = w
                yield

    def prep_o(k, part, spare=None):
        i, r = divmod(part * 16, E)
        for col in range(0, DH, E):
            w = [pltpu.bitcast(wo_raw[k, 2 * i + a, pl.ds(r, 16), pl.ds(b * DH + col, E)], U32)
                 for a in range(2) for b in range(2)]
            if spare is not None:
                tq[spare, k, pl.ds(part * 16 + col // E * 8, 8)] = pltpu.bitcast(w[0], F32)
                w[0] = pltpu.bitcast(tq[spare, k, pl.ds(part * 16 + col // E * 8, 8)], U32)
            ops = [_pack(v) for v in _strassen_rhs(*(_unpack(v).astype(F32) for v in w))]
            ops[0], ops[3] = w[0], w[3]
            for m, v in enumerate(ops):
                wos[m, k, pl.ds(part * 8, 8), pl.ds(col, E)] = v

    def ahead_qkv(c, ng, others, count):
        point = 0
        for m in (0, 2, 1):
            dst = int(m != 2)
            for ks in (range(4), range(4, 7)):
                for n in range(2):
                    prods = {k: _dot(_unpack(hn[7 * m + k, :ng].reshape(ng * GR // 4, E)),
                                     _unpack(wn[c, n, 7 * m + k])) for k in ks}
                    for g in range(ng):
                        point += 1
                        for _ in range(*(-(-q * count // (11 * ng)) for q in (point - 1, point))):
                            next(others, None)
                        p = {k: v[g * GR // 2:(g + 1) * GR // 2] for k, v in prods.items()}
                        if 0 in p:
                            upd = {(1, 0): p[0] + p[1], (0, 1): p[2] + p[3], (1, 1): p[2] - p[0], (0, 0): p[1] - p[3]}
                        else:
                            upd = {(1, 1): p[5] + p[4], (0, 0): p[6] + p[4]}
                        for (half, i), v in upd.items():
                            def rows(k):
                                return t_rows(2 * n + i, k, half * GR // 2, GR // 2)
                            if m or 4 in p:
                                v = v + tq[g, c, rows(dst if 4 in p else 1)]
                            tq[g, c, rows(dst)] = v
        assert not list(others)

    cp_w(0, 0).wait()
    for _ in prep_qkv(0):
        pass

    def stream(c, carry):
        @pl.when(c < NC - 1)
        def _():
            pltpu.make_async_copy(raw.at[c + 1], raw.at[c + 1], sems.at[c + 1]).wait()
            ahead_qkv(c, PRE, prep_qkv(c + 1), 32)

        @pl.when(c == NC - 1)
        def _():
            for k in range(NO):
                cp_o(k).wait()
            ahead_qkv(c, PRE, (prep_o(k, part, R + c % 2) for k in range(NO) for part in range(32)), 32 * NO)
        return carry
    lax.fori_loop(0, NC, stream, 0)
    for k in range(NO, NHG):
        cp_o(k).wait()
        for part in range(32):
            prep_o(k, part)

    def reset_state():
        state[:M] = mem0_ref[...].astype(F32)
        state[M:] = jnp.full((8, D), -jnp.inf, F32)
        bidx_ref[:, :128] = jnp.full((8, 128), S, I32)
    reset_state()

    def router(xn):
        return _rb(jnp.sum(xn * wr_ref[...].astype(F32).reshape(1, D), axis=-1, keepdims=True))

    def epilogue(g, u, t, par, best, bidx):
        rows = pl.ds(t * 8, 8)
        half = t * 8 // TH
        c = oc[par, u, rows]
        n = to[par, half, pl.ds(u * TH + t * 8 % TH, 8)]
        c = jnp.concatenate([c[:, :DH] + n, c[:, DH:]] if half == 0 else [c[:, :DH], c[:, DH:] + n], axis=1)
        x1 = _rb(xbuf[g, u, rows].astype(F32) + _rb(c))
        xn = _layernorm(x1)
        xmid[0, g, u, rows] = x1
        xmid[1, g, u, rows] = xn
        xbuf[g, u, rows] = (x1 + xn).astype(BF)
        it = lax.broadcasted_iota(I32, (8, 128), 0) + ((g * GS + u) * T + t * 8)
        r = jnp.where(it < S, jnp.broadcast_to(router(xn), (8, 128)), -jnp.inf)
        better = (r > best) | ((r == best) & (it < bidx))
        return jnp.where(better, r, best), jnp.where(better, it, bidx)

    def qkv_group_rounds(G, par):
        g, slot = G % NG, G % R

        def tiles():
            for c in range(NC // 2):
                c = par * (NC // 2) + c

                def put(half, i, k, v):
                    for d in range(2):
                        tq[slot + d, c, t_rows(i, k, half * GR // 2, GR // 2)] = v[d * GR // 2:(d + 1) * GR // 2]
                for n in range(2):
                    yield from ahead_products(lambda q: _unpack(hn[q, pl.ds(g, 2)].reshape(GR // 2, E)), c, n, put)
        it = tiles()
        return [lambda: [next(it) for _ in range(4)]] * (NC * 21 // 4)

    def out_group_rounds(par, st):
        def rnd(c, m, k):
            cols = pl.ds(c * 128, 128)
            d = _dot(_unpack(on[par, m, k]), _unpack(wos[4 + m, k, :, cols]))
            st[c, m] = d if k == 0 else d + st[c, m]
            if k == NHG - 1 and m == 1:
                to[par, 1, :, cols] = st[c, 0] + st[c, 1]
            if k == NHG - 1 and m == 2:
                to[par, 0, :, cols] = st[c, 0] + st[c, 2]
        return [functools.partial(rnd, c, m, k)
                for c, m in ((0, 0), (0, 1), (1, 0), (1, 1), (1, 2), (0, 2)) for k in range(NHG)]

    def segment(G, par, u, mem, seq, longs, norms):
        g = G % NG
        st = {}
        row = lax.broadcasted_iota(I32, (L, L), 0)
        col = lax.broadcasted_iota(I32, (L, L), 1)
        mask = (row < M) | (row >= col)
        a1, a2 = mem[:, :DH], mem[:, DH:]
        a12 = a1 + a2
        lhs = [jnp.concatenate([hc[g, u, m], a], axis=0) for m, a in enumerate((a12, a2, a1, a12))]

        def qkv(*prods):
            for p, j, m in prods:
                unit = (j * NHG + p // 4, p % 4)
                st[p, j, m] = _dot(lhs[m], _unpack(ws[unit + (m,)]))
                if m == 3:
                    m2, m4, m3, m5 = (st.pop((p, j, k)) for k in range(4))
                    ca, cb = m2 + m4, m3 + m5
                    c11 = tq[G % R, unit[0], t_rows(unit[1], 0, u * TH, TH)] + (m4[:TH] - m5[:TH])
                    c22 = tq[G % R, unit[0], t_rows(unit[1], 1, u * TH, TH)] + (m3[:TH] - m2[:TH])
                    ha = jnp.concatenate([ca[TH:], c11, ca[:TH]], axis=0)
                    hb = jnp.concatenate([cb[TH:], cb[:TH], c22], axis=0)
                    st[j, 2 * p] = ha if j == 0 else ha.astype(BF)
                    st[j, 2 * p + 1] = hb if j == 0 else hb.astype(BF)

        def scores(n):
            for a in range(4 * n, 4 * n + 4):
                sc = lax.dot_general(st.pop((0, a)), st.pop((1, a)), (((1,), (1,)), ((), ())),
                                     preferred_element_type=F32)
                sc = jnp.where(mask, sc, -1e9 * E ** 0.5)
                e = jnp.exp2((sc - jnp.max(sc, axis=-1, keepdims=True)) * (E ** -0.5 * 1.4426950408889634))
                st["p", a] = e * pltpu.reciprocal(jnp.sum(e, axis=-1, keepdims=True), full_range=False)

        def values(n):
            for a in range(4 * n, 4 * n + 4):
                st["o", a] = _dot(st.pop(("p", a)), st.pop((2, a)))

        def oproj(p, half):
            oa, ob = st["o", 2 * p], st["o", 2 * p + 1]
            k, blk = p // 4, pl.ds((p % 4) * (E // 2), E // 2)
            if half == 0:
                st["ab", p] = oa + ob
                left = [jnp.concatenate([v[:M], v[M + TH:]], axis=0) for v in (st["ab", p], ob)]
            else:
                left = [oa[:M + TH], st["ab", p][:M + TH]]
                a11, a12_, a21, a22 = oa[M:M + TH], ob[M:M + TH], oa[M + TH:], ob[M + TH:]
                for m, v in enumerate((a11 + a22, a21 - a11, a12_ - a22)):
                    on[par, m, k, pl.ds(u * (TH // 2), TH // 2), pl.ds((p % 4) * E, E)] = _pack(v)
            for m, v in zip((2 * half, 2 * half + 1), left):
                d = _dot(v, _unpack(wos[m, k, blk]))
                st["acc", m] = d if p == 0 else d + st["acc", m]

        units = [(p, j) for n in range(H // 4) for j in range(3) for p in (2 * n, 2 * n + 1)]
        prods = [un + (2,) for un in units[:4]] + [un + (m,) for un in units[:4] for m in (0, 1, 3)]
        prods += [un + (m,) for un in units[4:] for m in range(4)]
        chain = [functools.partial(qkv, *prods[k:k + 2]) for k in range(0, len(prods), 2)]
        outs = [(p, half) for p in range(NP - 2) for half in (0, 1)]
        outs += [(p, half) for half in (0, 1) for p in range(NP - 2, NP)]
        its = {".": iter(chain), "o": iter([functools.partial(oproj, *a) for a in outs]),
               "L": longs[0], "N": longs[1], "E": iter(norms[2:]), "H": iter(norms[:1]), "A": iter(norms[1:2]),
               "q": iter([functools.partial(scores, n) for n in range(H // 4)]),
               "p": iter([functools.partial(values, n) for n in range(H // 4)])}
        for ch in seq:
            next(its[ch])()
        assert all(next(its[ch], None) is None for ch in ".oqpEHA")
        m2, m4, m3, m5 = (st["acc", m] for m in range(4))
        ca, cb = m2 + m4, m3 + m5
        oc[par, u, :TH, :DH] = m4[M:] - m5[M:]
        oc[par, u, :TH, DH:] = cb[M:]
        oc[par, u, TH:, :DH] = ca[M:]
        oc[par, u, TH:, DH:] = m3[M:] - m2[M:]
        return _rb(jnp.concatenate([ca[:M], cb[:M]], axis=1))

    def group(G, seqs):
        mem, top = state[:M], [state[M:, :128], bidx_ref[:, :128]]
        full = "L" in seqs[0]
        g, par = G % NG, G % 2
        longs = [iter(qkv_group_rounds(G + 2 - par, par) if full else []),
                 iter(out_group_rounds(1 - par, {}))]

        def post(u, t):
            top[:] = epilogue(jnp.where(g >= 2, g - 2, NG), u, t, par, *top)
            if full:
                hn[0, NG + par, 0] = pltpu.bitcast(top[0], U32)
            else:
                tq[R + par, 0, :8] = top[0]
        for u in range(GS):
            mem = segment(G, par, u, mem, seqs[u], longs,
                          [functools.partial(prenorm, (G + 5) % NG, u),
                           functools.partial(ahead_lhs, (G + 4) % NG, u // 2, 10 * (u % 2), 10 + 11 * (u % 2))]
                          + [functools.partial(post, u, t) for t in range(T // 8)])
        assert all(next(it, None) is None for it in longs)
        state[:M] = mem
        state[M:, :128], bidx_ref[:, :128] = top

    def finish_layer(G):
        last = G == 2 * NG - 1
        best, bidx = state[M:, :128], bidx_ref[:, :128]
        todo = [(0, u, t) for u in range(GS) for t in range(4)]
        todo += [(1, u, t) for ts in ((2, 3), (0, 1)) for u in range(GS) for t in ts]
        todo = iter(todo)
        for n, f in enumerate(out_group_rounds(G % 2, {})):
            for par, u, t in [next(todo) for _ in range((n >= 8) + (n >= 22))]:
                best, bidx = epilogue(NG - 2 + par, u, t, par, best, bidx)
                on[1 - G % 2, 0, 0, :8, :128] = pltpu.bitcast(best, U32)
            f()
        for par, u, t in todo:
            best, bidx = epilogue(NG - 2 + par, u, t, par, best, bidx)

        @pl.when(last)
        def _():
            cp_out(NG - 3, NG, 1).start()

        top = jnp.max(best, axis=0, keepdims=True)
        idx = jnp.min(jnp.where(best == top, bidx, S))
        idx = jnp.where(idx >= S, 0, idx)
        g, u = idx // (T * GS), idx // T % GS
        rows = pl.ds(pl.multiple_of(idx % T // 8 * 8, 8), 8)
        x1, xn = xmid[0, g, u, rows], xmid[1, g, u, rows]
        gate = _rb(_dot(xn, wg_s[...]))
        up = _rb(_dot(xn, wu_s[...]))
        gate = _rb(gate * _rb(jax.nn.sigmoid(gate)))
        y = _rb(_dot(_rb(gate * up), wd_s[...]))
        y = _rb(y * _rb(jax.nn.sigmoid(router(xn))))
        sel = lax.broadcasted_iota(I32, (8, D), 0) == idx % 8
        x2 = (x1 + _rb(xn + jnp.where(sel, y, 0.0))).astype(BF)

        @pl.when(last)
        def _():
            cp_out(0, NG - 3, 0).wait()
            cp_out(NG - 3, NG, 1).wait()
            xbuf[g, u, rows] = x2
            cp = pltpu.make_async_copy(xbuf.at[g, u], out_hbm.at[g, u], sems.at[0])
            cp.start()
            cp.wait()

        @pl.when(jnp.logical_not(last))
        def _():
            xbuf[g, u, rows] = x2
            prenorm(g, u)
            ahead_lhs(g, u % (GS // 2))
            reset_state()

            @pl.when(g < 2)
            def _():
                l1 = hc[g, u, 2] + hc[g, u, 1]
                left = [(x[:, :E] + x[:, E:], x[:, E:], x[:, :E]) for x in (l1, hc[g, u, 0] - l1, hc[g, u, 3] - l1)]

                def redo(c2, carry):
                    for c in (2 * c2, 2 * c2 + 1):
                        for i in range(4):
                            ks = (2, 3) if i % 2 else (0, 1)
                            m1, m6, m7 = (sum(_dot(left[m][k % 3], _unpack(wn[c, i // 2, 7 * m + k])) for k in ks)
                                          for m in range(3))
                            tq[NG % R + g, c, t_rows(i, 0, pl.multiple_of(u * TH, TH), TH)] = m1 + m7
                            tq[NG % R + g, c, t_rows(i, 1, pl.multiple_of(u * TH, TH), TH)] = m1 + m6
                    return carry
                lax.fori_loop(0, NC // 2, redo, 0)

    def light_group(G, carry):
        @pl.when(G == 1)
        def _():
            cp_x(XG, NG, 1).wait()
            for c in cp_b:
                c.wait()

        @pl.when(G == 2 * NG - 1)
        def _():
            cp_out(0, NG - 3, 0).start()
        group(G, SEQ_LIGHT)
        return carry

    def full_group(G, carry):
        group(G, SEQ_FULL)
        return carry

    def phase(n, carry):
        edges = (0, PRE - 2, NG, 2 * NG - 2, 2 * NG)
        lo, hi = (functools.reduce(lambda a, k: jnp.where(n == k, edges[k + d], a), range(4), 0) for d in (0, 1))
        light = (n == 0) | (n == 3)
        lax.fori_loop(lo, jnp.where(light, hi, lo), light_group, 0)
        lax.fori_loop(lo, jnp.where(light, lo, hi), full_group, 0)
        pl.when(n % 2 == 1)(lambda: finish_layer(hi - 1))
        return carry

    lax.fori_loop(0, 4, phase, 0)


@functools.partial(jax.jit, static_argnames=("A_seg_len",))
def pallas_interleave_layers__memory_aug_recurrent_mem_tr__moe_arch_mod__prompt_kernel(
    A_x, A_mem0, A_Wq, A_Wk, A_Wv, A_Wo, A_seg_len, B_x, B_w_r, B_w_gate, B_w_up, B_w_down,
):
    del B_x
    B, S, D = A_x.shape
    _, H, E = A_Wq.shape
    M = A_mem0.shape[1]
    F = B_w_gate.shape[1]
    T = int(A_seg_len)
    assert (B, S, D, H, E, M, T) == (1, 2048, 512, 32, 128, 8, 32)
    NG = S // (T * GS)
    NHG = H // 8
    GR = GS * T // 2
    hbm = pl.BlockSpec(memory_space=pl.ANY)
    vmem = pl.BlockSpec(memory_space=pltpu.VMEM)
    out = pl.pallas_call(
        functools.partial(_kernel, S=S, D=D, H=H, E=E, M=M, T=T),
        out_shape=jax.ShapeDtypeStruct((NG, GS, T, D), A_x.dtype),
        in_specs=[hbm, vmem, hbm, hbm, hbm, hbm, vmem, hbm, hbm, hbm],
        out_specs=hbm,
        scratch_shapes=[
            pltpu.VMEM((3 * NHG, D, 8, E), BF),
            pltpu.VMEM((NHG, 8, E, D), BF),
            pltpu.VMEM((3 * NHG, 4, 4, D // 4, E), U32),
            pltpu.VMEM((3 * NHG, 2, 21, E // 2, E), U32),
            pltpu.VMEM((7, NHG, 2 * E, D // 2), U32),
            pltpu.VMEM((NG + 1, GS, T, D), BF),
            pltpu.VMEM((2, NG + 1, GS, T, D), F32),
            pltpu.VMEM((NG, GS, 4, T // 2, D // 2), F32),
            pltpu.VMEM((21, NG + 2, GS // 2, T // 4, E), U32),
            pltpu.VMEM((PRE + 2, 3 * NHG, 8 * GR, E), F32),
            pltpu.VMEM((2, 3, NHG, GR // 2, 4 * E), U32),
            pltpu.VMEM((2, GS, T, D), F32),
            pltpu.VMEM((2, 2, GR, D // 2), F32),
            pltpu.VMEM((M + 8, D), F32),
            pltpu.VMEM((8, 512), I32),
            pltpu.VMEM((D, F), BF),
            pltpu.VMEM((D, F), BF),
            pltpu.VMEM((F, D), BF),
            pltpu.SemaphoreType.DMA((4 * NHG + 5,)),
        ],
        compiler_params=pltpu.CompilerParams(vmem_limit_bytes=120 * 2**20),
        name="rmt_mod",
    )(
        A_x.reshape(NG, GS, T, D), A_mem0.reshape(M, D),
        A_Wq.reshape(D, NHG, 8, E), A_Wk.reshape(D, NHG, 8, E), A_Wv.reshape(D, NHG, 8, E),
        A_Wo.reshape(NHG, 8, E, D),
        B_w_r, B_w_gate, B_w_up, B_w_down,
    )
    return out.reshape(B, S, D)
```

```python
import functools

import numpy as np
import jax
import jax.numpy as jnp
from jax import lax
import jax.experimental.pallas as pl
import jax.experimental.pallas.tpu as pltpu

BF = jnp.bfloat16
F32 = jnp.float32
U32 = jnp.uint32
I32 = jnp.int32

GS = 4

LHS = {1: ((0, 0, 1), (1, 1, 1)), 2: ((1, 0, 1), (1, 1, 1)), 3: ((0, 0, 1),), 4: ((1, 1, 1),),
       5: ((0, 0, 1), (0, 1, 1)), 6: ((1, 0, 1), (0, 0, -1)), 7: ((0, 1, 1), (1, 1, -1))}
RHS = {1: ((0, 0, 1), (1, 1, 1)), 2: ((0, 0, 1),), 3: ((0, 1, 1), (1, 1, -1)), 4: ((1, 0, 1), (0, 0, -1)),
       5: ((1, 1, 1),), 6: ((0, 0, 1), (0, 1, 1)), 7: ((1, 0, 1), (1, 1, 1))}
OUT = {(0, 0): ((4, 1), (7, 1), (1, 1), (5, -1)), (0, 1): ((3, 1), (5, 1)),
       (1, 0): ((2, 1), (4, 1)), (1, 1): ((3, 1), (6, 1), (1, 1), (2, -1))}
BASIS = ((3, 1, 5, 7), (4, 1, 2, 6))
PHASES = ((1, 1, 0), (1, 0, 1), (0, 0, 0), (0, 1, 1))

SEQ_FULL = (
    "...............q...A.....q.......pE.....q.......pE.....q.......pE.....q.......pE.....q.......pH.....q.......p.....q.oooooopoooopoooooooooooooooooooooo",
    "...............q...A.....q.......pE.....q.......pE.....q.......pE.....q.......pE.....q.......pH.....q.......p.....q.oooooopoooopoooooooooooooooooooooo",
    "...............q...A.....q.......pE.....q.......pE.....q.......pE.....q.......pE.....q.......pH.....q.......p.....q.oooooopoooopoooooooooooooooooooooo",
    "...............q...A.....q.......pE.....q.......pE.....q.......pE.....q.......pE.....q.......pH.....q.......p.....q.oooooopoooopoooooooooooooooooooooo",
)


def _rb(v):
    return v.astype(BF).astype(F32)


def _layernorm(x):
    inv_n = 1.0 / x.shape[-1]
    m = jnp.sum(x, axis=-1, keepdims=True) * inv_n
    d = x - m
    v = _rb(jnp.sum(d * d, axis=-1, keepdims=True) * inv_n)
    den = _rb(jnp.sqrt(_rb(v + 1.0013580322265625e-05)))
    return _rb(_rb(x - _rb(m)) * (1.0 / den))


def _dot(a, b):
    return jnp.dot(a, b, preferred_element_type=F32)


def _signed_sum(terms):
    terms = sorted(terms, key=lambda t: -t[1])
    total = terms[0][0] if terms[0][1] > 0 else -terms[0][0]
    for v, sign in terms[1:]:
        total = total + v if sign > 0 else total - v
    return total


def _operand(table, a, b, block, rows=None):
    return _signed_sum([(block(2 * i + k, 2 * j + l), s * t) for i, j, s in table[a] for k, l, t in table[b]
                        if rows is None or 2 * i + k == rows])


def _output(pos, prods):
    terms = [(prods[m], s) for m, s in OUT[pos] if prods.get(m) is not None]
    return _signed_sum(terms) if terms else None


def _weight_operands(block):
    vals = []
    for a in RHS:
        outer = {(k, l): _signed_sum([(block(2 * i + k, 2 * j + l), s) for i, j, s in RHS[a]])
                 for k in range(2) for l in range(2)}
        vals += [_signed_sum([(outer[k, l], t) for k, l, t in RHS[b]]) for b in RHS]
    out = []
    for k in range(0, len(vals), 2):
        w = pltpu.bitcast(jnp.concatenate(vals[k:k + 2], axis=1).astype(BF), U32)
        out += [w[:, c:c + 128] for c in range(0, w.shape[1], 128)]
    return out


class _Phase:
    def __init__(self, u):
        h0, h1, self.wide = PHASES[u]
        self.u, self.row = u, 2 * h0 + h1
        self.ws, self.ns = (BASIS[h] for h in ((h0, h1) if self.wide == 0 else (h1, h0)))

    def pair(self, w, n):
        return (w, n) if self.wide == 0 else (n, w)

    def index(self, w, n):
        a, b = self.pair(w, n)
        return 7 * (a - 1) + b - 1

    def tiles(self, w, n):
        return range(4) if n != 1 else range(self.u, self.u + 1) if w == 1 else range(0)

    def place(self, pw, pn):
        (i, j), (k, l) = self.pair(pw, pn)
        return 2 * i + k, 2 * j + l

    def touched(self):
        return {self.place(pw, pn) for pw in OUT for pn in OUT
                if any(m in self.ws for m, _ in OUT[pw] if m != 1) and any(m in self.ns for m, _ in OUT[pn] if m != 1)}

    def run(self, product, emit, wide_first, order=None, shift=0):
        first, second = (self.ws, self.ns) if wide_first else (self.ns, self.ws)
        first, second = first[shift:] + first[:shift], order or second
        partial = {}
        for m2 in second:
            got = {}
            for m1 in first:
                for t, v in product(*((m1, m2) if wide_first else (m2, m1))).items():
                    got.setdefault(t, {})[m1] = v
                if m1 != first[-1]:
                    yield
            for t, prods in got.items():
                for p1 in OUT:
                    partial.setdefault((t, p1), {})[m2] = _output(p1, prods)
            for p2, terms in OUT.items():
                need = [m for m in second if m in dict(terms)]
                if need and need[-1] == m2:
                    for (t, p1), prods in partial.items():
                        i, j = self.place(*((p1, p2) if wide_first else (p2, p1)))
                        if (i == self.row) if t is None else ((i, j) in self.touched()):
                            emit(i, j, t, _output(p2, prods))
            yield


def _kernel(x_hbm, mem0_ref, wq_hbm, wk_hbm, wv_hbm, wo_hbm, wr_ref, wg_hbm, wu_hbm, wd_hbm,
            out_hbm,
            raw, wo_raw, wqkv, wout, xbuf, xmid, hbuf, hl, qkv, obuf, oacc, state, bidx_ref,
            wg_s, wu_s, wd_s, sems,
            *, S, D, H, E, M, T):
    NG = S // (T * GS)
    L = M + T
    NQ = H // 4
    NHG = H // 8
    NC = 3 * NHG
    XG = 5
    w_hbm = (wq_hbm, wk_hbm, wv_hbm)
    phases = [_Phase(u) for u in range(GS)]

    def cp_w(j, hg):
        return pltpu.make_async_copy(w_hbm[j].at[:, hg], raw.at[j * NHG + hg], sems.at[j * NHG + hg])

    def cp_o(k):
        return pltpu.make_async_copy(wo_hbm.at[k], wo_raw.at[k], sems.at[NC + k])

    def cp_x(lo, hi, k):
        return pltpu.make_async_copy(x_hbm.at[pl.ds(lo, hi - lo)], xbuf.at[pl.ds(lo, hi - lo)], sems.at[NC + NHG + k])

    def cp_out(lo, hi, k):
        return pltpu.make_async_copy(xbuf.at[pl.ds(lo, hi - lo)], out_hbm.at[pl.ds(lo, hi - lo)], sems.at[NC + NHG + k])

    cp_b = [pltpu.make_async_copy(w, s, sems.at[NC + NHG + 2 + j])
            for j, (w, s) in enumerate(((wg_hbm, wg_s), (wu_hbm, wu_s), (wd_hbm, wd_s)))]

    def normed(x):
        x = x.astype(F32)
        d = x - jnp.sum(x, axis=-1, keepdims=True) * (1.0 / D)
        return d * lax.rsqrt(jnp.sum(d * d, axis=-1, keepdims=True) * (1.0 / D) + 1e-5)

    def prenorm(g, u):
        hbuf[g, u] = normed(xbuf[g, u])

    def rows_of(tiles):
        return pl.ds(tiles[0] * 8, len(tiles) * 8)

    def build_lhs(g, ph):
        for n in ph.ns:
            for w in ph.ws:
                if ph.tiles(w, n):
                    rows = rows_of(ph.tiles(w, n))
                    hl[ph.index(w, n), rows] = _operand(LHS, *ph.pair(w, n),
                                                        lambda s, k: hbuf[g, s, rows, pl.ds(k * E, E)])

    def accumulate(ref, ph, i, j, index, v):
        seen = any((i, j) in p.touched() for p in phases[:ph.u])
        ref[index] = v + ref[index] if seen else v

    def split(res, tiles, mem_first, with_mem):
        off = M if with_mem and mem_first else 0
        out = {t: res[off + 8 * n:off + 8 * n + 8] for n, t in enumerate(tiles)}
        if with_mem:
            out[None] = res[:M] if mem_first else res[-M:]
        return out

    def qkv_block(ph, par, blk, mem_lhs, mem_out, shift=0):
        def product(w, n):
            tiles = ph.tiles(w, n)
            left = [hl[ph.index(w, n), rows_of(tiles)]] if tiles else []
            left += [mem_lhs[w, n]] if mem_lhs else []
            if not left:
                return {}
            res = _dot(jnp.concatenate(left, axis=0), pltpu.bitcast(wqkv[blk, ph.index(w, n)], BF))
            return split(res, tiles, False, mem_lhs)

        def emit(i, j, t, v):
            if t is None:
                mem_out[j] = v
            else:
                accumulate(qkv, ph, i, j, (par, blk, pl.ds((4 * i + j) * T + t * 8, 8)), v)
        return ph.run(product, emit, True, shift=shift)

    def out_rounds(ph, par, mem_in, mem_out):
        def half(w, n, k):
            tiles = ph.tiles(w, n)
            left = [_operand(LHS, *ph.pair(w, n), lambda s, j: mem_in(j, k), ph.row)] if mem_in else []
            if tiles:
                left += [_operand(LHS, *ph.pair(w, n),
                                  lambda s, j: obuf[par, s, j, rows_of(tiles), pl.ds(k * 4 * E, 4 * E)])]
            if left:
                return _dot(jnp.concatenate(left, axis=0),
                            pltpu.bitcast(wout[ph.index(w, n), pl.ds(k * 2 * E, 2 * E)], BF))

        def product(w, n):
            res = half(w, n, 1)
            return {} if res is None else split(res + early[w, n], ph.tiles(w, n), True, mem_in)

        def emit(i, j, t, v):
            if t is None:
                mem_out[j] = v
            else:
                accumulate(oacc, ph, i, j, (par, i, pl.ds(t * 8, 8), pl.ds(j * E, E)), v)
        early = {}
        for w in ph.ws[::-1]:
            for n in ph.ns:
                early[w, n] = half(w, n, 0)
                yield
        yield from ph.run(product, emit, False, ph.ws[::-1])

    cp_w(0, 0).start()
    cp_x(0, XG, 0).start()
    for c in range(1, NC):
        cp_w(c // NHG, c % NHG).start()
    for k in range(NHG):
        cp_o(k).start()
    cp_x(XG, NG, 1).start()
    for c in cp_b:
        c.start()
    xbuf[NG] = jnp.zeros((GS, T, D), BF)
    oacc[0] = jnp.zeros(oacc.shape[1:], F32)
    obuf[1] = jnp.zeros(obuf.shape[1:], F32)

    def prep_qkv(c, r, carry):
        for k in range(4):
            words = pltpu.bitcast(raw[c, pl.ds(k * E + r * 16, 16)].reshape(128, E), U32)
            qkv[1, 0, pl.ds(k * 64, 64)] = pltpu.bitcast(words, F32)
        for n in range(2):
            words = {(k, i): pltpu.bitcast(qkv[1, 0, pl.ds(k * 64 + 2 * n + i, 16, stride=4), :], U32)
                     for k in range(4) for i in range(2)}
            blocks = {(k, 2 * i + h): pltpu.bitcast(w & np.uint32(0xFFFF0000) if h else w << 16, F32)
                      for (k, i), w in words.items() for h in range(2)}
            for m, w in enumerate(_weight_operands(lambda k, j: blocks[k, j])):
                wqkv[2 * c + n, m, pl.ds(pl.multiple_of(r * 8, 8), 8)] = w
        return carry

    def stream(c, carry):
        pltpu.make_async_copy(raw.at[c], raw.at[c], sems.at[c]).wait()
        lax.fori_loop(0, E // 16, functools.partial(prep_qkv, c), 0, unroll=2)

        @pl.when(c == 0)
        def _():
            cp_x(0, XG, 0).wait()
            hbuf[:3] = normed(xbuf[:3].reshape((3) * GS * T, D)).reshape(3, GS, T, D)
            for ph in phases:
                build_lhs(0, ph)
        for ph in phases:
            for n in range(2):
                for _ in qkv_block(ph, 0, 2 * c + n, None, None):
                    pass
        return carry
    lax.fori_loop(0, NC, stream, 0)
    build_lhs(1, phases[0])

    def prep_out(k, r, carry):
        rows = pl.ds(pl.multiple_of(r * 16, 16), 16)
        for n in range(2):
            heads = [wo_raw[k, 4 * n + i, rows].astype(F32) for i in range(4)]
            for m, w in enumerate(_weight_operands(lambda i, j: heads[i][:, j * E:j * E + E])):
                wout[m, pl.ds(pl.multiple_of((2 * k + n) * (E // 2) + r * 8, 8), 8)] = w
        return carry

    def stream_o(k, carry):
        cp_o(k).wait()
        lax.fori_loop(0, E // 16, functools.partial(prep_out, k), 0, unroll=2)
        return carry
    lax.fori_loop(0, NHG, stream_o, 0)

    def reset_state():
        state[:M] = mem0_ref[...].astype(F32)
        state[M:] = jnp.full((8, D), -jnp.inf, F32)
        bidx_ref[:, :128] = jnp.full((8, 128), S, I32)
    reset_state()

    def router(xn):
        return _rb(jnp.sum(xn * wr_ref[...].astype(F32).reshape(1, D), axis=-1, keepdims=True))

    def epilogue(g, u, t, par, best, bidx):
        rows = pl.ds(t * 8, 8)
        x1 = _rb(xbuf[g, u, rows].astype(F32) + _rb(oacc[par, u, rows]))
        xn = _layernorm(x1)
        xmid[0, g, u, rows] = x1
        xmid[1, g, u, rows] = xn
        xbuf[g, u, rows] = (x1 + xn).astype(BF)
        it = lax.broadcasted_iota(I32, (8, 128), 0) + ((g * GS + u) * T + t * 8)
        r = jnp.where(it < S, jnp.broadcast_to(router(xn), (8, 128)), -jnp.inf)
        better = r > best
        return jnp.where(better, r, best), jnp.where(better, it, bidx)

    def segment(par, ph, mem, seq, jobs):
        u = ph.u
        row = lax.broadcasted_iota(I32, (L, L), 0)
        col = lax.broadcasted_iota(I32, (L, L), 1)
        mask = (row < M) | (row >= col)
        mem_lhs = {(w, n): _operand(LHS, *ph.pair(w, n), lambda s, k: mem[k], ph.row) for n in ph.ns for w in ph.ws}
        proj = [{} for _ in range(3 * NQ)]
        probs, outs, new_mem = {}, {}, {}

        def head(j, n, i):
            return jnp.concatenate([proj[j * NQ + n][i], qkv[par, j * NQ + n, pl.ds((4 * u + i) * T, T)]], axis=0)

        def scores(n):
            for i in range(4):
                sc = lax.dot_general(head(0, n, i), head(1, n, i).astype(BF), (((1,), (1,)), ((), ())),
                                     preferred_element_type=F32)
                sc = jnp.where(mask, sc, -1e9 * E ** 0.5)
                e = jnp.exp2((sc - jnp.max(sc, axis=-1, keepdims=True)) * (E ** -0.5 * 1.4426950408889634))
                probs[n, i] = e * pltpu.reciprocal(jnp.sum(e, axis=-1, keepdims=True), full_range=False)

        def values(n):
            for i in range(4):
                o = _dot(probs[n, i], head(2, n, i).astype(BF))
                outs[n, i] = o[:M]
                obuf[par, u, i, :, pl.ds(n * E, E)] = o[M:]

        def rounds():
            order = [(j, n - (j == 2)) for n in range(NQ + 1) for j in range(3) if 0 <= n - (j == 2) < NQ]
            for count, (j, n) in enumerate(order):
                for k, _ in enumerate(qkv_block(ph, 1 - par, j * NQ + n, mem_lhs, proj[j * NQ + n], count % 4)):
                    if k % 4 == 3:
                        yield

        def mem_in(i, k):
            return jnp.concatenate([outs[n, i] for n in range(4 * k, 4 * k + 4)], axis=1)
        its = {".": rounds(), "o": out_rounds(ph, 1 - par, mem_in, new_mem),
               "q": map(scores, range(NQ)), "p": map(values, range(NQ))}
        its.update({ch: (f() for f in fs) for ch, fs in jobs.items()})
        for ch in seq:
            next(its[ch])
        assert not any(list(it) for it in its.values())
        return [_rb(new_mem[j]) for j in range(4)]

    def group_pair(G0):
        mem, top = [state[:M, pl.ds(j * E, E)] for j in range(4)], [state[M:, :128], bidx_ref[:, :128]]
        for par in range(2):
            G = G0 + par
            g = G % NG

            def post(u, t):
                top[:] = epilogue(jnp.where(g >= 2, g - 2, NG), u, t, par, *top)
                hl[49 + G0 // NG, :8] = top[0]

            for u in range(GS):
                mem = segment(par, phases[u], mem, SEQ_FULL[(par * GS + u) % len(SEQ_FULL)], {
                    "H": [functools.partial(prenorm, (G + 3) % NG, u)],
                    "A": [functools.partial(build_lhs, (G + 1 + (u + 1) // GS) % NG, phases[(u + 1) % GS])],
                    "E": [functools.partial(post, u, t) for t in range(T // 8)]})
        for j in range(4):
            state[:M, pl.ds(j * E, E)] = mem[j]
        state[M:, :128], bidx_ref[:, :128] = top

    def finish_layer(last):
        best, bidx = state[M:, :128], bidx_ref[:, :128]
        for par in range(2):
            if par:
                for ph in phases:
                    for _ in out_rounds(ph, par, None, None):
                        pass
            for u in range(GS):
                for t in range(T // 8):
                    best, bidx = epilogue(NG - 2 + par, u, t, par, best, bidx)

        @pl.when(last)
        def _():
            cp_out(NG - 4, NG, 1).start()

        top = jnp.max(best, axis=0, keepdims=True)
        idx = jnp.min(jnp.where(best == top, bidx, S))
        idx = jnp.where(idx >= S, 0, idx)
        g, u = idx // (T * GS), idx // T % GS
        tile = pl.multiple_of(idx % T // 8 * 8, 8)
        rows = pl.ds(tile, 8)
        x1, xn = xmid[0, g, u, rows], xmid[1, g, u, rows]
        gate = _rb(_dot(xn, wg_s[...]))
        up = _rb(_dot(xn, wu_s[...]))
        gate = _rb(gate * _rb(jax.nn.sigmoid(gate)))
        y = _rb(_dot(_rb(gate * up), wd_s[...]))
        y = _rb(y * _rb(jax.nn.sigmoid(router(xn))))
        sel = lax.broadcasted_iota(I32, (8, D), 0) == idx % 8
        x2 = (x1 + _rb(xn + jnp.where(sel, y, 0.0))).astype(BF)

        @pl.when(last)
        def _():
            cp_out(0, NG - 4, 0).wait()
            cp_out(NG - 4, NG, 1).wait()
            xbuf[g, u, rows] = x2
            cp = pltpu.make_async_copy(xbuf.at[g, u], out_hbm.at[g, u], sems.at[0])
            cp.start()
            cp.wait()

        @pl.when(jnp.logical_not(last))
        def _():
            xbuf[g, u, rows] = x2
            h = normed(x2)
            hbuf[g, u, rows] = h
            build_lhs(1, phases[0])
            reset_state()

            @pl.when(g == 0)
            def _():
                ph = phases[0]
                left = {(w, n): _operand(LHS, *ph.pair(w, n), lambda s, k: h[:, k * E:k * E + E], ph.row)
                        for n in ph.ns for w in ph.ws}

                def redo(blk, carry):
                    def emit(i, j, t, v):
                        qkv[0, blk, pl.ds(pl.multiple_of((4 * u + j) * T + tile, 8), 8)] = v
                    for _ in ph.run(lambda w, n: {None: _dot(left[w, n], pltpu.bitcast(wqkv[blk, ph.index(w, n)], BF))},
                                    emit, True):
                        pass
                    return carry
                lax.fori_loop(0, 3 * NQ, redo, 0, unroll=4)

    def iteration(it, carry):
        last = it == NG - 1

        @pl.when(it == 1)
        def _():
            cp_x(XG, NG, 1).wait()
            for c in cp_b:
                c.wait()

        @pl.when(last)
        def _():
            cp_out(0, NG - 4, 0).start()
        group_pair(2 * it)
        pl.when(it % (NG // 2) == NG // 2 - 1)(lambda: finish_layer(last))
        return carry

    lax.fori_loop(0, NG, iteration, 0)


@functools.partial(jax.jit, static_argnames=("A_seg_len",))
def pallas_interleave_layers__memory_aug_recurrent_mem_tr__moe_arch_mod__prompt_kernel(
    A_x, A_mem0, A_Wq, A_Wk, A_Wv, A_Wo, A_seg_len, B_x, B_w_r, B_w_gate, B_w_up, B_w_down,
):
    del B_x
    B, S, D = A_x.shape
    _, H, E = A_Wq.shape
    M = A_mem0.shape[1]
    F = B_w_gate.shape[1]
    T = int(A_seg_len)
    assert (B, S, D, H, E, M, T) == (1, 2048, 512, 32, 128, 8, 32)
    NG = S // (T * GS)
    NHG = H // 8
    hbm = pl.BlockSpec(memory_space=pl.ANY)
    vmem = pl.BlockSpec(memory_space=pltpu.VMEM)
    out = pl.pallas_call(
        functools.partial(_kernel, S=S, D=D, H=H, E=E, M=M, T=T),
        out_shape=jax.ShapeDtypeStruct((NG, GS, T, D), A_x.dtype),
        in_specs=[hbm, vmem, hbm, hbm, hbm, hbm, vmem, hbm, hbm, hbm],
        out_specs=hbm,
        scratch_shapes=[
            pltpu.VMEM((3 * NHG, D, 8, E), BF),
            pltpu.VMEM((NHG, 8, E, D), BF),
            pltpu.VMEM((3 * H // 4, 49, E // 2, E), U32),
            pltpu.VMEM((49, H // 4 * E // 2, E), U32),
            pltpu.VMEM((NG + 1, GS, T, D), BF),
            pltpu.VMEM((2, NG + 1, GS, T, D), F32),
            pltpu.VMEM((NG, GS, T, D), F32),
            pltpu.VMEM((51, T, E), F32),
            pltpu.VMEM((2, 3 * H // 4, GS * 4 * T, E), F32),
            pltpu.VMEM((2, GS, 4, T, H // 4 * E), F32),
            pltpu.VMEM((2, GS, T, D), F32),
            pltpu.VMEM((M + 8, D), F32),
            pltpu.VMEM((8, 512), I32),
            pltpu.VMEM((D, F), BF),
            pltpu.VMEM((D, F), BF),
            pltpu.VMEM((F, D), BF),
            pltpu.SemaphoreType.DMA((4 * NHG + 5,)),
        ],
        compiler_params=pltpu.CompilerParams(vmem_limit_bytes=120 * 2**20),
        name="rmt_mod",
    )(
        A_x.reshape(NG, GS, T, D), A_mem0.reshape(M, D),
        A_Wq.reshape(D, NHG, 8, E), A_Wk.reshape(D, NHG, 8, E), A_Wv.reshape(D, NHG, 8, E),
        A_Wo.reshape(NHG, 8, E, D),
        B_w_r, B_w_gate, B_w_up, B_w_down,
    )
    return out.reshape(B, S, D)
```

```python
import functools

import numpy as np
import jax
import jax.numpy as jnp
from jax import lax
import jax.experimental.pallas as pl
import jax.experimental.pallas.tpu as pltpu

BF = jnp.bfloat16
F32 = jnp.float32
U32 = jnp.uint32
I32 = jnp.int32

GS = 4

LHS = {1: ((0, 0, 1), (1, 1, 1)), 2: ((1, 0, 1), (1, 1, 1)), 3: ((0, 0, 1),), 4: ((1, 1, 1),),
       5: ((0, 0, 1), (0, 1, 1)), 6: ((1, 0, 1), (0, 0, -1)), 7: ((0, 1, 1), (1, 1, -1))}
RHS = {1: ((0, 0, 1), (1, 1, 1)), 2: ((0, 0, 1),), 3: ((0, 1, 1), (1, 1, -1)), 4: ((1, 0, 1), (0, 0, -1)),
       5: ((1, 1, 1),), 6: ((0, 0, 1), (0, 1, 1)), 7: ((1, 0, 1), (1, 1, 1))}
OUT = {(0, 0): ((4, 1), (7, 1), (1, 1), (5, -1)), (0, 1): ((3, 1), (5, 1)),
       (1, 0): ((2, 1), (4, 1)), (1, 1): ((3, 1), (6, 1), (1, 1), (2, -1))}
BASIS = ((3, 1, 5, 7), (4, 1, 2, 6))
PHASES = ((1, 1, 0), (1, 0, 1), (0, 0, 0), (0, 1, 1))

SEQ_FULL = (
    "xx....A............q......q........p......q......p......q......p......EqEEE......p......q.....p.......q......p......qoooooopooooopoooooooHoooooooooooooo",
    "x........A........q........q......p......q......p......q......p......EqEEE..p..........q.....p.......q......p......qoooooopooooopoooHoooooooooooooooooo",
    "xx........A........q........q.......p.........q...p.....qEEEE..........p..q......p......q......p......q......p......qooooopooooopooooHoooooooooooooooooo",
    "x........A........q........q......p......q......p......q......p......qEE..p...E..E.....q.....p.......q......p......qoooooopooooopoooHoooooooooooooooooo",
)


def _rb(v):
    return v.astype(BF).astype(F32)


def _layernorm(x):
    inv_n = 1.0 / x.shape[-1]
    m = jnp.sum(x, axis=-1, keepdims=True) * inv_n
    d = x - m
    v = _rb(jnp.sum(d * d, axis=-1, keepdims=True) * inv_n)
    den = _rb(jnp.sqrt(_rb(v + 1.0013580322265625e-05)))
    return _rb(_rb(x - _rb(m)) * (1.0 / den))


def _dot(a, b):
    return jnp.dot(a, b, preferred_element_type=F32)


def _signed_sum(terms):
    terms = sorted(terms, key=lambda t: -t[1])
    total = terms[0][0] if terms[0][1] > 0 else -terms[0][0]
    for v, sign in terms[1:]:
        total = total + v if sign > 0 else total - v
    return total


def _operand(table, a, b, block, rows=None):
    return _signed_sum([(block(2 * i + k, 2 * j + l), s * t) for i, j, s in table[a] for k, l, t in table[b]
                        if rows is None or 2 * i + k == rows])


def _output(pos, prods):
    terms = [(prods[m], s) for m, s in OUT[pos] if prods.get(m) is not None]
    return _signed_sum(terms) if terms else None


def _weight_operands(block):
    vals = []
    for a in RHS:
        outer = {(k, l): _signed_sum([(block(2 * i + k, 2 * j + l), s) for i, j, s in RHS[a]])
                 for k in range(2) for l in range(2)}
        for b in RHS:
            vals.append(_signed_sum([(outer[k, l], t) for k, l, t in RHS[b]]))
            if len(vals) == 2 or a == b == 7:
                w = pltpu.bitcast(jnp.concatenate(vals, axis=1).astype(BF), U32)
                yield from (w[:, c:c + 128] for c in range(0, w.shape[1], 128))
                vals = []


class _Phase:
    def __init__(self, u):
        h0, h1, self.wide = PHASES[u]
        self.u, self.row = u, 2 * h0 + h1
        self.ws, self.ns = (BASIS[h] for h in ((h0, h1) if self.wide == 0 else (h1, h0)))

    def pair(self, w, n):
        return (w, n) if self.wide == 0 else (n, w)

    def index(self, w, n):
        a, b = self.pair(w, n)
        return 7 * (a - 1) + b - 1

    def tiles(self, w, n):
        return range(4) if n != 1 else range(self.u, self.u + 1) if w == 1 else range(0)

    def place(self, pw, pn):
        (i, j), (k, l) = self.pair(pw, pn)
        return 2 * i + k, 2 * j + l

    def touched(self):
        return {self.place(pw, pn) for pw in OUT for pn in OUT
                if any(m in self.ws for m, _ in OUT[pw] if m != 1) and any(m in self.ns for m, _ in OUT[pn] if m != 1)}

    def run(self, product, emit, wide_first, order=None):
        first, second = (self.ws, self.ns) if wide_first else (self.ns, self.ws)
        second = order or second
        partial = {}
        for m2 in second:
            got = {}
            for m1 in first:
                for t, v in product(*((m1, m2) if wide_first else (m2, m1))).items():
                    got.setdefault(t, {})[m1] = v
                if m1 != first[-1]:
                    yield
            for t, prods in got.items():
                for p1 in OUT:
                    partial.setdefault((t, p1), {})[m2] = _output(p1, prods)
            for p2, terms in OUT.items():
                need = [m for m in second if m in dict(terms)]
                if need and need[-1] == m2:
                    for (t, p1), prods in partial.items():
                        i, j = self.place(*((p1, p2) if wide_first else (p2, p1)))
                        if (i == self.row) if t is None else ((i, j) in self.touched()):
                            emit(i, j, t, _output(p2, prods))
            yield


def _kernel(x_hbm, mem0_ref, wq_hbm, wk_hbm, wv_hbm, wo_hbm, wr_ref, wg_hbm, wu_hbm, wd_hbm,
            out_hbm,
            raw, wo_raw, wqkv, wout, xbuf, xmid, hbuf, hl, qkv, obuf, oacc, state, bidx_ref,
            wg_s, wu_s, wd_s, sems,
            *, S, D, H, E, M, T):
    NG = S // (T * GS)
    L = M + T
    NQ = H // 4
    NHG = H // 8
    NC = 3 * NHG
    XG = 5
    w_hbm = (wq_hbm, wk_hbm, wv_hbm)
    phases = [_Phase(u) for u in range(GS)]

    def cp_w(j, hg):
        return pltpu.make_async_copy(w_hbm[j].at[:, hg], raw.at[j * NHG + hg], sems.at[j * NHG + hg])

    def cp_o(k):
        return pltpu.make_async_copy(wo_hbm.at[k], wo_raw.at[k], sems.at[NC + k])

    def cp_x(lo, hi, k):
        return pltpu.make_async_copy(x_hbm.at[pl.ds(lo, hi - lo)], xbuf.at[pl.ds(lo, hi - lo)], sems.at[NC + NHG + k])

    def cp_out(lo, hi, k):
        return pltpu.make_async_copy(xbuf.at[pl.ds(lo, hi - lo)], out_hbm.at[pl.ds(lo, hi - lo)], sems.at[NC + NHG + k])

    cp_b = [pltpu.make_async_copy(w, s, sems.at[NC + NHG + 2 + j])
            for j, (w, s) in enumerate(((wg_hbm, wg_s), (wu_hbm, wu_s), (wd_hbm, wd_s)))]

    def normed(x):
        x = x.astype(F32)
        d = x - jnp.sum(x, axis=-1, keepdims=True) * (1.0 / D)
        return d * lax.rsqrt(jnp.sum(d * d, axis=-1, keepdims=True) * (1.0 / D) + 1e-5)

    def prenorm(g, u):
        hbuf[g, u] = normed(xbuf[g, u])

    def rows_of(tiles):
        return pl.ds(tiles[0] * 8, len(tiles) * 8)

    def build_lhs(g, ph):
        for n in ph.ns:
            for w in ph.ws:
                if n != 1 or (w, ph.u) == (1, 0):
                    hl[ph.index(w, n)] = _operand(LHS, *ph.pair(w, n), lambda s, k: hbuf[g, s, :, pl.ds(k * E, E)])

    def accumulate(ref, ph, i, j, index, v):
        seen = any((i, j) in p.touched() for p in phases[:ph.u])
        ref[index] = v + ref[index] if seen else v

    def split(res, tiles, mem_first, with_mem):
        off = M if with_mem and mem_first else 0
        out = {t: res[off + 8 * n:off + 8 * n + 8] for n, t in enumerate(tiles)}
        if with_mem:
            out[None] = res[:M] if mem_first else res[-M:]
        return out

    def first_product(blk):
        return _dot(hl[0], pltpu.bitcast(wqkv[blk, 0], BF))

    def qkv_block(ph, par, blk, mem_lhs, mem_out, first):
        def product(w, n):
            tiles = range(4 * (n != 1))
            left = [hl[ph.index(w, n)]] if tiles else []
            left += [mem_lhs[w, n]] if mem_lhs else []
            out = split(first, range(4), False, False) if (w, n) == (1, 1) and first is not None else {}
            if left:
                res = _dot(jnp.concatenate(left, axis=0), pltpu.bitcast(wqkv[blk, ph.index(w, n)], BF))
                out.update(split(res, tiles, False, mem_lhs))
            return out

        def emit(i, j, t, v):
            if t is None:
                mem_out[j] = v
            else:
                accumulate(qkv, ph, i, j, (par, blk, pl.ds((4 * i + j) * T + t * 8, 8)), v)
        return ph.run(product, emit, True)

    def out_rounds(ph, par, mem_in, mem_out):
        def half(w, n, k):
            tiles = ph.tiles(w, n)
            left = [_operand(LHS, *ph.pair(w, n), lambda s, j: mem_in(j, k), ph.row)] if mem_in else []
            if tiles:
                left += [_operand(LHS, *ph.pair(w, n),
                                  lambda s, j: obuf[par, s, j, rows_of(tiles), pl.ds(k * 4 * E, 4 * E)])]
            if left:
                return _dot(jnp.concatenate(left, axis=0),
                            pltpu.bitcast(wout[ph.index(w, n), pl.ds(k * 2 * E, 2 * E)], BF))

        def product(w, n):
            res = half(w, n, 1)
            return {} if res is None else split(res + early[w, n], ph.tiles(w, n), True, mem_in)

        def emit(i, j, t, v):
            if t is None:
                mem_out[j] = v
            else:
                accumulate(oacc, ph, i, j, (par, i, pl.ds(t * 8, 8), pl.ds(j * E, E)), v)
        early = {}
        for w in ph.ws[::-1]:
            for n in ph.ns:
                early[w, n] = half(w, n, 0)
                yield
        yield from ph.run(product, emit, False, ph.ws[::-1])

    cp_w(0, 0).start()
    cp_x(0, XG, 0).start()
    for c in range(1, NC):
        cp_w(c // NHG, c % NHG).start()
    for k in range(NHG):
        cp_o(k).start()
    cp_x(XG, NG, 1).start()
    for c in cp_b:
        c.start()
    xbuf[NG] = jnp.zeros((GS, T, D), BF)
    oacc[0] = jnp.zeros(oacc.shape[1:], F32)
    obuf[1] = jnp.zeros(obuf.shape[1:], F32)

    def prep_qkv(c):
        for r in range(E // 16):
            for k in range(4):
                words = pltpu.bitcast(raw[c, pl.ds(k * E + r * 16, 16)].reshape(128, E), U32)
                qkv[1, r, pl.ds(k * 64, 64)] = pltpu.bitcast(words, F32)
            for n in range(2):
                def block(k, j):
                    w = pltpu.bitcast(qkv[1, r, pl.ds(k * 64 + 2 * n + j // 2, 16, stride=4), :], U32)
                    return pltpu.bitcast(w & np.uint32(0xFFFF0000) if j % 2 else w << 16, F32)
                for m, w in enumerate(_weight_operands(block)):
                    wqkv[2 * c + n, m, pl.ds(r * 8, 8)] = w

    def stream(c, carry):
        pltpu.make_async_copy(raw.at[c], raw.at[c], sems.at[c]).wait()
        prep_qkv(c)

        @pl.when(c == 0)
        def _():
            cp_x(0, XG, 0).wait()
            hbuf[:3] = normed(xbuf[:3].reshape(3 * GS * T, D)).reshape(3, GS, T, D)
            for ph in phases:
                build_lhs(0, ph)

        @pl.when(c % 2 == 1)
        def _():
            blocks = [2 * c - 2 + n for n in range(4)]
            firsts = [first_product(blk) for blk in blocks]
            for ph in phases:
                for blk, first in zip(blocks, firsts):
                    list(qkv_block(ph, 0, blk, None, None, None if ph.u else first))
        return carry
    lax.fori_loop(0, NC, stream, 0)
    build_lhs(1, phases[0])

    def stream_o(k, carry):
        cp_o(k).wait()
        for r in range(E // 16):
            for n in range(2):
                heads = [wo_raw[k, 4 * n + i, pl.ds(r * 16, 16)].astype(F32) for i in range(4)]
                for m, w in enumerate(_weight_operands(lambda i, j: heads[i][:, j * E:j * E + E])):
                    wout[m, pl.ds(pl.multiple_of((2 * k + n) * (E // 2) + r * 8, 8), 8)] = w
        return carry
    lax.fori_loop(0, NHG, stream_o, 0)

    def reset_state():
        state[:M] = mem0_ref[...].astype(F32)
        state[M:] = jnp.full((8, D), -jnp.inf, F32)
        bidx_ref[:, :128] = jnp.full((8, 128), S, I32)
    reset_state()

    def router(xn):
        return _rb(jnp.sum(xn * wr_ref[...].astype(F32).reshape(1, D), axis=-1, keepdims=True))

    def epilogue(g, u, t, par, best, bidx):
        rows = pl.ds(t * 8, 8)
        x1 = _rb(xbuf[g, u, rows].astype(F32) + _rb(oacc[par, u, rows]))
        xn = _layernorm(x1)
        xmid[0, g, u, rows] = x1
        xmid[1, g, u, rows] = xn
        xbuf[g, u, rows] = (x1 + xn).astype(BF)
        it = lax.broadcasted_iota(I32, (8, 128), 0) + ((g * GS + u) * T + t * 8)
        r = jnp.where(it < S, jnp.broadcast_to(router(xn), (8, 128)), -jnp.inf)
        better = r > best
        return jnp.where(better, r, best), jnp.where(better, it, bidx)

    def segment(par, ph, mem, seq, jobs, firsts, first_rounds):
        u = ph.u
        row = lax.broadcasted_iota(I32, (L, L), 0)
        col = lax.broadcasted_iota(I32, (L, L), 1)
        mask = (row < M) | (row >= col)
        mem_lhs = {(w, n): _operand(LHS, *ph.pair(w, n), lambda s, k: mem[k], ph.row) for n in ph.ns for w in ph.ws}
        proj = [{} for _ in range(3 * NQ)]
        probs, outs, new_mem = {}, {}, {}

        def head(j, n, i):
            return jnp.concatenate([proj[j * NQ + n][i], qkv[par, j * NQ + n, pl.ds((4 * u + i) * T, T)]], axis=0)

        def scores(n):
            for i in range(4):
                sc = lax.dot_general(head(0, n, i), head(1, n, i).astype(BF), (((1,), (1,)), ((), ())),
                                     preferred_element_type=F32)
                sc = jnp.where(mask, sc, -1e9 * E ** 0.5)
                e = jnp.exp2((sc - jnp.max(sc, axis=-1, keepdims=True)) * (E ** -0.5 * 1.4426950408889634))
                probs[n, i] = e * pltpu.reciprocal(jnp.sum(e, axis=-1, keepdims=True), full_range=False)

        def values(n):
            for i in range(4):
                o = _dot(probs[n, i], head(2, n, i).astype(BF))
                outs[n, i] = o[:M]
                obuf[par, u, i, :, pl.ds(n * E, E)] = o[M:]

        def rounds():
            order = [(j, n - (j == 2)) for n in range(NQ + 1) for j in range(3) if 0 <= n - (j == 2) < NQ]
            for blk in (j * NQ + n for j, n in order):
                for k, _ in enumerate(qkv_block(ph, 1 - par, blk, mem_lhs, proj[blk], firsts.pop(blk, None))):
                    if k % 4 == 3:
                        yield

        def mem_in(i, k):
            return jnp.concatenate([outs[n, i] for n in range(4 * k, 4 * k + 4)], axis=1)
        its = {".": rounds(), "o": out_rounds(ph, 1 - par, mem_in, new_mem),
               "q": map(scores, range(NQ)), "p": map(values, range(NQ))}
        its.update({ch: (f() for f in fs) for ch, fs in jobs.items()})
        for ch in seq:
            next(first_rounds if ch == "x" else its[ch])
        assert not any(list(it) for it in its.values())
        return [_rb(new_mem[j]) for j in range(4)]

    def group_pair(G0):
        mem, top = [state[:M, pl.ds(j * E, E)] for j in range(4)], [state[M:, :128], bidx_ref[:, :128]]
        for par in range(2):
            G = G0 + par
            g = G % NG

            def post(u, t):
                top[:] = epilogue(jnp.where(g >= 2, g - 2, NG), u, t, par, *top)
                hl[49 + G0 // NG, :8] = top[0]

            firsts = {}
            first_rounds = (firsts.update({blk: first_product(blk) for blk in range(k, k + 4)})
                            for k in range(0, 3 * NQ, 4))
            for u in range(GS):
                mem = segment(par, phases[u], mem, SEQ_FULL[(par * GS + u) % len(SEQ_FULL)], {
                    "H": [functools.partial(prenorm, (G + 3) % NG, u)],
                    "A": [functools.partial(build_lhs, (G + 1 + (u + 1) // GS) % NG, phases[(u + 1) % GS])],
                    "E": [functools.partial(post, u, t) for t in range(T // 8)]}, firsts, first_rounds)
            assert not firsts and not list(first_rounds)
        for j in range(4):
            state[:M, pl.ds(j * E, E)] = mem[j]
        state[M:, :128], bidx_ref[:, :128] = top

    def finish_layer(last):
        best, bidx = state[M:, :128], bidx_ref[:, :128]
        for par in range(2):
            if par:
                for ph in phases:
                    for _ in out_rounds(ph, par, None, None):
                        pass
            for u in range(GS):
                for t in range(T // 8):
                    best, bidx = epilogue(NG - 2 + par, u, t, par, best, bidx)

        @pl.when(last)
        def _():
            cp_out(NG - 4, NG, 1).start()

        top = jnp.max(best, axis=0, keepdims=True)
        idx = jnp.min(jnp.where(best == top, bidx, S))
        idx = jnp.where(idx >= S, 0, idx)
        g, u = idx // (T * GS), idx // T % GS
        tile = pl.multiple_of(idx % T // 8 * 8, 8)
        rows = pl.ds(tile, 8)
        x1, xn = xmid[0, g, u, rows], xmid[1, g, u, rows]
        gate = _rb(_dot(xn, wg_s[...]))
        up = _rb(_dot(xn, wu_s[...]))
        gate = _rb(gate * _rb(jax.nn.sigmoid(gate)))
        y = _rb(_dot(_rb(gate * up), wd_s[...]))
        y = _rb(y * _rb(jax.nn.sigmoid(router(xn))))
        sel = lax.broadcasted_iota(I32, (8, D), 0) == idx % 8
        x2 = (x1 + _rb(xn + jnp.where(sel, y, 0.0))).astype(BF)

        @pl.when(last)
        def _():
            cp_out(0, NG - 4, 0).wait()
            cp_out(NG - 4, NG, 1).wait()
            xbuf[g, u, rows] = x2
            cp = pltpu.make_async_copy(xbuf.at[g, u], out_hbm.at[g, u], sems.at[0])
            cp.start()
            cp.wait()

        @pl.when(jnp.logical_not(last))
        def _():
            xbuf[g, u, rows] = x2
            h = normed(x2)
            hbuf[g, u, rows] = h
            build_lhs(1, phases[0])
            reset_state()

            @pl.when(g == 0)
            def _():
                ph = phases[0]
                left = {(w, n): _operand(LHS, *ph.pair(w, n), lambda s, k: h[:, k * E:k * E + E], ph.row)
                        for n in ph.ns for w in ph.ws}

                def redo(blk, carry):
                    def product(w, n):
                        return {None: _dot(left[w, n], pltpu.bitcast(wqkv[blk, ph.index(w, n)], BF))}

                    def emit(i, j, t, v):
                        qkv[0, blk, pl.ds(pl.multiple_of((4 * u + j) * T + tile, 8), 8)] = v
                    list(ph.run(product, emit, True))
                    return carry
                lax.fori_loop(0, 3 * NQ, redo, 0, unroll=4)

    def iteration(it, carry):
        last = it == NG - 1

        @pl.when(it == 1)
        def _():
            cp_x(XG, NG, 1).wait()
            for c in cp_b:
                c.wait()

        @pl.when(last)
        def _():
            cp_out(0, NG - 4, 0).start()
        group_pair(2 * it)
        pl.when(it % (NG // 2) == NG // 2 - 1)(lambda: finish_layer(last))
        return carry

    lax.fori_loop(0, NG, iteration, 0)


@functools.partial(jax.jit, static_argnames=("A_seg_len",))
def pallas_interleave_layers__memory_aug_recurrent_mem_tr__moe_arch_mod__prompt_kernel(
    A_x, A_mem0, A_Wq, A_Wk, A_Wv, A_Wo, A_seg_len, B_x, B_w_r, B_w_gate, B_w_up, B_w_down,
):
    del B_x
    B, S, D = A_x.shape
    _, H, E = A_Wq.shape
    M = A_mem0.shape[1]
    F = B_w_gate.shape[1]
    T = int(A_seg_len)
    assert (B, S, D, H, E, M, T) == (1, 2048, 512, 32, 128, 8, 32)
    NG = S // (T * GS)
    NHG = H // 8
    hbm = pl.BlockSpec(memory_space=pl.ANY)
    vmem = pl.BlockSpec(memory_space=pltpu.VMEM)
    out = pl.pallas_call(
        functools.partial(_kernel, S=S, D=D, H=H, E=E, M=M, T=T),
        out_shape=jax.ShapeDtypeStruct((NG, GS, T, D), A_x.dtype),
        in_specs=[hbm, vmem, hbm, hbm, hbm, hbm, vmem, hbm, hbm, hbm],
        out_specs=hbm,
        scratch_shapes=[
            pltpu.VMEM((3 * NHG, D, 8, E), BF),
            pltpu.VMEM((NHG, 8, E, D), BF),
            pltpu.VMEM((3 * H // 4, 49, E // 2, E), U32),
            pltpu.VMEM((49, H // 4 * E // 2, E), U32),
            pltpu.VMEM((NG + 1, GS, T, D), BF),
            pltpu.VMEM((2, NG + 1, GS, T, D), F32),
            pltpu.VMEM((NG, GS, T, D), F32),
            pltpu.VMEM((51, T, E), F32),
            pltpu.VMEM((2, 3 * H // 4, GS * 4 * T, E), F32),
            pltpu.VMEM((2, GS, 4, T, H // 4 * E), F32),
            pltpu.VMEM((2, GS, T, D), F32),
            pltpu.VMEM((M + 8, D), F32),
            pltpu.VMEM((8, 512), I32),
            pltpu.VMEM((D, F), BF),
            pltpu.VMEM((D, F), BF),
            pltpu.VMEM((F, D), BF),
            pltpu.SemaphoreType.DMA((4 * NHG + 5,)),
        ],
        compiler_params=pltpu.CompilerParams(vmem_limit_bytes=120 * 2**20),
        name="rmt_mod",
    )(
        A_x.reshape(NG, GS, T, D), A_mem0.reshape(M, D),
        A_Wq.reshape(D, NHG, 8, E), A_Wk.reshape(D, NHG, 8, E), A_Wv.reshape(D, NHG, 8, E),
        A_Wo.reshape(NHG, 8, E, D),
        B_w_r, B_w_gate, B_w_up, B_w_down,
    )
    return out.reshape(B, S, D)
```

```python
import functools

import numpy as np
import jax
import jax.numpy as jnp
from jax import lax
import jax.experimental.pallas as pl
import jax.experimental.pallas.tpu as pltpu

BF = jnp.bfloat16
F32 = jnp.float32
U32 = jnp.uint32
I32 = jnp.int32

GS = 4

LHS = {1: ((0, 0, 1), (1, 1, 1)), 2: ((1, 0, 1), (1, 1, 1)), 3: ((0, 0, 1),), 4: ((1, 1, 1),),
       5: ((0, 0, 1), (0, 1, 1)), 6: ((1, 0, 1), (0, 0, -1)), 7: ((0, 1, 1), (1, 1, -1))}
RHS = {1: ((0, 0, 1), (1, 1, 1)), 2: ((0, 0, 1),), 3: ((0, 1, 1), (1, 1, -1)), 4: ((1, 0, 1), (0, 0, -1)),
       5: ((1, 1, 1),), 6: ((0, 0, 1), (0, 1, 1)), 7: ((1, 0, 1), (1, 1, 1))}
OUT = {(0, 0): ((4, 1), (7, 1), (1, 1), (5, -1)), (0, 1): ((3, 1), (5, 1)),
       (1, 0): ((2, 1), (4, 1)), (1, 1): ((3, 1), (6, 1), (1, 1), (2, -1))}
BASIS = ((3, 1, 5, 7), (4, 1, 2, 6))
PHASES = ((1, 1, 0), (1, 0, 1), (0, 0, 0), (0, 1, 1))

SEQ_FULL = (
    "xx....A............q......q........p......q......p......q......p......EqEEE......p......q.....p.......q......p....q..oooooopooooopoooooooHoooooooooooooo",
    "x........A........q........q......p......q.....p.......q......p......EEqEE..p..........q.....p.......q......p......qoooooopooooopoooHoooooooooooooooooo",
    "xx........A.........q.......q.......p.........q...p.....qEEEE.........q.p.....p.........q......p......q......p......qooooopooooopooooHoooooooooooooooooo",
    "x........A........q........q......p......q......p......q....p........qEE..p...E..E.....q....p........q......p......qoooooopooooopoooHoooooooooooooooooo",
)


def _rb(v):
    return v.astype(BF).astype(F32)


def _layernorm(x):
    inv_n = 1.0 / x.shape[-1]
    m = jnp.sum(x, axis=-1, keepdims=True) * inv_n
    d = x - m
    v = _rb(jnp.sum(d * d, axis=-1, keepdims=True) * inv_n)
    den = _rb(jnp.sqrt(_rb(v + 1.0013580322265625e-05)))
    return _rb(_rb(x - _rb(m)) * (1.0 / den))


def _dot(a, b):
    return jnp.dot(a, b, preferred_element_type=F32)


def _signed_sum(terms):
    terms = sorted(terms, key=lambda t: -t[1])
    total = terms[0][0] if terms[0][1] > 0 else -terms[0][0]
    for v, sign in terms[1:]:
        total = total + v if sign > 0 else total - v
    return total


def _left_operand(a, b, block, rows=None):
    return _signed_sum([(block(2 * i + k, 2 * j + l), s * t) for i, j, s in LHS[a] for k, l, t in LHS[b]
                        if rows is None or 2 * i + k == rows])


def _output(pos, prods):
    terms = [(prods[m], s) for m, s in OUT[pos] if prods.get(m) is not None]
    return _signed_sum(terms) if terms else None


def _weight_operands(block):
    vals = []
    for a in RHS:
        outer = {(k, l): _signed_sum([(block(2 * i + k, 2 * j + l), s) for i, j, s in RHS[a]])
                 for k in range(2) for l in range(2)}
        for b in RHS:
            vals.append(_signed_sum([(outer[k, l], t) for k, l, t in RHS[b]]))
            if len(vals) == 2 or a == b == 7:
                w = pltpu.bitcast(jnp.concatenate(vals, axis=1).astype(BF), U32)
                yield from (w[:, c:c + 128] for c in range(0, w.shape[1], 128))
                vals = []


class _Phase:
    def __init__(self, u):
        h0, h1, self.wide = PHASES[u]
        self.u, self.row = u, 2 * h0 + h1
        self.ws, self.ns = (BASIS[h] for h in ((h0, h1) if self.wide == 0 else (h1, h0)))

    def pair(self, w, n):
        return (w, n) if self.wide == 0 else (n, w)

    def index(self, w, n):
        a, b = self.pair(w, n)
        return 7 * (a - 1) + b - 1

    def place(self, pw, pn):
        (i, j), (k, l) = self.pair(pw, pn)
        return 2 * i + k, 2 * j + l

    def touched(self):
        return {self.place(pw, pn) for pw in OUT for pn in OUT
                if any(m in self.ws for m, _ in OUT[pw] if m != 1) and any(m in self.ns for m, _ in OUT[pn] if m != 1)}

    def run(self, product, emit, wide_first, order=None):
        first, second = (self.ws, self.ns) if wide_first else (self.ns, self.ws)
        second = order or second
        partial = {}
        for m2 in second:
            got = {}
            for m1 in first:
                for t, v in product(*((m1, m2) if wide_first else (m2, m1))).items():
                    got.setdefault(t, {})[m1] = v
                if m1 != first[-1]:
                    yield
            for t, prods in got.items():
                for p1 in OUT:
                    partial.setdefault((t, p1), {})[m2] = _output(p1, prods)
            for p2, terms in OUT.items():
                need = [m for m in second if m in dict(terms)]
                if need and need[-1] == m2:
                    for (t, p1), prods in partial.items():
                        i, j = self.place(*((p1, p2) if wide_first else (p2, p1)))
                        if (i == self.row) if t is None else ((i, j) in self.touched()):
                            emit(i, j, t, _output(p2, prods))
            yield


def _kernel(x_hbm, mem0_ref, wq_hbm, wk_hbm, wv_hbm, wo_hbm, wr_ref, wg_hbm, wu_hbm, wd_hbm,
            out_hbm,
            raw, wo_raw, wqkv, wout, xbuf, xmid, hbuf, hl, qkv, obuf, oacc, state, bidx_ref,
            wg_s, wu_s, wd_s, sems,
            *, S, D, H, E, M, T):
    NG = S // (T * GS)
    L = M + T
    NQ = H // 4
    NHG = H // 8
    NC = 3 * NHG
    w_hbm = (wq_hbm, wk_hbm, wv_hbm)
    phases = [_Phase(u) for u in range(GS)]

    def cp_w(c):
        return pltpu.make_async_copy(w_hbm[c // NHG].at[:, c % NHG], raw.at[c], sems.at[c])

    def cp_o(k):
        return pltpu.make_async_copy(wo_hbm.at[k], wo_raw.at[k], sems.at[NC + k])

    cp_x = [pltpu.make_async_copy(x_hbm.at[pl.ds(lo, hi - lo)], xbuf.at[pl.ds(lo, hi - lo)], sems.at[NC + NHG + k])
            for k, (lo, hi) in enumerate(((0, 3), (3, 5), (5, NG)))]
    cp_out = [pltpu.make_async_copy(xbuf.at[pl.ds(lo, hi - lo)], out_hbm.at[pl.ds(lo, hi - lo)], sems.at[NC + NHG + k])
              for k, (lo, hi) in enumerate(((0, NG - 4), (NG - 4, NG)))]
    cp_b = [pltpu.make_async_copy(w, s, sems.at[NC + NHG + 3 + j])
            for j, (w, s) in enumerate(((wg_hbm, wg_s), (wu_hbm, wu_s), (wd_hbm, wd_s)))]

    def normed(x):
        x = x.astype(F32)
        d = x - jnp.sum(x, axis=-1, keepdims=True) * (1.0 / D)
        return d * lax.rsqrt(jnp.sum(d * d, axis=-1, keepdims=True) * (1.0 / D) + 1e-5)

    def prenorm(g, u):
        hbuf[g, u] = normed(xbuf[g, u])

    def rows_of(tiles):
        return pl.ds(tiles[0] * 8, len(tiles) * 8)

    def build_lhs(g, ph):
        for n in ph.ns:
            for w in ph.ws:
                if n != 1 or (w, ph.u) == (1, 0):
                    hl[ph.index(w, n)] = _left_operand(*ph.pair(w, n), lambda s, k: hbuf[g, s, :, pl.ds(k * E, E)])

    def accumulate(ref, ph, i, j, index, v):
        seen = any((i, j) in p.touched() for p in phases[:ph.u])
        ref[index] = v + ref[index] if seen else v

    def split(res, tiles, mem_first, with_mem):
        off = M if with_mem and mem_first else 0
        out = {t: res[off + 8 * n:off + 8 * n + 8] for n, t in enumerate(tiles)}
        if with_mem:
            out[None] = res[:M] if mem_first else res[-M:]
        return out

    def first_product(blk):
        return _dot(hl[0], pltpu.bitcast(wqkv[blk, 0], BF))

    def qkv_block(ph, par, blk, mem_lhs, mem_out, first):
        def product(w, n):
            tiles = range(4 * (n != 1))
            left = [hl[ph.index(w, n)]] if tiles else []
            left += [mem_lhs[w, n]] if mem_lhs else []
            out = split(first, range(4), False, False) if (w, n) == (1, 1) and first is not None else {}
            if left:
                res = _dot(jnp.concatenate(left, axis=0), pltpu.bitcast(wqkv[blk, ph.index(w, n)], BF))
                out.update(split(res, tiles, False, mem_lhs))
            return out

        def emit(i, j, t, v):
            if t is None:
                mem_out[j] = v
            else:
                accumulate(qkv, ph, i, j, (par, blk, pl.ds((4 * i + j) * T + t * 8, 8)), v)
        return ph.run(product, emit, True)

    def out_rounds(ph, par, mem_in, mem_out):
        def tiles_of(w, n):
            if (w, n) == (1, 1):
                return range(ph.u, ph.u + 1) if mem_in else range(4 * (ph.u == 0))
            return range(4 * (n != 1))

        def half(w, n, k):
            tiles = tiles_of(w, n)
            left = [_left_operand(*ph.pair(w, n), lambda s, j: mem_in(j, k), ph.row)] if mem_in else []
            if tiles:
                left += [_left_operand(*ph.pair(w, n),
                                  lambda s, j: obuf[par, s, j, rows_of(tiles), pl.ds(k * 4 * E, 4 * E)])]
            if left:
                return _dot(jnp.concatenate(left, axis=0),
                            pltpu.bitcast(wout[ph.index(w, n), pl.ds(k * 2 * E, 2 * E)], BF))

        def product(w, n):
            res = half(w, n, 1)
            return {} if res is None else split(res + early[w, n], tiles_of(w, n), True, mem_in)

        def emit(i, j, t, v):
            if t is None:
                mem_out[j] = v
            else:
                accumulate(oacc, ph, i, j, (par, i, pl.ds(t * 8, 8), pl.ds(j * E, E)), v)
        early = {}
        for w in ph.ws[::-1]:
            for n in ph.ns:
                early[w, n] = half(w, n, 0)
                yield
        yield from ph.run(product, emit, False, ph.ws[::-1])

    cp_w(0).start()
    cp_x[0].start()
    for c in range(1, NC):
        cp_w(c).start()
    for k in range(NHG):
        cp_o(k).start()
    for c in cp_x[1:] + cp_b:
        c.start()
    xbuf[NG] = jnp.zeros((GS, T, D), BF)
    oacc[0] = jnp.zeros(oacc.shape[1:], F32)
    obuf[1] = jnp.zeros(obuf.shape[1:], F32)

    def prep_qkv(c):
        for r in range(E // 16):
            for k in range(4):
                words = pltpu.bitcast(raw[c, pl.ds(k * E + r * 16, 16)].reshape(128, E), U32)
                qkv[1, r, pl.ds(k * 64, 64)] = pltpu.bitcast(words, F32)
        for r in range(E // 16):
            for n in range(2):
                def block(k, j):
                    w = pltpu.bitcast(qkv[1, r, pl.ds(k * 64 + 2 * n + j // 2, 16, stride=4), :], U32)
                    return pltpu.bitcast(w & np.uint32(0xFFFF0000) if j % 2 else w << 16, F32)
                for m, w in enumerate(_weight_operands(block)):
                    wqkv[2 * c + n, m, pl.ds(r * 8, 8)] = w

    def stream(c, carry):
        pltpu.make_async_copy(raw.at[c], raw.at[c], sems.at[c]).wait()
        prep_qkv(c)

        @pl.when(c == 0)
        def _():
            cp_x[0].wait()
            hbuf[:3] = normed(xbuf[:3].reshape(3 * GS * T, D)).reshape(3, GS, T, D)
            for ph in phases:
                build_lhs(0, ph)

        @pl.when(c % 2 == 1)
        def _():
            blocks = [2 * c - 2 + n for n in range(4)]
            firsts = [first_product(blk) for blk in blocks]
            for ph in phases:
                for blk, first in zip(blocks, firsts):
                    list(qkv_block(ph, 0, blk, None, None, None if ph.u else first))
        return carry
    lax.fori_loop(0, NC, stream, 0)
    build_lhs(1, phases[0])

    def stream_o(k, carry):
        cp_o(k).wait()
        for r in range(E // 16):
            for n in range(2):
                heads = [wo_raw[k, 4 * n + i, pl.ds(r * 16, 16)].astype(F32) for i in range(4)]
                for m, w in enumerate(_weight_operands(lambda i, j: heads[i][:, j * E:j * E + E])):
                    wout[m, pl.ds(pl.multiple_of((2 * k + n) * (E // 2) + r * 8, 8), 8)] = w
        return carry
    lax.fori_loop(0, NHG, stream_o, 0)
    cp_x[1].wait()

    def reset_state():
        state[:M] = mem0_ref[...].astype(F32)
        state[M:] = jnp.full((8, D), -jnp.inf, F32)
        bidx_ref[:, :128] = jnp.full((8, 128), S, I32)
    reset_state()

    def router(xn):
        return _rb(jnp.sum(xn * wr_ref[...].astype(F32).reshape(1, D), axis=-1, keepdims=True))

    def epilogue(g, u, t, par, best, bidx):
        rows = pl.ds(t * 8, 8)
        x1 = _rb(xbuf[g, u, rows].astype(F32) + _rb(oacc[par, u, rows]))
        xn = _layernorm(x1)
        xmid[0, g, u, rows] = x1
        xmid[1, g, u, rows] = xn
        xbuf[g, u, rows] = (x1 + xn).astype(BF)
        it = lax.broadcasted_iota(I32, (8, 128), 0) + ((g * GS + u) * T + t * 8)
        r = jnp.where(it < S, jnp.broadcast_to(router(xn), (8, 128)), -jnp.inf)
        better = r > best
        return jnp.where(better, r, best), jnp.where(better, it, bidx)

    def segment(par, ph, mem, seq, jobs, firsts, first_rounds):
        u = ph.u
        row = lax.broadcasted_iota(I32, (L, L), 0)
        col = lax.broadcasted_iota(I32, (L, L), 1)
        mask = (row < M) | (row >= col)
        mem_lhs = {(w, n): _left_operand(*ph.pair(w, n), lambda s, k: mem[k], ph.row) for n in ph.ns for w in ph.ws}
        proj = [{} for _ in range(3 * NQ)]
        probs, outs, new_mem = {}, {}, {}

        def head(j, n, i):
            return jnp.concatenate([proj[j * NQ + n][i], qkv[par, j * NQ + n, pl.ds((4 * u + i) * T, T)]], axis=0)

        def scores(n):
            for i in range(4):
                sc = lax.dot_general(head(0, n, i), head(1, n, i).astype(BF), (((1,), (1,)), ((), ())),
                                     preferred_element_type=F32)
                sc = jnp.where(mask, sc, -1e9 * E ** 0.5)
                e = jnp.exp2((sc - jnp.max(sc, axis=-1, keepdims=True)) * (E ** -0.5 * 1.4426950408889634))
                probs[n, i] = e * pltpu.reciprocal(jnp.sum(e, axis=-1, keepdims=True), full_range=False)

        def values(n):
            for i in range(4):
                o = _dot(probs[n, i], head(2, n, i).astype(BF))
                outs[n, i] = o[:M]
                obuf[par, u, i, :, pl.ds(n * E, E)] = o[M:]

        def rounds():
            order = [(j, n - (j == 2)) for n in range(NQ + 1) for j in range(3) if 0 <= n - (j == 2) < NQ]
            for blk in (j * NQ + n for j, n in order):
                for k, _ in enumerate(qkv_block(ph, 1 - par, blk, mem_lhs, proj[blk], firsts.pop(blk, None))):
                    if k % 4 == 3:
                        yield

        def mem_in(i, k):
            return jnp.concatenate([outs[n, i] for n in range(4 * k, 4 * k + 4)], axis=1)
        its = {".": rounds(), "o": out_rounds(ph, 1 - par, mem_in, new_mem),
               "q": map(scores, range(NQ)), "p": map(values, range(NQ))}
        its.update({ch: (f() for f in fs) for ch, fs in jobs.items()})
        assert "x" not in seq.lstrip("x")
        for ch in seq:
            next(first_rounds if ch == "x" else its[ch])
        assert not any(list(it) for it in its.values())
        return [_rb(new_mem[j]) for j in range(4)]

    def group_pair(G0):
        mem, top = [state[:M, pl.ds(j * E, E)] for j in range(4)], [state[M:, :128], bidx_ref[:, :128]]
        for par in range(2):
            G = G0 + par
            g = G % NG

            def post(u, t):
                top[:] = epilogue(jnp.where(g >= 2, g - 2, NG), u, t, par, *top)
                hl[49 + G0 // NG, :8] = top[0]

            firsts = {}
            first_rounds = (firsts.update({blk: first_product(blk) for blk in range(k, k + 4)})
                            for k in range(0, 3 * NQ, 4))
            for u in range(GS):
                mem = segment(par, phases[u], mem, SEQ_FULL[(par * GS + u) % len(SEQ_FULL)], {
                    "H": [functools.partial(prenorm, (G + 3) % NG, u)],
                    "A": [functools.partial(build_lhs, (G + 1 + (u + 1) // GS) % NG, phases[(u + 1) % GS])],
                    "E": [functools.partial(post, u, t) for t in range(T // 8)]}, firsts, first_rounds)
            assert not firsts and not list(first_rounds)
        for j in range(4):
            state[:M, pl.ds(j * E, E)] = mem[j]
        state[M:, :128], bidx_ref[:, :128] = top

    def finish_layer(it):
        last = it == NG - 1
        best, bidx = state[M:, :128], bidx_ref[:, :128]
        for ph in phases:
            list(out_rounds(ph, 1, None, None))
        for par in range(2):
            for u in range(GS):
                for t in range(T // 8):
                    best, bidx = epilogue(NG - 2 + par, u, t, par, best, bidx)

        @pl.when(last)
        def _():
            cp_out[1].start()

        top = jnp.max(best, axis=0, keepdims=True)
        idx = jnp.min(jnp.where(best == top, bidx, S))
        idx = jnp.where(idx >= S, 0, idx)
        g, u = idx // (T * GS), idx // T % GS
        tile = pl.multiple_of(idx % T // 8 * 8, 8)
        rows = pl.ds(tile, 8)
        x1, xn = xmid[0, g, u, rows], xmid[1, g, u, rows]
        gate = _rb(_dot(xn, wg_s[...]))
        up = _rb(_dot(xn, wu_s[...]))
        gate = _rb(gate * _rb(jax.nn.sigmoid(gate)))
        y = _rb(_dot(_rb(gate * up), wd_s[...]))
        y = _rb(y * _rb(jax.nn.sigmoid(router(xn))))
        sel = lax.broadcasted_iota(I32, (8, D), 0) == idx % 8
        x2 = (x1 + _rb(xn + jnp.where(sel, y, 0.0))).astype(BF)

        @pl.when(last)
        def _():
            cp_out[0].wait()
            cp_out[1].wait()
            xbuf[g, u, rows] = x2
            cp = pltpu.make_async_copy(xbuf.at[g, u], out_hbm.at[g, u], sems.at[0])
            cp.start()
            cp.wait()

        @pl.when(jnp.logical_not(last))
        def _():
            xbuf[g, u, rows] = x2
            h = normed(x2)
            hbuf[g, u, rows] = h
            build_lhs(1, phases[0])
            reset_state()

            @pl.when(g == 0)
            def _():
                ph = phases[0]
                left = {(w, n): _left_operand(*ph.pair(w, n), lambda s, k: h[:, k * E:k * E + E], ph.row)
                        for n in ph.ns for w in ph.ws}

                def redo(blk, carry):
                    def product(w, n):
                        return {None: _dot(left[w, n], pltpu.bitcast(wqkv[blk, ph.index(w, n)], BF))}

                    def emit(i, j, t, v):
                        qkv[0, blk, pl.ds(pl.multiple_of((4 * u + j) * T + tile, 8), 8)] = v
                    list(ph.run(product, emit, True))
                    return carry
                lax.fori_loop(0, 3 * NQ, redo, 0, unroll=4)

    def iteration(it, carry):
        last = it == NG - 1

        @pl.when(it == 1)
        def _():
            for c in cp_x[2:] + cp_b:
                c.wait()

        @pl.when(last)
        def _():
            cp_out[0].start()
        group_pair(2 * it)
        pl.when(it % (NG // 2) == NG // 2 - 1)(lambda: finish_layer(it))
        return carry

    lax.fori_loop(0, NG, iteration, 0)


@functools.partial(jax.jit, static_argnames=("A_seg_len",))
def pallas_interleave_layers__memory_aug_recurrent_mem_tr__moe_arch_mod__prompt_kernel(
    A_x, A_mem0, A_Wq, A_Wk, A_Wv, A_Wo, A_seg_len, B_x, B_w_r, B_w_gate, B_w_up, B_w_down,
):
    del B_x
    B, S, D = A_x.shape
    _, H, E = A_Wq.shape
    M = A_mem0.shape[1]
    F = B_w_gate.shape[1]
    T = int(A_seg_len)
    assert (B, S, D, H, E, M, T) == (1, 2048, 512, 32, 128, 8, 32)
    NG = S // (T * GS)
    NHG = H // 8
    hbm = pl.BlockSpec(memory_space=pl.ANY)
    vmem = pl.BlockSpec(memory_space=pltpu.VMEM)
    out = pl.pallas_call(
        functools.partial(_kernel, S=S, D=D, H=H, E=E, M=M, T=T),
        out_shape=jax.ShapeDtypeStruct((NG, GS, T, D), A_x.dtype),
        in_specs=[hbm, vmem, hbm, hbm, hbm, hbm, vmem, hbm, hbm, hbm],
        out_specs=hbm,
        scratch_shapes=[
            pltpu.VMEM((3 * NHG, D, 8, E), BF),
            pltpu.VMEM((NHG, 8, E, D), BF),
            pltpu.VMEM((3 * H // 4, 49, E // 2, E), U32),
            pltpu.VMEM((49, H // 4 * E // 2, E), U32),
            pltpu.VMEM((NG + 1, GS, T, D), BF),
            pltpu.VMEM((2, NG + 1, GS, T, D), F32),
            pltpu.VMEM((NG, GS, T, D), F32),
            pltpu.VMEM((51, T, E), F32),
            pltpu.VMEM((2, 3 * H // 4, GS * 4 * T, E), F32),
            pltpu.VMEM((2, GS, 4, T, H // 4 * E), F32),
            pltpu.VMEM((2, GS, T, D), F32),
            pltpu.VMEM((M + 8, D), F32),
            pltpu.VMEM((8, 512), I32),
            pltpu.VMEM((D, F), BF),
            pltpu.VMEM((D, F), BF),
            pltpu.VMEM((F, D), BF),
            pltpu.SemaphoreType.DMA((4 * NHG + 6,)),
        ],
        compiler_params=pltpu.CompilerParams(vmem_limit_bytes=120 * 2**20),
        name="rmt_mod",
    )(
        A_x.reshape(NG, GS, T, D), A_mem0.reshape(M, D),
        A_Wq.reshape(D, NHG, 8, E), A_Wk.reshape(D, NHG, 8, E), A_Wv.reshape(D, NHG, 8, E),
        A_Wo.reshape(NHG, 8, E, D),
        B_w_r, B_w_gate, B_w_up, B_w_down,
    )
    return out.reshape(B, S, D)
```

```python
import functools

import numpy as np
import jax
import jax.numpy as jnp
from jax import lax
import jax.experimental.pallas as pl
import jax.experimental.pallas.tpu as pltpu

BF = jnp.bfloat16
F32 = jnp.float32
U32 = jnp.uint32
I32 = jnp.int32

GS = 4

LHS = {1: ((0, 0, 1), (1, 1, 1)), 2: ((1, 0, 1), (1, 1, 1)), 3: ((0, 0, 1),), 4: ((1, 1, 1),),
       5: ((0, 0, 1), (0, 1, 1)), 6: ((1, 0, 1), (0, 0, -1)), 7: ((0, 1, 1), (1, 1, -1))}
RHS = {1: ((0, 0, 1), (1, 1, 1)), 2: ((0, 0, 1),), 3: ((0, 1, 1), (1, 1, -1)), 4: ((1, 0, 1), (0, 0, -1)),
       5: ((1, 1, 1),), 6: ((0, 0, 1), (0, 1, 1)), 7: ((1, 0, 1), (1, 1, 1))}
OUT = {(0, 0): ((4, 1), (7, 1), (1, 1), (5, -1)), (0, 1): ((3, 1), (5, 1)),
       (1, 0): ((2, 1), (4, 1)), (1, 1): ((3, 1), (6, 1), (1, 1), (2, -1))}
BASIS = ((3, 1, 5, 7), (4, 1, 2, 6))
PHASES = ((1, 1, 0), (1, 0, 1), (0, 0, 0), (0, 1, 1))

SEQ_FULL = (
    "xx....A............q......q........p......q......p......q......p......EqEEE......p......q.....p.......q......p....q..oooooopooooopoooooooHoooooooooooooo",
    "x........A........q........q......p......q.....p.......q......p......EEqEE..p..........q.....p.......q......p......qoooooopooooopoooHoooooooooooooooooo",
    "xx........A.........q.......q.......p.........q...p.....qEEEE.........q.p.....p.........q......p......q......p......qooooopooooopooooHoooooooooooooooooo",
    "x........A........q........q......p......q......p......q....p........qEE..p...E..E.....q....p........q......p......qoooooopooooopoooHoooooooooooooooooo",
)


def _rb(v):
    return v.astype(BF).astype(F32)


def _layernorm(x):
    inv_n = 1.0 / x.shape[-1]
    m = jnp.sum(x, axis=-1, keepdims=True) * inv_n
    d = x - m
    v = _rb(jnp.sum(d * d, axis=-1, keepdims=True) * inv_n)
    den = _rb(jnp.sqrt(_rb(v + 1.0013580322265625e-05)))
    return _rb(_rb(x - _rb(m)) * (1.0 / den))


def _dot(a, b):
    return jnp.dot(a, b, preferred_element_type=F32)


def _signed_sum(terms):
    terms = sorted(terms, key=lambda t: -t[1])
    total = terms[0][0] if terms[0][1] > 0 else -terms[0][0]
    for v, sign in terms[1:]:
        total = total + v if sign > 0 else total - v
    return total


def _left_operand(a, b, block, rows=None):
    return _signed_sum([(block(2 * i + k, 2 * j + l), s * t) for i, j, s in LHS[a] for k, l, t in LHS[b]
                        if rows is None or 2 * i + k == rows])


def _output(pos, prods):
    terms = [(prods[m], s) for m, s in OUT[pos] if prods.get(m) is not None]
    return _signed_sum(terms) if terms else None


def _weight_operands(block):
    vals = []
    for a in RHS:
        outer = {(k, l): _signed_sum([(block(2 * i + k, 2 * j + l), s) for i, j, s in RHS[a]])
                 for k in range(2) for l in range(2)}
        for b in RHS:
            vals.append(_signed_sum([(outer[k, l], t) for k, l, t in RHS[b]]))
            if len(vals) == 2 or a == b == 7:
                w = pltpu.bitcast(jnp.concatenate(vals, axis=1).astype(BF), U32)
                yield from (w[:, c:c + 128] for c in range(0, w.shape[1], 128))
                vals = []


class _Phase:
    def __init__(self, u):
        h0, h1, self.wide = PHASES[u]
        self.u, self.row = u, 2 * h0 + h1
        self.ws, self.ns = (BASIS[h] for h in ((h0, h1) if self.wide == 0 else (h1, h0)))

    def pair(self, w, n):
        return (w, n) if self.wide == 0 else (n, w)

    def index(self, w, n):
        a, b = self.pair(w, n)
        return 7 * (a - 1) + b - 1

    def place(self, pw, pn):
        (i, j), (k, l) = self.pair(pw, pn)
        return 2 * i + k, 2 * j + l

    def touched(self):
        return {self.place(pw, pn) for pw in OUT for pn in OUT
                if any(m in self.ws for m, _ in OUT[pw] if m != 1) and any(m in self.ns for m, _ in OUT[pn] if m != 1)}

    def run(self, product, emit, wide_first, order=None):
        first, second = (self.ws, self.ns) if wide_first else (self.ns, self.ws)
        second = order or second
        partial = {}
        for m2 in second:
            got = {}
            for m1 in first:
                for t, v in product(*((m1, m2) if wide_first else (m2, m1))).items():
                    got.setdefault(t, {})[m1] = v
                if m1 != first[-1]:
                    yield
            for t, prods in got.items():
                for p1 in OUT:
                    partial.setdefault((t, p1), {})[m2] = _output(p1, prods)
            for p2, terms in OUT.items():
                need = [m for m in second if m in dict(terms)]
                if need and need[-1] == m2:
                    for (t, p1), prods in partial.items():
                        i, j = self.place(*((p1, p2) if wide_first else (p2, p1)))
                        if (i == self.row) if t is None else ((i, j) in self.touched()):
                            emit(i, j, t, _output(p2, prods))
            yield


def _kernel(x_hbm, mem0_ref, wq_hbm, wk_hbm, wv_hbm, wo_hbm, wr_ref, wg_hbm, wu_hbm, wd_hbm,
            out_hbm,
            raw, wo_raw, wqkv, wout, xbuf, xmid, hbuf, hl, qkv, obuf, oacc, state, bidx_ref,
            wg_s, wu_s, wd_s, late, sems,
            *, S, D, H, E, M, T):
    NG = S // (T * GS)
    L = M + T
    NQ = H // 4
    NHG = H // 8
    NC = 3 * NHG
    w_hbm = (wq_hbm, wk_hbm, wv_hbm)
    phases = [_Phase(u) for u in range(GS)]

    def cp_w(c):
        return pltpu.make_async_copy(w_hbm[c // NHG].at[:, c % NHG], raw.at[c], sems.at[c])

    def cp_o(k):
        return pltpu.make_async_copy(wo_hbm.at[k], wo_raw.at[k], sems.at[NC + k])

    cp_x = [pltpu.make_async_copy(x_hbm.at[pl.ds(lo, hi - lo)], xbuf.at[pl.ds(lo, hi - lo)], sems.at[NC + NHG + k])
            for k, (lo, hi) in enumerate(((0, 3), (3, 5), (5, NG)))]
    cp_out = [pltpu.make_async_copy(xbuf.at[pl.ds(lo, hi - lo)], out_hbm.at[pl.ds(lo, hi - lo)], sems.at[NC + NHG + k])
              for k, (lo, hi) in enumerate(((0, NG - 4), (NG - 4, NG)))]
    cp_b = [pltpu.make_async_copy(w, s, sems.at[NC + NHG + 3 + j])
            for j, (w, s) in enumerate(((wg_hbm, wg_s), (wu_hbm, wu_s), (wd_hbm, wd_s)))]

    def normed(x):
        x = x.astype(F32)
        d = x - jnp.sum(x, axis=-1, keepdims=True) * (1.0 / D)
        return d * lax.rsqrt(jnp.sum(d * d, axis=-1, keepdims=True) * (1.0 / D) + 1e-5)

    def prenorm(g, u):
        hbuf[g, u] = normed(xbuf[g, u])

    def rows_of(tiles):
        return pl.ds(tiles[0] * 8, len(tiles) * 8)

    def build_lhs(g, ph):
        for n in ph.ns:
            for w in ph.ws:
                if n != 1 or (w, ph.u) == (1, 0):
                    hl[ph.index(w, n)] = _left_operand(*ph.pair(w, n), lambda s, k: hbuf[g, s, :, pl.ds(k * E, E)])

    def accumulate(ref, ph, i, j, index, v):
        seen = any((i, j) in p.touched() for p in phases[:ph.u])
        ref[index] = v + ref[index] if seen else v

    def split(res, tiles, mem_first, with_mem):
        off = M if with_mem and mem_first else 0
        out = {t: res[off + 8 * n:off + 8 * n + 8] for n, t in enumerate(tiles)}
        if with_mem:
            out[None] = res[:M] if mem_first else res[-M:]
        return out

    def first_product(blk):
        return _dot(hl[0], pltpu.bitcast(wqkv[blk, 0], BF))

    def qkv_block(ph, par, blk, mem_lhs, mem_out, first):
        def product(w, n):
            tiles = range(4 * (n != 1))
            left = [hl[ph.index(w, n)]] if tiles else []
            left += [mem_lhs[w, n]] if mem_lhs else []
            out = split(first, range(4), False, False) if (w, n) == (1, 1) and first is not None else {}
            if left:
                res = _dot(jnp.concatenate(left, axis=0), pltpu.bitcast(wqkv[blk, ph.index(w, n)], BF))
                out.update(split(res, tiles, False, mem_lhs))
            return out

        def emit(i, j, t, v):
            if t is None:
                mem_out[j] = v
            else:
                accumulate(qkv, ph, i, j, (par, blk, pl.ds((4 * i + j) * T + t * 8, 8)), v)
        return ph.run(product, emit, True)

    def out_rounds(ph, par, mem_in, mem_out):
        def tiles_of(w, n):
            if (w, n) == (1, 1):
                return range(ph.u, ph.u + 1) if mem_in else range(4 * (ph.u == 0))
            return range(4 * (n != 1))

        def half(w, n, k):
            tiles = tiles_of(w, n)
            left = [_left_operand(*ph.pair(w, n), lambda s, j: mem_in(j, k), ph.row)] if mem_in else []
            if tiles:
                left += [_left_operand(*ph.pair(w, n),
                                  lambda s, j: obuf[par, s, j, rows_of(tiles), pl.ds(k * 4 * E, 4 * E)])]
            if left:
                return _dot(jnp.concatenate(left, axis=0),
                            pltpu.bitcast(wout[ph.index(w, n), pl.ds(k * 2 * E, 2 * E)], BF))

        def product(w, n):
            res = half(w, n, 1)
            return {} if res is None else split(res + early[w, n], tiles_of(w, n), True, mem_in)

        def emit(i, j, t, v):
            if t is None:
                mem_out[j] = v
            else:
                accumulate(oacc, ph, i, j, (par, i, pl.ds(t * 8, 8), pl.ds(j * E, E)), v)
        early = {}
        for w in ph.ws[::-1]:
            for n in ph.ns:
                early[w, n] = half(w, n, 0)
                yield
        yield from ph.run(product, emit, False, ph.ws[::-1])

    cp_w(0).start()
    cp_x[0].start()
    for c in range(1, NC):
        cp_w(c).start()
    for k in range(NHG):
        cp_o(k).start()
    for c in cp_x[1:] + cp_b:
        c.start()
    xbuf[NG] = jnp.zeros((GS, T, D), BF)
    oacc[0] = jnp.zeros(oacc.shape[1:], F32)
    obuf[1] = jnp.zeros(obuf.shape[1:], F32)

    def prep_qkv(c):
        for r in range(E // 16):
            for k in range(4):
                words = pltpu.bitcast(raw[c, pl.ds(k * E + r * 16, 16)].reshape(128, E), U32)
                qkv[1, r, pl.ds(k * 64, 64)] = pltpu.bitcast(words, F32)
        for r in range(E // 16):
            for n in range(2):
                def block(k, j):
                    w = pltpu.bitcast(qkv[1, r, pl.ds(k * 64 + 2 * n + j // 2, 16, stride=4), :], U32)
                    return pltpu.bitcast(w & np.uint32(0xFFFF0000) if j % 2 else w << 16, F32)
                for m, w in enumerate(_weight_operands(block)):
                    wqkv[2 * c + n, m, pl.ds(r * 8, 8)] = w

    def stream(c, carry):
        pltpu.make_async_copy(raw.at[c], raw.at[c], sems.at[c]).wait()
        prep_qkv(c)

        @pl.when(c == 0)
        def _():
            cp_x[0].wait()
            hbuf[:3] = normed(xbuf[:3].reshape(3 * GS * T, D)).reshape(3, GS, T, D)
            for ph in phases:
                build_lhs(0, ph)

        @pl.when(c % 2 == 1)
        def _():
            blocks = [2 * c - 2 + n for n in range(4)]
            firsts = [first_product(blk) for blk in blocks]
            for ph in phases:
                for blk, first in zip(blocks, firsts):
                    list(qkv_block(ph, 0, blk, None, None, None if ph.u else first))
        return carry
    lax.fori_loop(0, NC, stream, 0)
    build_lhs(1, phases[0])

    def stream_o(k, carry):
        cp_o(k).wait()
        for r in range(E // 16):
            for n in range(2):
                heads = [wo_raw[k, 4 * n + i, pl.ds(r * 16, 16)].astype(F32) for i in range(4)]
                for m, w in enumerate(_weight_operands(lambda i, j: heads[i][:, j * E:j * E + E])):
                    wout[m, pl.ds(pl.multiple_of((2 * k + n) * (E // 2) + r * 8, 8), 8)] = w
        return carry
    lax.fori_loop(0, NHG, stream_o, 0)
    cp_x[1].wait()

    def reset_memory():
        state[:M] = mem0_ref[...].astype(F32)

    def reset_router():
        state[M:] = jnp.full((8, D), -jnp.inf, F32)
        bidx_ref[:, :128] = jnp.full((8, 128), S, I32)
    reset_memory()
    reset_router()

    def router(xn):
        return _rb(jnp.sum(xn * wr_ref[...].astype(F32).reshape(1, D), axis=-1, keepdims=True))

    def epilogue(g, u, t, par, best, bidx):
        rows = pl.ds(t * 8, 8)
        x1 = _rb(xbuf[g, u, rows].astype(F32) + _rb(oacc[par, u, rows]))
        xn = _layernorm(x1)
        xmid[0, g, u, rows] = x1
        xmid[1, g, u, rows] = xn
        xbuf[g, u, rows] = (x1 + xn).astype(BF)
        it = lax.broadcasted_iota(I32, (8, 128), 0) + ((g * GS + u) * T + t * 8)
        r = jnp.where(it < S, jnp.broadcast_to(router(xn), (8, 128)), -jnp.inf)
        better = r > best
        return jnp.where(better, r, best), jnp.where(better, it, bidx)

    def segment(par, ph, mem, seq, jobs, firsts, first_rounds):
        u = ph.u
        row = lax.broadcasted_iota(I32, (L, L), 0)
        col = lax.broadcasted_iota(I32, (L, L), 1)
        mask = (row < M) | (row >= col)
        mem_lhs = {(w, n): _left_operand(*ph.pair(w, n), lambda s, k: mem[k], ph.row) for n in ph.ns for w in ph.ws}
        proj = [{} for _ in range(3 * NQ)]
        probs, outs, new_mem = {}, {}, {}

        def head(j, n, i):
            return jnp.concatenate([proj[j * NQ + n][i], qkv[par, j * NQ + n, pl.ds((4 * u + i) * T, T)]], axis=0)

        def scores(n):
            for i in range(4):
                sc = lax.dot_general(head(0, n, i), head(1, n, i).astype(BF), (((1,), (1,)), ((), ())),
                                     preferred_element_type=F32)
                sc = jnp.where(mask, sc, -1e9 * E ** 0.5)
                e = jnp.exp2((sc - jnp.max(sc, axis=-1, keepdims=True)) * (E ** -0.5 * 1.4426950408889634))
                probs[n, i] = e * pltpu.reciprocal(jnp.sum(e, axis=-1, keepdims=True), full_range=False)

        def values(n):
            for i in range(4):
                o = _dot(probs[n, i], head(2, n, i).astype(BF))
                outs[n, i] = o[:M]
                obuf[par, u, i, :, pl.ds(n * E, E)] = o[M:]

        def rounds():
            order = [(j, n - (j == 2)) for n in range(NQ + 1) for j in range(3) if 0 <= n - (j == 2) < NQ]
            for blk in (j * NQ + n for j, n in order):
                for k, _ in enumerate(qkv_block(ph, 1 - par, blk, mem_lhs, proj[blk], firsts.pop(blk, None))):
                    if k % 4 == 3:
                        yield

        def mem_in(i, k):
            return jnp.concatenate([outs[n, i] for n in range(4 * k, 4 * k + 4)], axis=1)
        its = {".": rounds(), "o": out_rounds(ph, 1 - par, mem_in, new_mem),
               "q": map(scores, range(NQ)), "p": map(values, range(NQ))}
        its.update({ch: (f() for f in fs) for ch, fs in jobs.items()})
        assert "x" not in seq.lstrip("x")
        for ch in seq:
            next(first_rounds if ch == "x" else its[ch])
        assert not any(list(it) for it in its.values())
        return [_rb(new_mem[j]) for j in range(4)]

    def group_pair(G0, pending):
        mem, top = [state[:M, pl.ds(j * E, E)] for j in range(4)], [state[M:, :128], bidx_ref[:, :128]]
        for par in range(2):
            G = G0 + par
            g = G % NG

            def post(u, t):
                top[:] = epilogue(jnp.where(g >= 2, g - 2, jnp.where(pending, g + NG - 2, NG)), u, t, par, *top)
                hl[49 + G0 // NG, :8] = top[0]

            firsts = {}
            first_rounds = (firsts.update({blk: first_product(blk) for blk in range(k, k + 4)})
                            for k in range(0, 3 * NQ, 4))
            for u in range(GS):
                mem = segment(par, phases[u], mem, SEQ_FULL[(par * GS + u) % len(SEQ_FULL)], {
                    "H": [functools.partial(prenorm, (G + 3) % NG, u)],
                    "A": [functools.partial(build_lhs, (G + 1 + (u + 1) // GS) % NG, phases[(u + 1) % GS])],
                    "E": [functools.partial(post, u, t) for t in range(T // 8)]}, firsts, first_rounds)
            assert not firsts and not list(first_rounds)
        for j in range(4):
            state[:M, pl.ds(j * E, E)] = mem[j]
        state[M:, :128], bidx_ref[:, :128] = top

    def drain():
        best, bidx = state[M:, :128], bidx_ref[:, :128]
        for ph in phases:
            list(out_rounds(ph, 1, None, None))
        for par in range(2):
            for u in range(GS):
                for t in range(T // 8):
                    best, bidx = epilogue(NG - 2 + par, u, t, par, best, bidx)
        state[M:, :128], bidx_ref[:, :128] = best, bidx

    def top_token():
        best = state[M:, :128]
        idx = jnp.min(jnp.where(best == jnp.max(best, axis=0, keepdims=True), bidx_ref[:, :128], S))
        return jnp.where(idx >= S, 0, idx)

    def expert(last, nxt):
        idx = top_token()
        g, u = idx // (T * GS), idx // T % GS
        tile = pl.multiple_of(idx % T // 8 * 8, 8)
        rows = pl.ds(tile, 8)
        x1, xn = xmid[0, g, u, rows], xmid[1, g, u, rows]
        gate = _rb(_dot(xn, wg_s[...]))
        up = _rb(_dot(xn, wu_s[...]))
        gate = _rb(gate * _rb(jax.nn.sigmoid(gate)))
        y = _rb(_dot(_rb(gate * up), wd_s[...]))
        y = _rb(y * _rb(jax.nn.sigmoid(router(xn))))
        sel = lax.broadcasted_iota(I32, (8, D), 0) == idx % 8
        x2 = (x1 + _rb(xn + jnp.where(sel, y, 0.0))).astype(BF)

        @pl.when(last)
        def _():
            cp_out[0].wait()
            cp_out[1].wait()
            xbuf[g, u, rows] = x2
            cp = pltpu.make_async_copy(xbuf.at[g, u], out_hbm.at[g, u], sems.at[0])
            cp.start()
            cp.wait()

        @pl.when(jnp.logical_not(last))
        def _():
            xbuf[g, u, rows] = x2
            h = normed(x2)
            hbuf[g, u, rows] = h
            build_lhs(nxt + 1, phases[0])
            reset_router()

            @pl.when(g == nxt)
            def _():
                ph = phases[0]
                left = {(w, n): _left_operand(*ph.pair(w, n), lambda s, k: h[:, k * E:k * E + E], ph.row)
                        for n in ph.ns for w in ph.ws}

                def redo(blk, carry):
                    def product(w, n):
                        return {None: _dot(left[w, n], pltpu.bitcast(wqkv[blk, ph.index(w, n)], BF))}

                    def emit(i, j, t, v):
                        qkv[0, blk, pl.ds(pl.multiple_of((4 * u + j) * T + tile, 8), 8)] = v
                    list(ph.run(product, emit, True))
                    return carry
                lax.fori_loop(0, 3 * NQ, redo, 0, unroll=4)

    def iteration(it, carry):
        last = it == NG - 1
        seam = it == NG // 2 - 1
        pending = late[0] == 1

        @pl.when(it == 1)
        def _():
            for c in cp_x[2:] + cp_b:
                c.wait()

        @pl.when(last)
        def _():
            cp_out[0].start()
        group_pair(2 * it, pending)
        late[0] = 0

        @pl.when(seam)
        def _():
            late[0] = (top_token() >= 2 * GS * T).astype(I32)
            reset_memory()
        now = last | (seam & (late[0] == 0))
        pl.when(now)(drain)

        @pl.when(last)
        def _():
            cp_out[1].start()
        pl.when(now | pending)(lambda: expert(last, jnp.where(pending, 2, 0)))
        return carry

    late[0] = 0
    lax.fori_loop(0, NG, iteration, 0)


@functools.partial(jax.jit, static_argnames=("A_seg_len",))
def pallas_interleave_layers__memory_aug_recurrent_mem_tr__moe_arch_mod__prompt_kernel(
    A_x, A_mem0, A_Wq, A_Wk, A_Wv, A_Wo, A_seg_len, B_x, B_w_r, B_w_gate, B_w_up, B_w_down,
):
    del B_x
    B, S, D = A_x.shape
    _, H, E = A_Wq.shape
    M = A_mem0.shape[1]
    F = B_w_gate.shape[1]
    T = int(A_seg_len)
    assert (B, S, D, H, E, M, T) == (1, 2048, 512, 32, 128, 8, 32)
    NG = S // (T * GS)
    NHG = H // 8
    hbm = pl.BlockSpec(memory_space=pl.ANY)
    vmem = pl.BlockSpec(memory_space=pltpu.VMEM)
    out = pl.pallas_call(
        functools.partial(_kernel, S=S, D=D, H=H, E=E, M=M, T=T),
        out_shape=jax.ShapeDtypeStruct((NG, GS, T, D), A_x.dtype),
        in_specs=[hbm, vmem, hbm, hbm, hbm, hbm, vmem, hbm, hbm, hbm],
        out_specs=hbm,
        scratch_shapes=[
            pltpu.VMEM((3 * NHG, D, 8, E), BF),
            pltpu.VMEM((NHG, 8, E, D), BF),
            pltpu.VMEM((3 * H // 4, 49, E // 2, E), U32),
            pltpu.VMEM((49, H // 4 * E // 2, E), U32),
            pltpu.VMEM((NG + 1, GS, T, D), BF),
            pltpu.VMEM((2, NG + 1, GS, T, D), F32),
            pltpu.VMEM((NG, GS, T, D), F32),
            pltpu.VMEM((51, T, E), F32),
            pltpu.VMEM((2, 3 * H // 4, GS * 4 * T, E), F32),
            pltpu.VMEM((2, GS, 4, T, H // 4 * E), F32),
            pltpu.VMEM((2, GS, T, D), F32),
            pltpu.VMEM((M + 8, D), F32),
            pltpu.VMEM((8, 512), I32),
            pltpu.VMEM((D, F), BF),
            pltpu.VMEM((D, F), BF),
            pltpu.VMEM((F, D), BF),
            pltpu.SMEM((1,), I32),
            pltpu.SemaphoreType.DMA((4 * NHG + 6,)),
        ],
        compiler_params=pltpu.CompilerParams(vmem_limit_bytes=120 * 2**20),
        name="rmt_mod",
    )(
        A_x.reshape(NG, GS, T, D), A_mem0.reshape(M, D),
        A_Wq.reshape(D, NHG, 8, E), A_Wk.reshape(D, NHG, 8, E), A_Wv.reshape(D, NHG, 8, E),
        A_Wo.reshape(NHG, 8, E, D),
        B_w_r, B_w_gate, B_w_up, B_w_down,
    )
    return out.reshape(B, S, D)
```

```python
import functools

import numpy as np
import jax
import jax.numpy as jnp
from jax import lax
import jax.experimental.pallas as pl
import jax.experimental.pallas.tpu as pltpu

BF = jnp.bfloat16
F32 = jnp.float32
U32 = jnp.uint32
I32 = jnp.int32

GS = 4

LHS = {1: ((0, 0, 1), (1, 1, 1)), 2: ((1, 0, 1), (1, 1, 1)), 3: ((0, 0, 1),), 4: ((1, 1, 1),),
       5: ((0, 0, 1), (0, 1, 1)), 6: ((1, 0, 1), (0, 0, -1)), 7: ((0, 1, 1), (1, 1, -1))}
RHS = {1: ((0, 0, 1), (1, 1, 1)), 2: ((0, 0, 1),), 3: ((0, 1, 1), (1, 1, -1)), 4: ((1, 0, 1), (0, 0, -1)),
       5: ((1, 1, 1),), 6: ((0, 0, 1), (0, 1, 1)), 7: ((1, 0, 1), (1, 1, 1))}
OUT = {(0, 0): ((4, 1), (7, 1), (1, 1), (5, -1)), (0, 1): ((3, 1), (5, 1)),
       (1, 0): ((2, 1), (4, 1)), (1, 1): ((3, 1), (6, 1), (1, 1), (2, -1))}
BASIS = ((3, 1, 5, 7), (4, 1, 2, 6))
PHASES = ((1, 1, 0), (1, 0, 1), (0, 0, 0), (0, 1, 1))

SEQ_FULL = (
    "xx....A............q......q........p......q......p......q......p......EqEEE......p......q.....p.........q....p....q..oooooopooooopoooooooHoooooooooooooo",
    "x........A........q........q......p......q.....p.......q......p......EEqEE..p..........q.....p.......q......p......qoooooopooooopoooHoooooooooooooooooo",
    "xx........A.........q.......q.......p.........q...p.....qEEEE.........q.p.....p.........q......p......q......p......qooooopooooopooooHoooooooooooooooooo",
    "x........A........q........q......p......q......p......q....p........qEE..p...E..E.....q....p........q......p......qoooooopooooopoooHoooooooooooooooooo",
    "xx........A.........q.......q.......p.........q...p.....qEEEE.........q.p.....p.........q......p......q......p......qooooopooooopooooHoooooooooooooooooo",
    "x........A........q........q......p......q.....p.......q......p......EEqEE..p..........q.....p...........q..p......qoooooopooooopoooHoooooooooooooooooo",
    "xx........A.........q.......q.......p.........q...p.....qEEEE.........q.p.....p.........q......p......q......p......qooooopooooopooooHoooooooooooooooooo",
    "x........A........q........q......p......q......p......q....p........qEE..p...E.E......q....p........q......p......qoooooopooooopoooHoooooooooooooooooo",
)


def _rb(v):
    return v.astype(BF).astype(F32)


def _layernorm(x):
    inv_n = 1.0 / x.shape[-1]
    m = jnp.sum(x, axis=-1, keepdims=True) * inv_n
    d = x - m
    v = _rb(jnp.sum(d * d, axis=-1, keepdims=True) * inv_n)
    den = _rb(jnp.sqrt(_rb(v + 1.0013580322265625e-05)))
    return _rb(_rb(x - _rb(m)) * (1.0 / den))


def _dot(a, b):
    return jnp.dot(a, b, preferred_element_type=F32)


def _signed_sum(terms):
    terms = sorted(terms, key=lambda t: -t[1])
    total = terms[0][0] if terms[0][1] > 0 else -terms[0][0]
    for v, sign in terms[1:]:
        total = total + v if sign > 0 else total - v
    return total


def _left_operand(a, b, block, rows=None):
    return _signed_sum([(block(2 * i + k, 2 * j + l), s * t) for i, j, s in LHS[a] for k, l, t in LHS[b]
                        if rows is None or 2 * i + k == rows])


def _output(pos, prods):
    terms = [(prods[m], s) for m, s in OUT[pos] if prods.get(m) is not None]
    return _signed_sum(terms) if terms else None


def _weight_operands(block):
    vals = []
    for a in RHS:
        outer = {(k, l): _signed_sum([(block(2 * i + k, 2 * j + l), s) for i, j, s in RHS[a]])
                 for k in range(2) for l in range(2)}
        for b in RHS:
            vals.append(_signed_sum([(outer[k, l], t) for k, l, t in RHS[b]]))
            if len(vals) == 2 or a == b == 7:
                w = pltpu.bitcast(jnp.concatenate(vals, axis=1).astype(BF), U32)
                yield from (w[:, c:c + 128] for c in range(0, w.shape[1], 128))
                vals = []


class _Phase:
    def __init__(self, u):
        h0, h1, self.wide = PHASES[u]
        self.u, self.row = u, 2 * h0 + h1
        self.ws, self.ns = (BASIS[h] for h in ((h0, h1) if self.wide == 0 else (h1, h0)))

    def pair(self, w, n):
        return (w, n) if self.wide == 0 else (n, w)

    def index(self, w, n):
        a, b = self.pair(w, n)
        return 7 * (a - 1) + b - 1

    def place(self, pw, pn):
        (i, j), (k, l) = self.pair(pw, pn)
        return 2 * i + k, 2 * j + l

    def touched(self):
        return {self.place(pw, pn) for pw in OUT for pn in OUT
                if any(m in self.ws for m, _ in OUT[pw] if m != 1) and any(m in self.ns for m, _ in OUT[pn] if m != 1)}

    def run(self, product, emit, wide_first, order=None):
        first, second = (self.ws, self.ns) if wide_first else (self.ns, self.ws)
        second = order or second
        partial = {}
        for m2 in second:
            got = {}
            for m1 in first:
                for t, v in product(*((m1, m2) if wide_first else (m2, m1))).items():
                    got.setdefault(t, {})[m1] = v
                if m1 != first[-1]:
                    yield
            for t, prods in got.items():
                for p1 in OUT:
                    partial.setdefault((t, p1), {})[m2] = _output(p1, prods)
            for p2, terms in OUT.items():
                need = [m for m in second if m in dict(terms)]
                if need and need[-1] == m2:
                    for (t, p1), prods in partial.items():
                        i, j = self.place(*((p1, p2) if wide_first else (p2, p1)))
                        if (i == self.row) if t is None else ((i, j) in self.touched()):
                            emit(i, j, t, _output(p2, prods))
            yield


def _kernel(x_hbm, mem0_ref, wq_hbm, wk_hbm, wv_hbm, wo_hbm, wr_ref, wg_hbm, wu_hbm, wd_hbm,
            out_hbm,
            raw, wo_raw, wqkv, wout, xbuf, xmid, hbuf, hl, qkv, obuf, oacc, state, bidx_ref,
            wg_s, wu_s, wd_s, late, sems,
            *, S, D, H, E, M, T):
    NG = S // (T * GS)
    L = M + T
    NQ = H // 4
    NHG = H // 8
    NC = 3 * NHG
    w_hbm = (wq_hbm, wk_hbm, wv_hbm)
    phases = [_Phase(u) for u in range(GS)]

    def cp_w(c):
        return pltpu.make_async_copy(w_hbm[c // NHG].at[:, c % NHG], raw.at[c], sems.at[c])

    def cp_o(k):
        return pltpu.make_async_copy(wo_hbm.at[k], wo_raw.at[k], sems.at[NC + k])

    cp_x = [pltpu.make_async_copy(x_hbm.at[pl.ds(lo, hi - lo)], xbuf.at[pl.ds(lo, hi - lo)], sems.at[NC + NHG + k])
            for k, (lo, hi) in enumerate(((0, 3), (3, 5), (5, NG)))]
    cp_out = [pltpu.make_async_copy(xbuf.at[pl.ds(lo, hi - lo)], out_hbm.at[pl.ds(lo, hi - lo)], sems.at[NC + NHG + k])
              for k, (lo, hi) in enumerate(((0, NG - 4), (NG - 4, NG)))]
    cp_b = [pltpu.make_async_copy(w, s, sems.at[NC + NHG + 3 + j])
            for j, (w, s) in enumerate(((wg_hbm, wg_s), (wu_hbm, wu_s), (wd_hbm, wd_s)))]

    def normed(x):
        x = x.astype(F32)
        d = x - jnp.sum(x, axis=-1, keepdims=True) * (1.0 / D)
        return d * lax.rsqrt(jnp.sum(d * d, axis=-1, keepdims=True) * (1.0 / D) + 1e-5)

    def prenorm(g, u):
        hbuf[g, u] = normed(xbuf[g, u])

    def rows_of(tiles):
        return pl.ds(tiles[0] * 8, len(tiles) * 8)

    def build_lhs(g, ph):
        for n in ph.ns:
            for w in ph.ws:
                if n != 1 or (w, ph.u) == (1, 0):
                    hl[ph.index(w, n)] = _left_operand(*ph.pair(w, n), lambda s, k: hbuf[g, s, :, pl.ds(k * E, E)])

    def accumulate(ref, ph, i, j, index, v):
        seen = any((i, j) in p.touched() for p in phases[:ph.u])
        ref[index] = v + ref[index] if seen else v

    def split(res, tiles, mem_first, with_mem):
        off = M if with_mem and mem_first else 0
        out = {t: res[off + 8 * n:off + 8 * n + 8] for n, t in enumerate(tiles)}
        if with_mem:
            out[None] = res[:M] if mem_first else res[-M:]
        return out

    def first_product(blk):
        return _dot(hl[0], pltpu.bitcast(wqkv[blk, 0], BF))

    def qkv_block(ph, par, blk, mem_lhs, mem_out, first):
        def product(w, n):
            tiles = range(4 * (n != 1))
            left = [hl[ph.index(w, n)]] if tiles else []
            left += [mem_lhs[w, n]] if mem_lhs else []
            out = split(first, range(4), False, False) if (w, n) == (1, 1) and first is not None else {}
            if left:
                res = _dot(jnp.concatenate(left, axis=0), pltpu.bitcast(wqkv[blk, ph.index(w, n)], BF))
                out.update(split(res, tiles, False, mem_lhs))
            return out

        def emit(i, j, t, v):
            if t is None:
                mem_out[j] = v
            else:
                accumulate(qkv, ph, i, j, (par, blk, pl.ds((4 * i + j) * T + t * 8, 8)), v)
        return ph.run(product, emit, True)

    def out_rounds(ph, par, mem_in, mem_out):
        def tiles_of(w, n):
            if (w, n) == (1, 1):
                return range(ph.u, ph.u + 1) if mem_in else range(4 * (ph.u == 0))
            return range(4 * (n != 1))

        def half(w, n, k):
            tiles = tiles_of(w, n)
            left = [_left_operand(*ph.pair(w, n), lambda s, j: mem_in(j, k), ph.row)] if mem_in else []
            if tiles:
                left += [_left_operand(*ph.pair(w, n),
                                  lambda s, j: obuf[par, s, j, rows_of(tiles), pl.ds(k * 4 * E, 4 * E)])]
            if left:
                return _dot(jnp.concatenate(left, axis=0),
                            pltpu.bitcast(wout[ph.index(w, n), pl.ds(k * 2 * E, 2 * E)], BF))

        def product(w, n):
            res = half(w, n, 1)
            return {} if res is None else split(res + early[w, n], tiles_of(w, n), True, mem_in)

        def emit(i, j, t, v):
            if t is None:
                mem_out[j] = v
            else:
                accumulate(oacc, ph, i, j, (par, i, pl.ds(t * 8, 8), pl.ds(j * E, E)), v)
        early = {}
        for w in ph.ws[::-1]:
            for n in ph.ns:
                early[w, n] = half(w, n, 0)
                yield
        yield from ph.run(product, emit, False, ph.ws[::-1])

    cp_w(0).start()
    cp_x[0].start()
    for c in range(1, NC):
        cp_w(c).start()
    for k in range(NHG):
        cp_o(k).start()
    for c in cp_x[1:] + cp_b:
        c.start()
    xbuf[NG] = jnp.zeros((GS, T, D), BF)
    oacc[0] = jnp.zeros(oacc.shape[1:], F32)
    obuf[1] = jnp.zeros(obuf.shape[1:], F32)

    def prep_qkv(c):
        for r in range(E // 16):
            for k in range(4):
                words = pltpu.bitcast(raw[c, pl.ds(k * E + r * 16, 16)].reshape(128, E), U32)
                qkv[1, r, pl.ds(k * 64, 64)] = pltpu.bitcast(words, F32)
        for r in range(E // 16):
            for n in range(2):
                def block(k, j):
                    w = pltpu.bitcast(qkv[1, r, pl.ds(k * 64 + 2 * n + j // 2, 16, stride=4), :], U32)
                    return pltpu.bitcast(w & np.uint32(0xFFFF0000) if j % 2 else w << 16, F32)
                for m, w in enumerate(_weight_operands(block)):
                    wqkv[2 * c + n, m, pl.ds(r * 8, 8)] = w

    def prep_out(k):
        for r in range(E // 16):
            for n in range(2):
                heads = [wo_raw[k, 4 * n + i, pl.ds(r * 16, 16)].astype(F32) for i in range(4)]
                for m, w in enumerate(_weight_operands(lambda i, j: heads[i][:, j * E:j * E + E])):
                    wout[m, pl.ds(pl.multiple_of((2 * k + n) * (E // 2) + r * 8, 8), 8)] = w

    def project_first(c):
        for ph in phases:
            for blk in (2 * c, 2 * c + 1):
                list(qkv_block(ph, 0, blk, None, None, None if ph.u else first_product(blk)))

    cp_w(0).wait()
    prep_qkv(0)
    cp_x[0].wait()
    hbuf[:3] = normed(xbuf[:3].reshape(3 * GS * T, D)).reshape(3, GS, T, D)
    for ph in phases:
        build_lhs(0, ph)

    def stream(c, carry):
        pltpu.make_async_copy(raw.at[c + 1], raw.at[c + 1], sems.at[c + 1]).wait()
        prep_qkv(c + 1)
        project_first(c)
        return carry
    lax.fori_loop(0, NC - 1, stream, 0)
    project_first(NC - 1)
    build_lhs(1, phases[0])

    def stream_o(k, carry):
        cp_o(k).wait()
        prep_out(k)
        return carry
    lax.fori_loop(0, NHG, stream_o, 0)
    cp_x[1].wait()

    def reset_memory():
        state[:M] = mem0_ref[...].astype(F32)

    def reset_router():
        state[M:] = jnp.full((8, D), -jnp.inf, F32)
        bidx_ref[:, :128] = jnp.full((8, 128), S, I32)
    reset_memory()
    reset_router()

    def router(xn):
        return _rb(jnp.sum(xn * wr_ref[...].astype(F32).reshape(1, D), axis=-1, keepdims=True))

    def epilogue(g, u, t, par, best, bidx):
        rows = pl.ds(t * 8, 8)
        x1 = _rb(xbuf[g, u, rows].astype(F32) + _rb(oacc[par, u, rows]))
        xn = _layernorm(x1)
        xmid[0, g, u, rows] = x1
        xmid[1, g, u, rows] = xn
        xbuf[g, u, rows] = (x1 + xn).astype(BF)
        it = lax.broadcasted_iota(I32, (8, 128), 0) + ((g * GS + u) * T + t * 8)
        r = jnp.where(it < S, jnp.broadcast_to(router(xn), (8, 128)), -jnp.inf)
        better = r > best
        return jnp.where(better, r, best), jnp.where(better, it, bidx)

    def segment(par, ph, mem, seq, jobs, firsts, first_rounds):
        u = ph.u
        row = lax.broadcasted_iota(I32, (L, L), 0)
        col = lax.broadcasted_iota(I32, (L, L), 1)
        mask = (row < M) | (row >= col)
        mem_lhs = {(w, n): _left_operand(*ph.pair(w, n), lambda s, k: mem[k], ph.row) for n in ph.ns for w in ph.ws}
        proj = [{} for _ in range(3 * NQ)]
        probs, outs, new_mem = {}, {}, {}

        def head(j, n, i):
            return jnp.concatenate([proj[j * NQ + n][i], qkv[par, j * NQ + n, pl.ds((4 * u + i) * T, T)]], axis=0)

        def scores(n):
            for i in range(4):
                sc = lax.dot_general(head(0, n, i), head(1, n, i).astype(BF), (((1,), (1,)), ((), ())),
                                     preferred_element_type=F32)
                sc = jnp.where(mask, sc, -1e9 * E ** 0.5)
                e = jnp.exp2((sc - jnp.max(sc, axis=-1, keepdims=True)) * (E ** -0.5 * 1.4426950408889634))
                probs[n, i] = e * pltpu.reciprocal(jnp.sum(e, axis=-1, keepdims=True), full_range=False)

        def values(n):
            for i in range(4):
                o = _dot(probs[n, i], head(2, n, i).astype(BF))
                outs[n, i] = o[:M]
                obuf[par, u, i, :, pl.ds(n * E, E)] = o[M:]

        def rounds():
            order = [(j, n - (j == 2)) for n in range(NQ + 1) for j in range(3) if 0 <= n - (j == 2) < NQ]
            for blk in (j * NQ + n for j, n in order):
                for k, _ in enumerate(qkv_block(ph, 1 - par, blk, mem_lhs, proj[blk], firsts.pop(blk, None))):
                    if k % 4 == 3:
                        yield

        def mem_in(i, k):
            return jnp.concatenate([outs[n, i] for n in range(4 * k, 4 * k + 4)], axis=1)
        its = {".": rounds(), "o": out_rounds(ph, 1 - par, mem_in, new_mem),
               "q": map(scores, range(NQ)), "p": map(values, range(NQ))}
        its.update({ch: (f() for f in fs) for ch, fs in jobs.items()})
        assert "x" not in seq.lstrip("x")
        for ch in seq:
            next(first_rounds if ch == "x" else its[ch])
        assert not any(list(it) for it in its.values())
        return [_rb(new_mem[j]) for j in range(4)]

    def group_pair(G0, pending):
        mem, top = [state[:M, pl.ds(j * E, E)] for j in range(4)], [state[M:, :128], bidx_ref[:, :128]]
        for par in range(2):
            G = G0 + par
            g = G % NG

            def post(u, t):
                top[:] = epilogue(jnp.where(g >= 2, g - 2, jnp.where(pending, g + NG - 2, NG)), u, t, par, *top)
                hl[49 + G0 // NG, :8] = top[0]

            firsts = {}
            first_rounds = (firsts.update({blk: first_product(blk) for blk in range(k, k + 4)})
                            for k in range(0, 3 * NQ, 4))
            for u in range(GS):
                mem = segment(par, phases[u], mem, SEQ_FULL[(par * GS + u) % len(SEQ_FULL)], {
                    "H": [functools.partial(prenorm, (G + 3) % NG, u)],
                    "A": [functools.partial(build_lhs, (G + 1 + (u + 1) // GS) % NG, phases[(u + 1) % GS])],
                    "E": [functools.partial(post, u, t) for t in range(T // 8)]}, firsts, first_rounds)
            assert not firsts and not list(first_rounds)
        for j in range(4):
            state[:M, pl.ds(j * E, E)] = mem[j]
        state[M:, :128], bidx_ref[:, :128] = top

    def drain():
        best, bidx = state[M:, :128], bidx_ref[:, :128]
        for ph in phases:
            list(out_rounds(ph, 1, None, None))
        for par in range(2):
            for u in range(GS):
                for t in range(T // 8):
                    best, bidx = epilogue(NG - 2 + par, u, t, par, best, bidx)
        state[M:, :128], bidx_ref[:, :128] = best, bidx

    def top_token():
        best = state[M:, :128]
        idx = jnp.min(jnp.where(best == jnp.max(best, axis=0, keepdims=True), bidx_ref[:, :128], S))
        return jnp.where(idx >= S, 0, idx)

    def expert(last, nxt):
        idx = top_token()
        g, u = idx // (T * GS), idx // T % GS
        tile = pl.multiple_of(idx % T // 8 * 8, 8)
        rows = pl.ds(tile, 8)
        x1, xn = xmid[0, g, u, rows], xmid[1, g, u, rows]
        gate = _rb(_dot(xn, wg_s[...]))
        up = _rb(_dot(xn, wu_s[...]))
        gate = _rb(gate * _rb(jax.nn.sigmoid(gate)))
        y = _rb(_dot(_rb(gate * up), wd_s[...]))
        y = _rb(y * _rb(jax.nn.sigmoid(router(xn))))
        sel = lax.broadcasted_iota(I32, (8, D), 0) == idx % 8
        x2 = (x1 + _rb(xn + jnp.where(sel, y, 0.0))).astype(BF)

        @pl.when(last)
        def _():
            cp_out[0].wait()
            cp_out[1].wait()
            xbuf[g, u, rows] = x2
            cp = pltpu.make_async_copy(xbuf.at[g, u], out_hbm.at[g, u], sems.at[0])
            cp.start()
            cp.wait()

        @pl.when(jnp.logical_not(last))
        def _():
            xbuf[g, u, rows] = x2
            h = normed(x2)
            hbuf[g, u, rows] = h
            build_lhs(nxt + 1, phases[0])
            reset_router()

            @pl.when(g == nxt)
            def _():
                ph = phases[0]
                left = {(w, n): _left_operand(*ph.pair(w, n), lambda s, k: h[:, k * E:k * E + E], ph.row)
                        for n in ph.ns for w in ph.ws}

                def redo(blk, carry):
                    def product(w, n):
                        return {None: _dot(left[w, n], pltpu.bitcast(wqkv[blk, ph.index(w, n)], BF))}

                    def emit(i, j, t, v):
                        qkv[0, blk, pl.ds(pl.multiple_of((4 * u + j) * T + tile, 8), 8)] = v
                    list(ph.run(product, emit, True))
                    return carry
                lax.fori_loop(0, 3 * NQ, redo, 0, unroll=4)

    def iteration(it, carry):
        last = it == NG - 1
        seam = it == NG // 2 - 1
        pending = late[0] == 1

        @pl.when(it == 1)
        def _():
            for c in cp_x[2:] + cp_b:
                c.wait()

        @pl.when(last)
        def _():
            cp_out[0].start()
        group_pair(2 * it, pending)
        late[0] = 0

        @pl.when(seam)
        def _():
            late[0] = (top_token() >= 2 * GS * T).astype(I32)
            reset_memory()
        now = last | (seam & (late[0] == 0))
        pl.when(now)(drain)

        @pl.when(last)
        def _():
            cp_out[1].start()
        pl.when(now | pending)(lambda: expert(last, jnp.where(pending, 2, 0)))
        return carry

    late[0] = 0
    lax.fori_loop(0, NG, iteration, 0)


@functools.partial(jax.jit, static_argnames=("A_seg_len",))
def pallas_interleave_layers__memory_aug_recurrent_mem_tr__moe_arch_mod__prompt_kernel(
    A_x, A_mem0, A_Wq, A_Wk, A_Wv, A_Wo, A_seg_len, B_x, B_w_r, B_w_gate, B_w_up, B_w_down,
):
    del B_x
    B, S, D = A_x.shape
    _, H, E = A_Wq.shape
    M = A_mem0.shape[1]
    F = B_w_gate.shape[1]
    T = int(A_seg_len)
    assert (B, S, D, H, E, M, T) == (1, 2048, 512, 32, 128, 8, 32)
    NG = S // (T * GS)
    NHG = H // 8
    hbm = pl.BlockSpec(memory_space=pl.ANY)
    vmem = pl.BlockSpec(memory_space=pltpu.VMEM)
    out = pl.pallas_call(
        functools.partial(_kernel, S=S, D=D, H=H, E=E, M=M, T=T),
        out_shape=jax.ShapeDtypeStruct((NG, GS, T, D), A_x.dtype),
        in_specs=[hbm, vmem, hbm, hbm, hbm, hbm, vmem, hbm, hbm, hbm],
        out_specs=hbm,
        scratch_shapes=[
            pltpu.VMEM((3 * NHG, D, 8, E), BF),
            pltpu.VMEM((NHG, 8, E, D), BF),
            pltpu.VMEM((3 * H // 4, 49, E // 2, E), U32),
            pltpu.VMEM((49, H // 4 * E // 2, E), U32),
            pltpu.VMEM((NG + 1, GS, T, D), BF),
            pltpu.VMEM((2, NG + 1, GS, T, D), F32),
            pltpu.VMEM((NG, GS, T, D), F32),
            pltpu.VMEM((51, T, E), F32),
            pltpu.VMEM((2, 3 * H // 4, GS * 4 * T, E), F32),
            pltpu.VMEM((2, GS, 4, T, H // 4 * E), F32),
            pltpu.VMEM((2, GS, T, D), F32),
            pltpu.VMEM((M + 8, D), F32),
            pltpu.VMEM((8, 512), I32),
            pltpu.VMEM((D, F), BF),
            pltpu.VMEM((D, F), BF),
            pltpu.VMEM((F, D), BF),
            pltpu.SMEM((1,), I32),
            pltpu.SemaphoreType.DMA((4 * NHG + 6,)),
        ],
        compiler_params=pltpu.CompilerParams(vmem_limit_bytes=120 * 2**20),
        name="rmt_mod",
    )(
        A_x.reshape(NG, GS, T, D), A_mem0.reshape(M, D),
        A_Wq.reshape(D, NHG, 8, E), A_Wk.reshape(D, NHG, 8, E), A_Wv.reshape(D, NHG, 8, E),
        A_Wo.reshape(NHG, 8, E, D),
        B_w_r, B_w_gate, B_w_up, B_w_down,
    )
    return out.reshape(B, S, D)
```

```python
import functools

import numpy as np
import jax
import jax.numpy as jnp
from jax import lax
import jax.experimental.pallas as pl
import jax.experimental.pallas.tpu as pltpu

BF = jnp.bfloat16
F32 = jnp.float32
U32 = jnp.uint32
I32 = jnp.int32

GS = 4

LHS = {1: ((0, 0, 1), (1, 1, 1)), 2: ((1, 0, 1), (1, 1, 1)), 3: ((0, 0, 1),), 4: ((1, 1, 1),),
       5: ((0, 0, 1), (0, 1, 1)), 6: ((1, 0, 1), (0, 0, -1)), 7: ((0, 1, 1), (1, 1, -1))}
RHS = {1: ((0, 0, 1), (1, 1, 1)), 2: ((0, 0, 1),), 3: ((0, 1, 1), (1, 1, -1)), 4: ((1, 0, 1), (0, 0, -1)),
       5: ((1, 1, 1),), 6: ((0, 0, 1), (0, 1, 1)), 7: ((1, 0, 1), (1, 1, 1))}
OUT = {(0, 0): ((4, 1), (7, 1), (1, 1), (5, -1)), (0, 1): ((3, 1), (5, 1)),
       (1, 0): ((2, 1), (4, 1)), (1, 1): ((3, 1), (6, 1), (1, 1), (2, -1))}
BASIS = ((3, 1, 5, 7), (4, 1, 2, 6))
PHASES = ((1, 1, 0), (1, 0, 1), (0, 0, 0), (0, 1, 1))

SEQ_FULL = (
    "xx....A............q......q........p......q......p......q......p......EqEEE......p......q.....p.........q....p....q..oooooopooooopoooooooHoooooooooooooo",
    "x........A........q........q......p......q.....p.......q......p......EEqEE..p..........q.....p.......q......p......qoooooopooooopoooHoooooooooooooooooo",
    "xx........A.........q.......q.......p.........q...p.....qEEEE.........q.p.....p.........q......p......q......p......qooooopooooopooooHoooooooooooooooooo",
    "x........A........q........q......p......q......p......q....p........qEE..p...E..E.....q....p........q......p......qoooooopooooopoooHoooooooooooooooooo",
    "xx........A.........q.......q.......p.........q...p.....qEEEE.........q.p.....p.........q......p......q......p......qooooopooooopooooHoooooooooooooooooo",
    "x........A........q........q......p......q.....p.......q......p......EEqEE..p..........q.....p...........q..p......qoooooopooooopoooHoooooooooooooooooo",
    "xx........A.........q.......q.......p.........q...p.....qEEEE.........q.p.....p.........q......p......q......p......qooooopooooopooooHoooooooooooooooooo",
    "x........A........q........q......p......q......p......q....p........qEE..p...E.E......q....p........q......p......qoooooopooooopoooHoooooooooooooooooo",
)


def _rb(v):
    return v.astype(BF).astype(F32)


def _layernorm(x):
    inv_n = 1.0 / x.shape[-1]
    m = jnp.sum(x, axis=-1, keepdims=True) * inv_n
    d = x - m
    v = _rb(jnp.sum(d * d, axis=-1, keepdims=True) * inv_n)
    den = _rb(jnp.sqrt(_rb(v + 1.0013580322265625e-05)))
    return _rb(_rb(x - _rb(m)) * (1.0 / den))


def _dot(a, b):
    return jnp.dot(a, b, preferred_element_type=F32)


def _signed_sum(terms):
    terms = sorted(terms, key=lambda t: -t[1])
    total = terms[0][0] if terms[0][1] > 0 else -terms[0][0]
    for v, sign in terms[1:]:
        total = total + v if sign > 0 else total - v
    return total


def _left_operand(a, b, block, rows=None):
    return _signed_sum([(block(2 * i + k, 2 * j + l), s * t) for i, j, s in LHS[a] for k, l, t in LHS[b]
                        if rows is None or 2 * i + k == rows])


def _output(pos, prods):
    terms = [(prods[m], s) for m, s in OUT[pos] if prods.get(m) is not None]
    return _signed_sum(terms) if terms else None


def _weight_operands(block):
    vals = []
    for a in RHS:
        outer = {(k, l): _signed_sum([(block(2 * i + k, 2 * j + l), s) for i, j, s in RHS[a]])
                 for k in range(2) for l in range(2)}
        for b in RHS:
            vals.append(_signed_sum([(outer[k, l], t) for k, l, t in RHS[b]]))
            if len(vals) == 2 or a == b == 7:
                w = pltpu.bitcast(jnp.concatenate(vals, axis=1).astype(BF), U32)
                yield from (w[:, c:c + 128] for c in range(0, w.shape[1], 128))
                vals = []


class _Phase:
    def __init__(self, u):
        h0, h1, self.wide = PHASES[u]
        self.u, self.row = u, 2 * h0 + h1
        self.ws, self.ns = (BASIS[h] for h in ((h0, h1) if self.wide == 0 else (h1, h0)))

    def pair(self, w, n):
        return (w, n) if self.wide == 0 else (n, w)

    def index(self, w, n):
        a, b = self.pair(w, n)
        return 7 * (a - 1) + b - 1

    def place(self, pw, pn):
        (i, j), (k, l) = self.pair(pw, pn)
        return 2 * i + k, 2 * j + l

    def touched(self):
        return {self.place(pw, pn) for pw in OUT for pn in OUT
                if any(m in self.ws for m, _ in OUT[pw] if m != 1) and any(m in self.ns for m, _ in OUT[pn] if m != 1)}

    def run(self, product, emit, wide_first, order=None):
        first, second = (self.ws, self.ns) if wide_first else (self.ns, self.ws)
        second = order or second
        partial = {}
        for m2 in second:
            got = {}
            for m1 in first:
                for t, v in product(*((m1, m2) if wide_first else (m2, m1))).items():
                    got.setdefault(t, {})[m1] = v
                if m1 != first[-1]:
                    yield
            for t, prods in got.items():
                for p1 in OUT:
                    partial.setdefault((t, p1), {})[m2] = _output(p1, prods)
            for p2, terms in OUT.items():
                need = [m for m in second if m in dict(terms)]
                if need and need[-1] == m2:
                    for (t, p1), prods in partial.items():
                        i, j = self.place(*((p1, p2) if wide_first else (p2, p1)))
                        if (i == self.row) if t is None else ((i, j) in self.touched()):
                            emit(i, j, t, _output(p2, prods))
            yield


def _kernel(x_hbm, mem0_ref, wq_hbm, wk_hbm, wv_hbm, wo_hbm, wr_ref, wg_hbm, wu_hbm, wd_hbm,
            out_hbm,
            raw, wo_raw, wqkv, wout, xbuf, xmid, hbuf, hl, qkv, obuf, oacc, state, bidx_ref,
            wg_s, wu_s, wd_s, late, sems,
            *, S, D, H, E, M, T):
    NG = S // (T * GS)
    L = M + T
    NQ = H // 4
    NHG = H // 8
    NC = 3 * NHG
    w_hbm = (wq_hbm, wk_hbm, wv_hbm)
    phases = [_Phase(u) for u in range(GS)]

    def cp_w(c):
        return pltpu.make_async_copy(w_hbm[c // NHG].at[:, c % NHG], raw.at[c], sems.at[c])

    def cp_o(k):
        return pltpu.make_async_copy(wo_hbm.at[k], wo_raw.at[k], sems.at[NC + k])

    cp_x = [pltpu.make_async_copy(x_hbm.at[pl.ds(lo, hi - lo)], xbuf.at[pl.ds(lo, hi - lo)], sems.at[NC + NHG + k])
            for k, (lo, hi) in enumerate(((0, 3), (3, 5), (5, NG)))]
    cp_out = [pltpu.make_async_copy(xbuf.at[pl.ds(lo, hi - lo)], out_hbm.at[pl.ds(lo, hi - lo)], sems.at[NC + NHG + k])
              for k, (lo, hi) in enumerate(((0, NG - 4), (NG - 4, NG)))]
    cp_b = [pltpu.make_async_copy(w, s, sems.at[NC + NHG + 3 + j])
            for j, (w, s) in enumerate(((wg_hbm, wg_s), (wu_hbm, wu_s), (wd_hbm, wd_s)))]

    def normed(x):
        x = x.astype(F32)
        d = x - jnp.sum(x, axis=-1, keepdims=True) * (1.0 / D)
        return d * lax.rsqrt(jnp.sum(d * d, axis=-1, keepdims=True) * (1.0 / D) + 1e-5)

    def prenorm(g, u):
        hbuf[g, u] = normed(xbuf[g, u])

    def rows_of(tiles):
        return pl.ds(tiles[0] * 8, len(tiles) * 8)

    def build_lhs(g, ph):
        for n in ph.ns:
            for w in ph.ws:
                if n != 1 or (w, ph.u) == (1, 0):
                    hl[ph.index(w, n)] = _left_operand(*ph.pair(w, n), lambda s, k: hbuf[g, s, :, pl.ds(k * E, E)])

    def accumulate(ref, ph, i, j, index, v):
        seen = any((i, j) in p.touched() for p in phases[:ph.u])
        ref[index] = v + ref[index] if seen else v

    def first_product(blk):
        return _dot(hl[0], pltpu.bitcast(wqkv[blk, 0], BF))

    def qkv_block(ph, par, blk, mem_lhs, mem_out, first):
        def product(w, n):
            left = [hl[ph.index(w, n)]] if n != 1 else []
            left += [mem_lhs[w, n]] if mem_lhs else []
            out = {0: first} if (w, n) == (1, 1) else {}
            if left:
                res = _dot(jnp.concatenate(left, axis=0), pltpu.bitcast(wqkv[blk, ph.index(w, n)], BF))
                if n != 1:
                    out[0] = res[:T]
                if mem_lhs:
                    out[None] = res[-M:]
            return out

        def emit(i, j, t, v):
            if t is None:
                mem_out[j] = v
            else:
                accumulate(qkv, ph, i, j, (par, blk, pl.ds((4 * i + j) * T, T)), v)
        return ph.run(product, emit, True)

    def out_rounds(ph, par, mem_in, mem_out):
        def tiles_of(w, n):
            if (w, n) == (1, 1):
                return range(ph.u, ph.u + 1) if mem_in else range(4 * (ph.u == 0))
            return range(4 * (n != 1))

        def half(w, n, k):
            tiles = tiles_of(w, n)
            left = [_left_operand(*ph.pair(w, n), lambda s, j: mem_in(j, k), ph.row)] if mem_in else []
            if tiles:
                left += [_left_operand(*ph.pair(w, n),
                                  lambda s, j: obuf[par, s, j, rows_of(tiles), pl.ds(k * 4 * E, 4 * E)])]
            if left:
                return _dot(jnp.concatenate(left, axis=0),
                            pltpu.bitcast(wout[ph.index(w, n), pl.ds(k * 2 * E, 2 * E)], BF))

        def product(w, n):
            res = half(w, n, 1)
            if res is None:
                return {}
            res = res + early[w, n]
            return {t: res[8 * k:8 * k + 8] for k, t in enumerate([None] * bool(mem_in) + list(tiles_of(w, n)))}

        def emit(i, j, t, v):
            if t is None:
                mem_out[j] = v
            else:
                accumulate(oacc, ph, i, j, (par, i, pl.ds(t * 8, 8), pl.ds(j * E, E)), v)
        early = {}
        for w in ph.ws[::-1]:
            for n in ph.ns:
                early[w, n] = half(w, n, 0)
                yield
        yield from ph.run(product, emit, False, ph.ws[::-1])

    cp_w(0).start()
    cp_x[0].start()
    for c in range(1, NC):
        cp_w(c).start()
    for k in range(NHG):
        cp_o(k).start()
    for c in cp_x[1:] + cp_b:
        c.start()
    xbuf[NG] = jnp.zeros((GS, T, D), BF)
    oacc[0] = jnp.zeros(oacc.shape[1:], F32)
    obuf[1] = jnp.zeros(obuf.shape[1:], F32)

    def prep_qkv(c):
        for r in range(E // 16):
            for k in range(4):
                words = pltpu.bitcast(raw[c, pl.ds(k * E + r * 16, 16)].reshape(128, E), U32)
                qkv[1, r, pl.ds(k * 64, 64)] = pltpu.bitcast(words, F32)
        for r in range(E // 16):
            for n in range(2):
                def block(k, j):
                    w = pltpu.bitcast(qkv[1, r, pl.ds(k * 64 + 2 * n + j // 2, 16, stride=4), :], U32)
                    return pltpu.bitcast(w & np.uint32(0xFFFF0000) if j % 2 else w << 16, F32)
                for m, w in enumerate(_weight_operands(block)):
                    wqkv[2 * c + n, m, pl.ds(r * 8, 8)] = w

    def prep_out(k):
        for r in range(E // 16):
            for n in range(2):
                heads = [wo_raw[k, 4 * n + i, pl.ds(r * 16, 16)].astype(F32) for i in range(4)]
                for m, w in enumerate(_weight_operands(lambda i, j: heads[i][:, j * E:j * E + E])):
                    wout[m, pl.ds(pl.multiple_of((2 * k + n) * (E // 2) + r * 8, 8), 8)] = w

    def project_first(c):
        for ph in phases:
            for blk in (2 * c, 2 * c + 1):
                list(qkv_block(ph, 0, blk, None, None, None if ph.u else first_product(blk)))

    cp_w(0).wait()
    prep_qkv(0)
    cp_x[0].wait()
    hbuf[:3] = normed(xbuf[:3].reshape(3 * GS * T, D)).reshape(3, GS, T, D)
    for ph in phases:
        build_lhs(0, ph)

    def stream(c, carry):
        pltpu.make_async_copy(raw.at[c + 1], raw.at[c + 1], sems.at[c + 1]).wait()
        prep_qkv(c + 1)
        project_first(c)
        return carry
    lax.fori_loop(0, NC - 1, stream, 0)
    project_first(NC - 1)
    build_lhs(1, phases[0])

    def stream_o(k, carry):
        cp_o(k).wait()
        prep_out(k)
        return carry
    lax.fori_loop(0, NHG, stream_o, 0)
    cp_x[1].wait()

    def reset_memory():
        state[:M] = mem0_ref[...].astype(F32)

    def reset_router():
        state[M:] = jnp.full((8, D), -jnp.inf, F32)
        bidx_ref[:, :128] = jnp.full((8, 128), S, I32)
    reset_memory()
    reset_router()

    def router(xn):
        return _rb(jnp.sum(xn * wr_ref[...].astype(F32).reshape(1, D), axis=-1, keepdims=True))

    def epilogue(g, u, t, par, best, bidx):
        rows = pl.ds(t * 8, 8)
        x1 = _rb(xbuf[g, u, rows].astype(F32) + _rb(oacc[par, u, rows]))
        xn = _layernorm(x1)
        xmid[0, g, u, rows] = x1
        xmid[1, g, u, rows] = xn
        xbuf[g, u, rows] = (x1 + xn).astype(BF)
        it = lax.broadcasted_iota(I32, (8, 128), 0) + ((g * GS + u) * T + t * 8)
        r = jnp.where(it < S, jnp.broadcast_to(router(xn), (8, 128)), -jnp.inf)
        better = r > best
        return jnp.where(better, r, best), jnp.where(better, it, bidx)

    def segment(par, ph, mem, seq, jobs, firsts, first_rounds):
        u = ph.u
        row = lax.broadcasted_iota(I32, (L, L), 0)
        col = lax.broadcasted_iota(I32, (L, L), 1)
        mask = (row < M) | (row >= col)
        mem_lhs = {(w, n): _left_operand(*ph.pair(w, n), lambda s, k: mem[k], ph.row) for n in ph.ns for w in ph.ws}
        proj = [{} for _ in range(3 * NQ)]
        probs, outs, new_mem = {}, {}, {}

        def head(j, n, i):
            return jnp.concatenate([proj[j * NQ + n][i], qkv[par, j * NQ + n, pl.ds((4 * u + i) * T, T)]], axis=0)

        def scores(n):
            for i in range(4):
                sc = lax.dot_general(head(0, n, i), head(1, n, i).astype(BF), (((1,), (1,)), ((), ())),
                                     preferred_element_type=F32)
                sc = jnp.where(mask, sc, -1e9 * E ** 0.5)
                e = jnp.exp2((sc - jnp.max(sc, axis=-1, keepdims=True)) * (E ** -0.5 * 1.4426950408889634))
                probs[n, i] = e * pltpu.reciprocal(jnp.sum(e, axis=-1, keepdims=True), full_range=False)

        def values(n):
            for i in range(4):
                o = _dot(probs[n, i], head(2, n, i).astype(BF))
                outs[n, i] = o[:M]
                obuf[par, u, i, :, pl.ds(n * E, E)] = o[M:]

        def rounds():
            order = [(j, n - (j == 2)) for n in range(NQ + 1) for j in range(3) if 0 <= n - (j == 2) < NQ]
            for blk in (j * NQ + n for j, n in order):
                for k, _ in enumerate(qkv_block(ph, 1 - par, blk, mem_lhs, proj[blk], firsts.pop(blk, None))):
                    if k % 4 == 3:
                        yield

        def mem_in(i, k):
            return jnp.concatenate([outs[n, i] for n in range(4 * k, 4 * k + 4)], axis=1)
        its = {".": rounds(), "o": out_rounds(ph, 1 - par, mem_in, new_mem),
               "q": map(scores, range(NQ)), "p": map(values, range(NQ))}
        its.update({ch: (f() for f in fs) for ch, fs in jobs.items()})
        assert "x" not in seq.lstrip("x")
        for ch in seq:
            next(first_rounds if ch == "x" else its[ch])
        assert not any(list(it) for it in its.values())
        return [_rb(new_mem[j]) for j in range(4)]

    def group_pair(G0, pending):
        mem, top = [state[:M, pl.ds(j * E, E)] for j in range(4)], [state[M:, :128], bidx_ref[:, :128]]
        for par in range(2):
            G = G0 + par
            g = G % NG

            def post(u, t):
                top[:] = epilogue(jnp.where(g >= 2, g - 2, jnp.where(pending, g + NG - 2, NG)), u, t, par, *top)
                hl[49 + G0 // NG, :8] = top[0]

            firsts = {}
            first_rounds = (firsts.update({blk: first_product(blk) for blk in range(k, k + 4)})
                            for k in range(0, 3 * NQ, 4))
            for u in range(GS):
                mem = segment(par, phases[u], mem, SEQ_FULL[(par * GS + u) % len(SEQ_FULL)], {
                    "H": [functools.partial(prenorm, (G + 3) % NG, u)],
                    "A": [functools.partial(build_lhs, (G + 1 + (u + 1) // GS) % NG, phases[(u + 1) % GS])],
                    "E": [functools.partial(post, u, t) for t in range(T // 8)]}, firsts, first_rounds)
            assert not firsts and not list(first_rounds)
        for j in range(4):
            state[:M, pl.ds(j * E, E)] = mem[j]
        state[M:, :128], bidx_ref[:, :128] = top

    def drain():
        best, bidx = state[M:, :128], bidx_ref[:, :128]
        for ph in phases:
            list(out_rounds(ph, 1, None, None))
        for par in range(2):
            for u in range(GS):
                for t in range(T // 8):
                    best, bidx = epilogue(NG - 2 + par, u, t, par, best, bidx)
        state[M:, :128], bidx_ref[:, :128] = best, bidx

    def top_token():
        best = state[M:, :128]
        idx = jnp.min(jnp.where(best == jnp.max(best, axis=0, keepdims=True), bidx_ref[:, :128], S))
        return jnp.where(idx >= S, 0, idx)

    def expert(last, nxt):
        idx = top_token()
        g, u = idx // (T * GS), idx // T % GS
        tile = pl.multiple_of(idx % T // 8 * 8, 8)
        rows = pl.ds(tile, 8)
        x1, xn = xmid[0, g, u, rows], xmid[1, g, u, rows]
        gate = _rb(_dot(xn, wg_s[...]))
        up = _rb(_dot(xn, wu_s[...]))
        gate = _rb(gate * _rb(jax.nn.sigmoid(gate)))
        y = _rb(_dot(_rb(gate * up), wd_s[...]))
        y = _rb(y * _rb(jax.nn.sigmoid(router(xn))))
        sel = lax.broadcasted_iota(I32, (8, D), 0) == idx % 8
        x2 = (x1 + _rb(xn + jnp.where(sel, y, 0.0))).astype(BF)

        @pl.when(last)
        def _():
            cp_out[0].wait()
            cp_out[1].wait()
            xbuf[g, u, rows] = x2
            cp = pltpu.make_async_copy(xbuf.at[g, u], out_hbm.at[g, u], sems.at[0])
            cp.start()
            cp.wait()

        @pl.when(jnp.logical_not(last))
        def _():
            xbuf[g, u, rows] = x2
            h = normed(x2)
            hbuf[g, u, rows] = h
            build_lhs(nxt + 1, phases[0])
            reset_router()

            @pl.when(g == nxt)
            def _():
                ph = phases[0]
                left = {(w, n): _left_operand(*ph.pair(w, n), lambda s, k: h[:, k * E:k * E + E], ph.row)
                        for n in ph.ns for w in ph.ws}

                def redo(blk, carry):
                    def product(w, n):
                        return {None: _dot(left[w, n], pltpu.bitcast(wqkv[blk, ph.index(w, n)], BF))}

                    def emit(i, j, t, v):
                        qkv[0, blk, pl.ds(pl.multiple_of((4 * u + j) * T + tile, 8), 8)] = v
                    list(ph.run(product, emit, True))
                    return carry
                lax.fori_loop(0, 3 * NQ, redo, 0, unroll=4)

    def iteration(it, carry):
        last = it == NG - 1
        seam = it == NG // 2 - 1
        pending = late[0] == 1

        @pl.when(it == 1)
        def _():
            for c in cp_x[2:] + cp_b:
                c.wait()

        @pl.when(last)
        def _():
            cp_out[0].start()
        group_pair(2 * it, pending)
        late[0] = 0

        @pl.when(seam)
        def _():
            late[0] = (top_token() >= 2 * GS * T).astype(I32)
            reset_memory()
        now = last | (seam & (late[0] == 0))
        pl.when(now)(drain)

        @pl.when(last)
        def _():
            cp_out[1].start()
        pl.when(now | pending)(lambda: expert(last, jnp.where(pending, 2, 0)))
        return carry

    late[0] = 0
    lax.fori_loop(0, NG, iteration, 0)


@functools.partial(jax.jit, static_argnames=("A_seg_len",))
def pallas_interleave_layers__memory_aug_recurrent_mem_tr__moe_arch_mod__prompt_kernel(
    A_x, A_mem0, A_Wq, A_Wk, A_Wv, A_Wo, A_seg_len, B_x, B_w_r, B_w_gate, B_w_up, B_w_down,
):
    del B_x
    B, S, D = A_x.shape
    _, H, E = A_Wq.shape
    M = A_mem0.shape[1]
    F = B_w_gate.shape[1]
    T = int(A_seg_len)
    assert (B, S, D, H, E, M, T) == (1, 2048, 512, 32, 128, 8, 32)
    NG = S // (T * GS)
    NHG = H // 8
    hbm = pl.BlockSpec(memory_space=pl.ANY)
    vmem = pl.BlockSpec(memory_space=pltpu.VMEM)
    out = pl.pallas_call(
        functools.partial(_kernel, S=S, D=D, H=H, E=E, M=M, T=T),
        out_shape=jax.ShapeDtypeStruct((NG, GS, T, D), A_x.dtype),
        in_specs=[hbm, vmem, hbm, hbm, hbm, hbm, vmem, hbm, hbm, hbm],
        out_specs=hbm,
        scratch_shapes=[
            pltpu.VMEM((3 * NHG, D, 8, E), BF),
            pltpu.VMEM((NHG, 8, E, D), BF),
            pltpu.VMEM((3 * H // 4, 49, E // 2, E), U32),
            pltpu.VMEM((49, H // 4 * E // 2, E), U32),
            pltpu.VMEM((NG + 1, GS, T, D), BF),
            pltpu.VMEM((2, NG + 1, GS, T, D), F32),
            pltpu.VMEM((NG, GS, T, D), F32),
            pltpu.VMEM((51, T, E), F32),
            pltpu.VMEM((2, 3 * H // 4, GS * 4 * T, E), F32),
            pltpu.VMEM((2, GS, 4, T, H // 4 * E), F32),
            pltpu.VMEM((2, GS, T, D), F32),
            pltpu.VMEM((M + 8, D), F32),
            pltpu.VMEM((8, 512), I32),
            pltpu.VMEM((D, F), BF),
            pltpu.VMEM((D, F), BF),
            pltpu.VMEM((F, D), BF),
            pltpu.SMEM((1,), I32),
            pltpu.SemaphoreType.DMA((4 * NHG + 6,)),
        ],
        compiler_params=pltpu.CompilerParams(vmem_limit_bytes=120 * 2**20),
        name="rmt_mod",
    )(
        A_x.reshape(NG, GS, T, D), A_mem0.reshape(M, D),
        A_Wq.reshape(D, NHG, 8, E), A_Wk.reshape(D, NHG, 8, E), A_Wv.reshape(D, NHG, 8, E),
        A_Wo.reshape(NHG, 8, E, D),
        B_w_r, B_w_gate, B_w_up, B_w_down,
    )
    return out.reshape(B, S, D)
```

```python
import functools

import numpy as np
import jax
import jax.numpy as jnp
from jax import lax
import jax.experimental.pallas as pl
import jax.experimental.pallas.tpu as pltpu

BF = jnp.bfloat16
F32 = jnp.float32
U32 = jnp.uint32
I32 = jnp.int32

GS = 4

LHS = {1: ((0, 0, 1), (1, 1, 1)), 2: ((1, 0, 1), (1, 1, 1)), 3: ((0, 0, 1),), 4: ((1, 1, 1),),
       5: ((0, 0, 1), (0, 1, 1)), 6: ((1, 0, 1), (0, 0, -1)), 7: ((0, 1, 1), (1, 1, -1))}
RHS = {1: ((0, 0, 1), (1, 1, 1)), 2: ((0, 0, 1),), 3: ((0, 1, 1), (1, 1, -1)), 4: ((1, 0, 1), (0, 0, -1)),
       5: ((1, 1, 1),), 6: ((0, 0, 1), (0, 1, 1)), 7: ((1, 0, 1), (1, 1, 1))}
OUT = {(0, 0): ((4, 1), (7, 1), (1, 1), (5, -1)), (0, 1): ((3, 1), (5, 1)),
       (1, 0): ((2, 1), (4, 1)), (1, 1): ((3, 1), (6, 1), (1, 1), (2, -1))}
BASIS = ((3, 1, 5, 7), (4, 1, 2, 6))
PHASES = ((1, 1, 0), (1, 0, 1), (0, 0, 0), (0, 1, 1))

SEQ_FULL = (
    "xx....A............q......q........p......q......p......q......p......EqEEE......p......q.....p.........q....p....q..oooooopooooopoooooooHoooooooooooooo",
    "x........A........q........q......p......q.....p.......q......p......EEqEE..p..........q.....p.......q......p......qoooooopooooopoooHoooooooooooooooooo",
    "xx........A.........q.......q.......p.........q...p.....qEEEE.........q.p.....p.........q......p......q......p......qooooopooooopooooHoooooooooooooooooo",
    "x........A........q........q......p......q......p......q....p........qEE..p...E..E.....q....p........q......p......qoooooopooooopoooHoooooooooooooooooo",
    "xx........A.........q.......q.......p.........q...p.....qEEEE.........q.p.....p.........q......p......q......p......qooooopooooopooooHoooooooooooooooooo",
    "x........A........q........q......p......q.....p.......q......p......EEqEE..p..........q.....p...........q..p......qoooooopooooopoooHoooooooooooooooooo",
    "xx........A.........q.......q.......p.........q...p.....qEEEE.........q.p.....p.........q......p......q......p......qooooopooooopooooHoooooooooooooooooo",
    "x........A........q........q......p......q......p......q....p........qEE..p...E.E......q....p........q......p......qoooooopooooopoooHoooooooooooooooooo",
)


def _rb(v):
    return v.astype(BF).astype(F32)


def _layernorm(x):
    inv_n = 1.0 / x.shape[-1]
    m = jnp.sum(x, axis=-1, keepdims=True) * inv_n
    d = x - m
    v = _rb(jnp.sum(d * d, axis=-1, keepdims=True) * inv_n)
    den = _rb(jnp.sqrt(_rb(v + 1.0013580322265625e-05)))
    return _rb(_rb(x - _rb(m)) * (1.0 / den))


def _sigmoid(x):
    return _rb(1.0 / _rb(1.0 + _rb(jnp.exp(-x))))


def _dot(a, b):
    return jnp.dot(a, b, preferred_element_type=F32)


def _signed_sum(terms):
    terms = sorted(terms, key=lambda t: -t[1])
    total = terms[0][0] if terms[0][1] > 0 else -terms[0][0]
    for v, sign in terms[1:]:
        total = total + v if sign > 0 else total - v
    return total


def _left_operand(a, b, block, rows=None):
    return _signed_sum([(block(2 * i + k, 2 * j + l), s * t) for i, j, s in LHS[a] for k, l, t in LHS[b]
                        if rows is None or 2 * i + k == rows])


def _output(pos, prods):
    terms = [(prods[m], s) for m, s in OUT[pos] if prods.get(m) is not None]
    return _signed_sum(terms) if terms else None


def _weight_operands(block):
    vals = []
    for a in RHS:
        outer = {(k, l): _signed_sum([(block(2 * i + k, 2 * j + l), s) for i, j, s in RHS[a]])
                 for k in range(2) for l in range(2)}
        for b in RHS:
            vals.append(_signed_sum([(outer[k, l], t) for k, l, t in RHS[b]]))
            if len(vals) == 2 or a == b == 7:
                w = pltpu.bitcast(jnp.concatenate(vals, axis=1).astype(BF), U32)
                yield from (w[:, c:c + 128] for c in range(0, w.shape[1], 128))
                vals = []


class _Phase:
    def __init__(self, u):
        h0, h1, self.wide = PHASES[u]
        self.u, self.row = u, 2 * h0 + h1
        self.ws, self.ns = (BASIS[h] for h in ((h0, h1) if self.wide == 0 else (h1, h0)))

    def pair(self, w, n):
        return (w, n) if self.wide == 0 else (n, w)

    def index(self, w, n):
        a, b = self.pair(w, n)
        return 7 * (a - 1) + b - 1

    def place(self, pw, pn):
        (i, j), (k, l) = self.pair(pw, pn)
        return 2 * i + k, 2 * j + l

    def touched(self):
        return {self.place(pw, pn) for pw in OUT for pn in OUT
                if any(m in self.ws for m, _ in OUT[pw] if m != 1) and any(m in self.ns for m, _ in OUT[pn] if m != 1)}

    def run(self, product, emit, wide_first, order=None):
        first, second = (self.ws, self.ns) if wide_first else (self.ns, self.ws)
        second = order or second
        partial = {}
        for m2 in second:
            got = {}
            for m1 in first:
                for t, v in product(*((m1, m2) if wide_first else (m2, m1))).items():
                    got.setdefault(t, {})[m1] = v
                if m1 != first[-1]:
                    yield
            for t, prods in got.items():
                for p1 in OUT:
                    partial.setdefault((t, p1), {})[m2] = _output(p1, prods)
            for p2, terms in OUT.items():
                need = [m for m in second if m in dict(terms)]
                if need and need[-1] == m2:
                    for (t, p1), prods in partial.items():
                        i, j = self.place(*((p1, p2) if wide_first else (p2, p1)))
                        if (i == self.row) if t is None else ((i, j) in self.touched()):
                            emit(i, j, t, _output(p2, prods))
            yield


def _kernel(x_hbm, mem0_ref, wq_hbm, wk_hbm, wv_hbm, wo_hbm, wr_ref, wg_hbm, wu_hbm, wd_hbm,
            out_hbm,
            raw, wo_raw, wqkv, wout, xbuf, xmid, hbuf, hl, qkv, obuf, oacc, state, bidx_ref,
            wg_s, wu_s, wd_s, late, sems,
            *, S, D, H, E, M, T):
    NG = S // (T * GS)
    L = M + T
    NQ = H // 4
    NHG = H // 8
    NC = 3 * NHG
    w_hbm = (wq_hbm, wk_hbm, wv_hbm)
    phases = [_Phase(u) for u in range(GS)]

    def cp_w(c):
        return pltpu.make_async_copy(w_hbm[c // NHG].at[:, c % NHG], raw.at[c], sems.at[c])

    def cp_o(k):
        return pltpu.make_async_copy(wo_hbm.at[k], wo_raw.at[k], sems.at[NC + k])

    cp_x = [pltpu.make_async_copy(x_hbm.at[pl.ds(lo, hi - lo)], xbuf.at[pl.ds(lo, hi - lo)], sems.at[NC + NHG + k])
            for k, (lo, hi) in enumerate(((0, 3), (3, 5), (5, NG)))]
    cp_out = [pltpu.make_async_copy(xbuf.at[pl.ds(lo, hi - lo)], out_hbm.at[pl.ds(lo, hi - lo)], sems.at[NC + NHG + k])
              for k, (lo, hi) in enumerate(((0, NG - 4), (NG - 4, NG)))]
    cp_b = [pltpu.make_async_copy(w, s, sems.at[NC + NHG + 3 + j])
            for j, (w, s) in enumerate(((wg_hbm, wg_s), (wu_hbm, wu_s), (wd_hbm, wd_s)))]

    def normed(x):
        x = x.astype(F32)
        d = x - jnp.sum(x, axis=-1, keepdims=True) * (1.0 / D)
        return d * lax.rsqrt(jnp.sum(d * d, axis=-1, keepdims=True) * (1.0 / D) + 1e-5)

    def prenorm(g, u):
        hbuf[g, u] = normed(xbuf[g, u])

    def rows_of(tiles):
        return pl.ds(tiles[0] * 8, len(tiles) * 8)

    def build_lhs(g, ph):
        for n in ph.ns:
            for w in ph.ws:
                if n != 1 or (w, ph.u) == (1, 0):
                    hl[ph.index(w, n)] = _left_operand(*ph.pair(w, n), lambda s, k: hbuf[g, s, :, pl.ds(k * E, E)])

    def accumulate(ref, ph, i, j, index, v):
        seen = any((i, j) in p.touched() for p in phases[:ph.u])
        ref[index] = v + ref[index] if seen else v

    def first_product(blk):
        return _dot(hl[0], pltpu.bitcast(wqkv[blk, 0], BF))

    def qkv_block(ph, par, blk, mem_lhs, mem_out, first):
        def product(w, n):
            left = [hl[ph.index(w, n)]] if n != 1 else []
            left += [mem_lhs[w, n]] if mem_lhs else []
            out = {0: first} if (w, n) == (1, 1) else {}
            if left:
                res = _dot(jnp.concatenate(left, axis=0), pltpu.bitcast(wqkv[blk, ph.index(w, n)], BF))
                if n != 1:
                    out[0] = res[:T]
                if mem_lhs:
                    out[None] = res[-M:]
            return out

        def emit(i, j, t, v):
            if t is None:
                mem_out[j] = v
            else:
                accumulate(qkv, ph, i, j, (par, blk, pl.ds((4 * i + j) * T, T)), v)
        return ph.run(product, emit, True)

    def out_rounds(ph, par, mem_in, mem_out):
        def tiles_of(w, n):
            if (w, n) == (1, 1):
                return range(ph.u, ph.u + 1) if mem_in else range(4 * (ph.u == 0))
            return range(4 * (n != 1))

        def half(w, n, k):
            tiles = tiles_of(w, n)
            left = [_left_operand(*ph.pair(w, n), lambda s, j: mem_in(j, k), ph.row)] if mem_in else []
            if tiles:
                left += [_left_operand(*ph.pair(w, n),
                                       lambda s, j: obuf[par, s, j, rows_of(tiles), pl.ds(k * 4 * E, 4 * E)])]
            if left:
                return _dot(jnp.concatenate(left, axis=0),
                            pltpu.bitcast(wout[ph.index(w, n), pl.ds(k * 2 * E, 2 * E)], BF))

        def product(w, n):
            res = half(w, n, 1)
            if res is None:
                return {}
            res = res + early[w, n]
            return {t: res[8 * k:8 * k + 8] for k, t in enumerate([None] * bool(mem_in) + list(tiles_of(w, n)))}

        def emit(i, j, t, v):
            if t is None:
                mem_out[j] = v
            else:
                accumulate(oacc, ph, i, j, (par, i, pl.ds(t * 8, 8), pl.ds(j * E, E)), v)
        early = {}
        for w in ph.ws[::-1]:
            for n in ph.ns:
                early[w, n] = half(w, n, 0)
                yield
        yield from ph.run(product, emit, False, ph.ws[::-1])

    cp_w(0).start()
    cp_x[0].start()
    for c in range(1, NC):
        cp_w(c).start()
    for k in range(NHG):
        cp_o(k).start()
    for c in cp_x[1:] + cp_b:
        c.start()
    xbuf[NG] = jnp.zeros((GS, T, D), BF)
    oacc[0] = jnp.zeros(oacc.shape[1:], F32)
    obuf[1] = jnp.zeros(obuf.shape[1:], F32)

    def prep_qkv(c):
        for r in range(E // 16):
            for k in range(4):
                words = pltpu.bitcast(raw[c, pl.ds(k * E + r * 16, 16)].reshape(128, E), U32)
                qkv[1, r, pl.ds(k * 64, 64)] = pltpu.bitcast(words, F32)
        for r in range(E // 16):
            for n in range(2):
                def block(k, j):
                    w = pltpu.bitcast(qkv[1, r, pl.ds(k * 64 + 2 * n + j // 2, 16, stride=4), :], U32)
                    return pltpu.bitcast(w & np.uint32(0xFFFF0000) if j % 2 else w << 16, F32)
                for m, w in enumerate(_weight_operands(block)):
                    wqkv[2 * c + n, m, pl.ds(r * 8, 8)] = w

    def prep_out(k):
        for r in range(E // 16):
            for n in range(2):
                heads = [wo_raw[k, 4 * n + i, pl.ds(r * 16, 16)].astype(F32) for i in range(4)]
                for m, w in enumerate(_weight_operands(lambda i, j: heads[i][:, j * E:j * E + E])):
                    wout[m, pl.ds(pl.multiple_of((2 * k + n) * (E // 2) + r * 8, 8), 8)] = w

    def project_first(c):
        for ph in phases:
            for blk in (2 * c, 2 * c + 1):
                list(qkv_block(ph, 0, blk, None, None, None if ph.u else first_product(blk)))

    cp_w(0).wait()
    prep_qkv(0)
    cp_x[0].wait()
    hbuf[:3] = normed(xbuf[:3].reshape(3 * GS * T, D)).reshape(3, GS, T, D)
    for ph in phases:
        build_lhs(0, ph)

    def stream(c, carry):
        pltpu.make_async_copy(raw.at[c + 1], raw.at[c + 1], sems.at[c + 1]).wait()
        prep_qkv(c + 1)
        project_first(c)
        return carry
    lax.fori_loop(0, NC - 1, stream, 0)
    project_first(NC - 1)
    build_lhs(1, phases[0])

    def stream_o(k, carry):
        cp_o(k).wait()
        prep_out(k)
        return carry
    lax.fori_loop(0, NHG, stream_o, 0)
    cp_x[1].wait()

    def reset_memory():
        state[:M] = mem0_ref[...].astype(F32)

    def reset_router():
        state[M:] = jnp.full((8, D), -jnp.inf, F32)
        bidx_ref[:, :128] = jnp.full((8, 128), S, I32)
    reset_memory()
    reset_router()

    def router(xn):
        return _rb(jnp.sum(xn * wr_ref[...].astype(F32).reshape(1, D), axis=-1, keepdims=True))

    def epilogue(g, u, t, par, best, bidx):
        rows = pl.ds(t * 8, 8)
        x1 = _rb(xbuf[g, u, rows].astype(F32) + _rb(oacc[par, u, rows]))
        xn = _layernorm(x1)
        xmid[0, g, u, rows] = x1
        xmid[1, g, u, rows] = xn
        xbuf[g, u, rows] = (x1 + xn).astype(BF)
        it = lax.broadcasted_iota(I32, (8, 128), 0) + ((g * GS + u) * T + t * 8)
        r = jnp.where(it < S, jnp.broadcast_to(router(xn), (8, 128)), -jnp.inf)
        better = r > best
        return jnp.where(better, r, best), jnp.where(better, it, bidx)

    def segment(par, ph, mem, seq, jobs, firsts, first_rounds):
        u = ph.u
        row = lax.broadcasted_iota(I32, (L, L), 0)
        col = lax.broadcasted_iota(I32, (L, L), 1)
        mask = (row < M) | (row >= col)
        mem_lhs = {(w, n): _left_operand(*ph.pair(w, n), lambda s, k: mem[k], ph.row) for n in ph.ns for w in ph.ws}
        proj = [{} for _ in range(3 * NQ)]
        probs, outs, new_mem = {}, {}, {}

        def head(j, n, i):
            return jnp.concatenate([proj[j * NQ + n][i], qkv[par, j * NQ + n, pl.ds((4 * u + i) * T, T)]], axis=0)

        def scores(n):
            for i in range(4):
                sc = lax.dot_general(head(0, n, i), head(1, n, i).astype(BF), (((1,), (1,)), ((), ())),
                                     preferred_element_type=F32)
                sc = jnp.where(mask, sc, -1e9 * E ** 0.5)
                e = jnp.exp2((sc - jnp.max(sc, axis=-1, keepdims=True)) * (E ** -0.5 * 1.4426950408889634))
                probs[n, i] = e * pltpu.reciprocal(jnp.sum(e, axis=-1, keepdims=True), full_range=False)

        def values(n):
            for i in range(4):
                o = _dot(probs[n, i], head(2, n, i).astype(BF))
                outs[n, i] = o[:M]
                obuf[par, u, i, :, pl.ds(n * E, E)] = o[M:]

        def rounds():
            order = [(j, n - (j == 2)) for n in range(NQ + 1) for j in range(3) if 0 <= n - (j == 2) < NQ]
            for blk in (j * NQ + n for j, n in order):
                for k, _ in enumerate(qkv_block(ph, 1 - par, blk, mem_lhs, proj[blk], firsts.pop(blk, None))):
                    if k % 4 == 3:
                        yield

        def mem_in(i, k):
            return jnp.concatenate([outs[n, i] for n in range(4 * k, 4 * k + 4)], axis=1)
        its = {".": rounds(), "o": out_rounds(ph, 1 - par, mem_in, new_mem),
               "q": map(scores, range(NQ)), "p": map(values, range(NQ))}
        its.update({ch: (f() for f in fs) for ch, fs in jobs.items()})
        assert "x" not in seq.lstrip("x")
        for ch in seq:
            next(first_rounds if ch == "x" else its[ch])
        assert not any(list(it) for it in its.values())
        return [_rb(new_mem[j]) for j in range(4)]

    def group_pair(G0, pending):
        mem, top = [state[:M, pl.ds(j * E, E)] for j in range(4)], [state[M:, :128], bidx_ref[:, :128]]
        for par in range(2):
            G = G0 + par
            g = G % NG

            def post(u, t):
                top[:] = epilogue(jnp.where(g >= 2, g - 2, jnp.where(pending, g + NG - 2, NG)), u, t, par, *top)
                hl[49 + G0 // NG, :8] = top[0]

            firsts = {}
            first_rounds = (firsts.update({blk: first_product(blk) for blk in range(k, k + 4)})
                            for k in range(0, 3 * NQ, 4))
            for u in range(GS):
                mem = segment(par, phases[u], mem, SEQ_FULL[par * GS + u], {
                    "H": [functools.partial(prenorm, (G + 3) % NG, u)],
                    "A": [functools.partial(build_lhs, (G + 1 + (u + 1) // GS) % NG, phases[(u + 1) % GS])],
                    "E": [functools.partial(post, u, t) for t in range(T // 8)]}, firsts, first_rounds)
            assert not firsts and not list(first_rounds)
        for j in range(4):
            state[:M, pl.ds(j * E, E)] = mem[j]
        state[M:, :128], bidx_ref[:, :128] = top

    def drain():
        best, bidx = state[M:, :128], bidx_ref[:, :128]
        for ph in phases:
            list(out_rounds(ph, 1, None, None))
        for par in range(2):
            for u in range(GS):
                for t in range(T // 8):
                    best, bidx = epilogue(NG - 2 + par, u, t, par, best, bidx)
        state[M:, :128], bidx_ref[:, :128] = best, bidx

    def top_token():
        best = state[M:, :128]
        idx = jnp.min(jnp.where(best == jnp.max(best, axis=0, keepdims=True), bidx_ref[:, :128], S))
        return jnp.where(idx >= S, 0, idx)

    def expert(last, nxt):
        idx = top_token()
        g, u = idx // (T * GS), idx // T % GS
        tile = pl.multiple_of(idx % T // 8 * 8, 8)
        rows = pl.ds(tile, 8)
        x1, xn = xmid[0, g, u, rows], xmid[1, g, u, rows]
        gate = _rb(_dot(xn, wg_s[...]))
        up = _rb(_dot(xn, wu_s[...]))
        gate = _rb(gate * _sigmoid(gate))
        y = _rb(_dot(_rb(gate * up), wd_s[...]))
        y = _rb(y * _sigmoid(router(xn)))
        sel = lax.broadcasted_iota(I32, (8, D), 0) == idx % 8
        x2 = (x1 + _rb(xn + jnp.where(sel, y, 0.0))).astype(BF)

        @pl.when(last)
        def _():
            cp_out[0].wait()
            cp_out[1].wait()
            xbuf[g, u, rows] = x2
            cp = pltpu.make_async_copy(xbuf.at[g, u], out_hbm.at[g, u], sems.at[0])
            cp.start()
            cp.wait()

        @pl.when(jnp.logical_not(last))
        def _():
            xbuf[g, u, rows] = x2
            h = normed(x2)
            hbuf[g, u, rows] = h
            build_lhs(nxt + 1, phases[0])
            reset_router()

            @pl.when(g == nxt)
            def _():
                ph = phases[0]
                left = {(w, n): _left_operand(*ph.pair(w, n), lambda s, k: h[:, k * E:k * E + E], ph.row)
                        for n in ph.ns for w in ph.ws}

                def redo(blk, carry):
                    def product(w, n):
                        return {None: _dot(left[w, n], pltpu.bitcast(wqkv[blk, ph.index(w, n)], BF))}

                    def emit(i, j, t, v):
                        qkv[0, blk, pl.ds(pl.multiple_of((4 * u + j) * T + tile, 8), 8)] = v
                    list(ph.run(product, emit, True))
                    return carry
                lax.fori_loop(0, 3 * NQ, redo, 0, unroll=4)

    def iteration(it, carry):
        last = it == NG - 1
        seam = it == NG // 2 - 1
        pending = late[0] == 1

        @pl.when(it == 1)
        def _():
            for c in cp_x[2:] + cp_b:
                c.wait()

        @pl.when(last)
        def _():
            cp_out[0].start()
        group_pair(2 * it, pending)
        late[0] = 0

        @pl.when(seam)
        def _():
            late[0] = (top_token() >= 2 * GS * T).astype(I32)
            reset_memory()
        now = last | (seam & (late[0] == 0))
        pl.when(now)(drain)

        @pl.when(last)
        def _():
            cp_out[1].start()
        pl.when(now | pending)(lambda: expert(last, jnp.where(pending, 2, 0)))
        return carry

    late[0] = 0
    lax.fori_loop(0, NG, iteration, 0)


@functools.partial(jax.jit, static_argnames=("A_seg_len",))
def pallas_interleave_layers__memory_aug_recurrent_mem_tr__moe_arch_mod__prompt_kernel(
    A_x, A_mem0, A_Wq, A_Wk, A_Wv, A_Wo, A_seg_len, B_x, B_w_r, B_w_gate, B_w_up, B_w_down,
):
    del B_x
    B, S, D = A_x.shape
    _, H, E = A_Wq.shape
    M = A_mem0.shape[1]
    F = B_w_gate.shape[1]
    T = int(A_seg_len)
    assert (B, S, D, H, E, M, T) == (1, 2048, 512, 32, 128, 8, 32)
    NG = S // (T * GS)
    NHG = H // 8
    hbm = pl.BlockSpec(memory_space=pl.ANY)
    vmem = pl.BlockSpec(memory_space=pltpu.VMEM)
    out = pl.pallas_call(
        functools.partial(_kernel, S=S, D=D, H=H, E=E, M=M, T=T),
        out_shape=jax.ShapeDtypeStruct((NG, GS, T, D), A_x.dtype),
        in_specs=[hbm, vmem, hbm, hbm, hbm, hbm, vmem, hbm, hbm, hbm],
        out_specs=hbm,
        scratch_shapes=[
            pltpu.VMEM((3 * NHG, D, 8, E), BF),
            pltpu.VMEM((NHG, 8, E, D), BF),
            pltpu.VMEM((3 * H // 4, 49, E // 2, E), U32),
            pltpu.VMEM((49, H // 4 * E // 2, E), U32),
            pltpu.VMEM((NG + 1, GS, T, D), BF),
            pltpu.VMEM((2, NG + 1, GS, T, D), F32),
            pltpu.VMEM((NG, GS, T, D), F32),
            pltpu.VMEM((51, T, E), F32),
            pltpu.VMEM((2, 3 * H // 4, GS * 4 * T, E), F32),
            pltpu.VMEM((2, GS, 4, T, H // 4 * E), F32),
            pltpu.VMEM((2, GS, T, D), F32),
            pltpu.VMEM((M + 8, D), F32),
            pltpu.VMEM((8, 512), I32),
            pltpu.VMEM((D, F), BF),
            pltpu.VMEM((D, F), BF),
            pltpu.VMEM((F, D), BF),
            pltpu.SMEM((1,), I32),
            pltpu.SemaphoreType.DMA((4 * NHG + 6,)),
        ],
        compiler_params=pltpu.CompilerParams(vmem_limit_bytes=120 * 2**20),
        name="rmt_mod",
    )(
        A_x.reshape(NG, GS, T, D), A_mem0.reshape(M, D),
        A_Wq.reshape(D, NHG, 8, E), A_Wk.reshape(D, NHG, 8, E), A_Wv.reshape(D, NHG, 8, E),
        A_Wo.reshape(NHG, 8, E, D),
        B_w_r, B_w_gate, B_w_up, B_w_down,
    )
    return out.reshape(B, S, D)
```
